```python
import os as _os
_os.environ.setdefault("JAX_PLATFORMS", "cpu")
import jax
import jax.numpy as jnp

def _softmax(x, axis=-1):
    return jax.nn.softmax(x, axis=axis)
def _gelu(x):
    return jax.nn.gelu(x, approximate=True)
def _silu(x):
    return jax.nn.silu(x)
def _sigmoid(x):
    return jax.nn.sigmoid(x)
def _layernorm(x, axis=-1, eps=1e-5):
    m = jnp.mean(x, axis=axis, keepdims=True)
    v = jnp.var(x, axis=axis, keepdims=True)
    return (x - m) / jnp.sqrt(v + eps)
def _scatter_add(tgt, idx, src, axis=0):
    return tgt.at[idx].add(src)
def _segment_sum(src, seg, n):
    return jax.ops.segment_sum(src, seg, n)
class _Rng:
    def __init__(self, key):
        self._k = key
    def _next(self):
        self._k, sub = jax.random.split(self._k)
        return sub
    def normal(self, shape):
        return jax.random.normal(self._next(), shape, dtype=jnp.bfloat16)
    def randint(self, lo, hi, shape):
        return jax.random.randint(self._next(), shape, lo, hi, dtype=jnp.int32)
    def uniform(self, shape, lo=0.0, hi=1.0):
        return jax.random.uniform(self._next(), shape, jnp.bfloat16, lo, hi)
    def permutation(self, n):
        return jax.random.permutation(self._next(), n)


kernel_name = 'concat_heads__gqa_block_cached__mha_block_cached__near_ridge'

def setup_inputs():
    _rng = _Rng(jax.random.key(int.from_bytes(__import__("os").urandom(4), "little")))
    _w = (lambda a: (lambda t: t.astype(jnp.bfloat16) if jnp.issubdtype(t.dtype, jnp.floating) else t)(jnp.asarray(a)))
    def _A_setup():
        B, Sq, D = 16, 32, 1024
        Hq, Hkv, Sk, Dh = 32, 4, 32, 128
        assert Hq % Hkv == 0, (Hq, Hkv)
        return {
            "x": _w((lambda *s: _rng.normal(s) * 0.8)(B, Sq, D)),
            "k_cache": _w((lambda *s: _rng.normal(s) * 0.8)(B, Hkv, Sk, Dh)),
            "v_cache": _w((lambda *s: _rng.normal(s) * 0.05)(B, Hkv, Sk, Dh)),
            "wq": _w((lambda *s: _rng.normal(s) * 0.8)(D, Hq * Dh) * (D ** -0.5)),
            "wo": _w((lambda *s: _rng.normal(s) * 0.05)(Hq * Dh, D) * ((Hq * Dh) ** -0.5)),
        }
    _A_in = _A_setup()

    def _B_setup():
        B, Sq, D = 16, 32, 1024
        H, Sk, Dh = 32, 32, 128
        return {
            "x": _w((lambda *s: _rng.normal(s) * 0.8)(B, Sq, D)),
            "k_cache": _w((lambda *s: _rng.normal(s) * 0.8)(B, H, Sk, Dh)),
            "v_cache": _w((lambda *s: _rng.normal(s) * 0.05)(B, H, Sk, Dh)),
            "wq": _w((lambda *s: _rng.normal(s) * 0.8)(D, H * Dh) * (D ** -0.5)),
            "wo": _w((lambda *s: _rng.normal(s) * 0.05)(H * Dh, D) * ((H * Dh) ** -0.5)),
        }
    _B_in = _B_setup()

    return {
        "A_x": _A_in["x"],
        "A_k_cache": _A_in["k_cache"],
        "A_v_cache": _A_in["v_cache"],
        "A_wq": _A_in["wq"],
        "A_wo": _A_in["wo"],
        "B_x": _B_in["x"],
        "B_k_cache": _B_in["k_cache"],
        "B_v_cache": _B_in["v_cache"],
        "B_wq": _B_in["wq"],
        "B_wo": _B_in["wo"],
    }

def reference(A_x, A_k_cache, A_v_cache, A_wq, A_wo, B_x, B_k_cache, B_v_cache, B_wq, B_wo):
    def _A_ref(x, k_cache, v_cache, wq, wo):
        B, Sq, D = x.shape
        Hq, Dh = 32, 128
        Hkv = k_cache.shape[1]
        rep = Hq // Hkv
        q = (lambda x, *d: x.transpose(*d))((x @ wq).reshape(B, Sq, Hq, Dh), 0, 2, 1, 3)
        k = jnp.repeat(k_cache, rep, axis=1)
        v = jnp.repeat(v_cache, rep, axis=1)
        scores = jnp.einsum("bhqd,bhkd->bhqk", q, k) * (Dh ** -0.5)
        p = _softmax(scores, axis=-1)
        o = jnp.einsum("bhqk,bhkd->bhqd", p, v)
        return (lambda x, *d: x.transpose(*d))(o, 0, 2, 1, 3).reshape(B, Sq, Hq * Dh) @ wo

    def _B_ref(x, k_cache, v_cache, wq, wo):
        B, Sq, D = x.shape
        H, Dh = 32, 128
        q = (lambda x, *d: x.transpose(*d))((x @ wq).reshape(B, Sq, H, Dh), 0, 2, 1, 3)
        scores = jnp.einsum("bhqd,bhkd->bhqk", q, k_cache) * (Dh ** -0.5)
        p = _softmax(scores, axis=-1)
        o = jnp.einsum("bhqk,bhkd->bhqd", p, v_cache)
        return (lambda x, *d: x.transpose(*d))(o, 0, 2, 1, 3).reshape(B, Sq, H * Dh) @ wo

    a = _A_ref(A_x, A_k_cache, A_v_cache, A_wq, A_wo)
    b = _B_ref(B_x, B_k_cache, B_v_cache, B_wq, B_wo)
    return jnp.concatenate([a, b], axis=-1)
```

```python
import functools
import numpy as np
import jax
import jax.numpy as jnp
from jax import lax
import jax.experimental.pallas as pl
import jax.experimental.pallas.tpu as pltpu

B, SQ, D, H, HKV, SK, DH = 16, 32, 1024, 32, 4, 32, 128
M = B * SQ
HPS = 4
CH = HPS * DH
NSB = H // HPS
NS = 2 * NSB
NQ = HPS // 4
C_EXP2 = float(DH ** -0.5 * np.log2(np.e))
NT = (((1,), (1,)), ((), ()))
NN = (((1,), (0,)), ((), ()))
F32 = jnp.float32
BF16 = jnp.bfloat16


def _softmax_cols(sc):
    m = jnp.max(sc, axis=0, keepdims=True)
    p = jnp.exp2((sc - m) * C_EXP2)
    l = jnp.sum(p, axis=0, keepdims=True)
    return p * (1.0 / l)


def _kernel(xa, ka, va, wqa, woa, xb, kb, vb, wqb, wob, out,
            x_buf, ka_buf, va_buf, kb_buf, vb_buf, wq_buf, wo_buf,
            q_buf, o_buf, acc, out_buf,
            sems):
    class _S:
        def __init__(self, base): self.base = base
        @property
        def at(self): return self
        def __getitem__(self, i): return sems.at[self.base + i]
    sem_x, sem_kva, sem_kb, sem_vb, sem_wq, sem_wo, sem_out = (
        _S(0), _S(2), _S(4), _S(4 + NSB), _S(4 + 2 * NSB), _S(4 + 2 * NSB + NS), _S(4 + 2 * NSB + 2 * NS))


    def wq_copy(s):
        src = wqa if s < NSB else wqb
        return pltpu.make_async_copy(src.at[:, pl.ds((s % NSB) * CH, CH)], wq_buf.at[s], sem_wq.at[s])

    def wo_copy(s):
        src = woa if s < NSB else wob
        return pltpu.make_async_copy(src.at[pl.ds((s % NSB) * CH, CH), :], wo_buf.at[s], sem_wo.at[s])

    def x_copy(br):
        return pltpu.make_async_copy(xa if br == 0 else xb, x_buf.at[br], sem_x.at[br])

    def ka_copy():
        return pltpu.make_async_copy(ka, ka_buf, sem_kva.at[0])

    def va_copy():
        return pltpu.make_async_copy(va, va_buf, sem_kva.at[1])

    def kb_copy(j):
        return pltpu.make_async_copy(kb.at[:, pl.ds(j * NQ, NQ)], kb_buf.at[:, pl.ds(j * NQ, NQ)], sem_kb.at[j])

    def vb_copy(j):
        return pltpu.make_async_copy(vb.at[:, pl.ds(j * NQ, NQ)], vb_buf.at[:, pl.ds(j * NQ, NQ)], sem_vb.at[j])

    def out_copy(br):
        return pltpu.make_async_copy(out_buf.at[br], out.at[:, pl.ds(br * D, D)], sem_out.at[br])

    def wait_wq(s):
        pltpu.make_async_copy(wq_buf.at[s], wq_buf.at[s], sem_wq.at[s]).wait()

    def wait_wo(s):
        pltpu.make_async_copy(wo_buf.at[s], wo_buf.at[s], sem_wo.at[s]).wait()

    def wait_kvb(j):
        dst = kb_buf.at[:, pl.ds(j * NQ, NQ)]
        pltpu.make_async_copy(dst, dst, sem_kb.at[j]).wait()
        dst = vb_buf.at[:, pl.ds(j * NQ, NQ)]
        pltpu.make_async_copy(dst, dst, sem_vb.at[j]).wait()

    x_copy(0).start()
    wq_copy(0).start()
    ka_copy().start()
    wq_copy(1).start()
    va_copy().start()
    for s in range(1, NS):
        if s >= NSB:
            kb_copy(s - NSB).start()
        wo_copy(s - 1).start()
        if s >= NSB:
            vb_copy(s - NSB).start()
        if s + 1 == NSB:
            x_copy(1).start()
        if s + 1 < NS:
            wq_copy(s + 1).start()
    wo_copy(NS - 1).start()

    acc[...] = jnp.zeros(acc.shape, F32)

    lane_g = lax.broadcasted_iota(jnp.int32, (32, 128), 1) // 32

    def qproj(s, br):
        q_buf[...] = jnp.dot(x_buf[br], wq_buf[s], preferred_element_type=F32).astype(BF16)

    def oproj(s, br):
        acc[br] += jnp.dot(o_buf[...], wo_buf[s], preferred_element_type=F32)

    def q4_of(b, hq):
        return jnp.concatenate(
            [q_buf[b * 32:(b + 1) * 32, (hq * 4 + h) * DH:(hq * 4 + h + 1) * DH] for h in range(4)], axis=0)

    def qk(j, is_a):
        res = []
        for hq in range(NQ):
            for bb in range(4):
                pts = []
                for bi in range(4):
                    b = bb * 4 + bi
                    q4 = q4_of(b, hq)
                    if is_a:
                        g = (j * NQ + hq) // 2
                        sc = lax.dot_general(ka_buf[b, g], q4, NT, preferred_element_type=F32)
                    else:
                        st = lax.dot_general(kb_buf[b, j * NQ + hq], q4, NT, preferred_element_type=F32)
                        sc = st[0:32]
                        for h in range(1, 4):
                            sc = jnp.where(lane_g == h, st[h * 32:(h + 1) * 32], sc)
                    pts.append(_softmax_cols(sc))
                res.append(jnp.concatenate(pts, axis=0).T)
        return res

    def pv(j, is_a, tts):
        for hq in range(NQ):
            for bb in range(4):
                tt = tts[hq * 4 + bb]
                for h in range(4):
                    ph = tt[h * 32:(h + 1) * 32]
                    lhs = jnp.concatenate(
                        [jnp.where(lane_g == bi, ph, 0.0) for bi in range(4)], axis=0).astype(BF16)
                    if is_a:
                        g = (j * NQ + hq) // 2
                        vh = jnp.concatenate([va_buf[bb * 4 + bi, g] for bi in range(4)], axis=0)
                    else:
                        vh = jnp.concatenate(
                            [vb_buf[bb * 4 + bi, j * NQ + hq, h * 32:(h + 1) * 32, :] for bi in range(4)], axis=0)
                    o = lax.dot_general(lhs, vh, NN, preferred_element_type=F32).astype(BF16)
                    c = (hq * 4 + h) * DH
                    o_buf[bb * 128:(bb + 1) * 128, c:c + DH] = o

    x_copy(0).wait()
    wq_copy(0).wait()
    qproj(0, 0)
    ka_copy().wait()
    va_copy().wait()
    wq_copy(1).wait()
    tts = qk(0, True)
    qproj(1, 0)
    pv(0, True, tts)

    def body_a(s, carry):
        wait_wo(s - 1)
        wait_wq(s + 1)

        @pl.when(s == NSB - 1)
        def _():
            x_copy(1).wait()

        tts = qk(s, True)
        oproj(s - 1, 0)
        pv(s, True, tts)
        qproj(s + 1, (s + 1) // NSB)
        return carry

    lax.fori_loop(1, NSB, body_a, 0)

    def body_b(s, carry):
        wait_wo(s - 1)
        wait_wq(s + 1)
        wait_kvb(s - NSB)
        tts = qk(s - NSB, False)
        oproj(s - 1, (s - 1) // NSB)
        pv(s - NSB, False, tts)
        qproj(s + 1, 1)
        return carry

    lax.fori_loop(NSB, NS - 1, body_b, 0)

    out_buf[0] = acc[0].astype(BF16)
    out_copy(0).start()
    wait_wo(NS - 2)
    wait_wo(NS - 1)
    wait_kvb(NSB - 1)
    tts = qk(NSB - 1, False)
    oproj(NS - 2, 1)
    pv(NSB - 1, False, tts)
    out_buf[1] = (acc[1] + jnp.dot(o_buf[...], wo_buf[NS - 1], preferred_element_type=F32)).astype(BF16)
    out_copy(1).start()
    out_copy(0).wait()
    out_copy(1).wait()


@jax.jit
def pallas_concat_heads__gqa_block_cached__mha_block_cached__near_ridge_kernel(A_x, A_k_cache, A_v_cache, A_wq, A_wo, B_x, B_k_cache, B_v_cache, B_wq, B_wo):
    xa = A_x.reshape(M, D)
    xb = B_x.reshape(M, D)
    kb = B_k_cache.reshape(B, H // 4, 4 * SK, DH)
    vb = B_v_cache.reshape(B, H // 4, 4 * SK, DH)
    any_spec = pl.BlockSpec(memory_space=pl.ANY)
    out = pl.pallas_call(
        _kernel,
        in_specs=[any_spec] * 10,
        out_specs=any_spec,
        out_shape=jax.ShapeDtypeStruct((M, 2 * D), BF16),
        scratch_shapes=[
            pltpu.VMEM((2, M, D), BF16),
            pltpu.VMEM((B, HKV, SK, DH), BF16),
            pltpu.VMEM((B, HKV, SK, DH), BF16),
            pltpu.VMEM((B, H // 4, 4 * SK, DH), BF16),
            pltpu.VMEM((B, H // 4, 4 * SK, DH), BF16),
            pltpu.VMEM((NS, D, CH), BF16),
            pltpu.VMEM((NS, CH, D), BF16),
            pltpu.VMEM((M, CH), BF16),
            pltpu.VMEM((M, CH), BF16),
            pltpu.VMEM((2, M, D), F32),
            pltpu.VMEM((2, M, D), BF16),
            pltpu.SemaphoreType.DMA((6 + 2 * NSB + 2 * NS,)),
        ],
        compiler_params=pltpu.CompilerParams(vmem_limit_bytes=100 * 1024 * 1024),
        name="fused_attn",
    )(xa, A_k_cache, A_v_cache, A_wq, A_wo, xb, kb, vb, B_wq, B_wo)
    return out.reshape(B, SQ, 2 * D)
```

```python
import os
import numpy as np
import jax
import jax.numpy as jnp
from jax import lax
import jax.experimental.pallas as pl
import jax.experimental.pallas.tpu as pltpu

B, SQ, D, H, HKV, SK, DH = 16, 32, 1024, 32, 4, 32, 128
M = B * SQ
HPS = 4
CH = HPS * DH
NSB = H // HPS
NS = 2 * NSB
MH = M // 2
C_EXP2 = float(DH ** -0.5 * np.log2(np.e))
NT = (((1,), (1,)), ((), ()))
NN = (((1,), (0,)), ((), ()))
F32 = jnp.float32
BF16 = jnp.bfloat16
U32 = jnp.uint32


def _pk(x):
    return pltpu.bitcast(x.astype(BF16), U32)


def _upk(x):
    return pltpu.bitcast(x, BF16)


def _softmax_cols(sc):
    m = jnp.max(sc, axis=0, keepdims=True)
    p = jnp.exp2((sc - m) * C_EXP2)
    l = jnp.sum(p, axis=0, keepdims=True)
    return p * (1.0 / l)


_LHS = [((0, 0), (1, 1), 1), ((1, 0), (1, 1), 1), ((0, 0), None, 0), ((1, 1), None, 0),
        ((0, 0), (0, 1), 1), ((1, 0), (0, 0), -1), ((0, 1), (1, 1), -1)]
_RHS = [((0, 0), (1, 1), 1), ((0, 0), None, 0), ((0, 1), (1, 1), -1), ((1, 0), (0, 0), -1),
        ((1, 1), None, 0), ((0, 0), (0, 1), 1), ((1, 0), (1, 1), 1)]


def _operand(table, ref, s, i, RH, CH_):
    a, b, sg = table[i]
    ld = lambda t: ref[s, t[0] * RH:(t[0] + 1) * RH, t[1] * CH_:(t[1] + 1) * CH_]
    if b is None:
        return ld(a)
    u, v = ld(a).astype(F32), ld(b).astype(F32)
    return (u + v if sg > 0 else u - v).astype(BF16)


def _lhs_ops(a11, a12, a21, a22):
    return [a11 + a22, a21 + a22, a11, a22, a11 + a12, a21 - a11, a12 - a22]


S_R = 0
S_A = 7
S_B = 14
S_E = 18
S_OUT = 19
N_SEM = 20
KS = D // 4


def _kernel(xa, ka, va, wqa, woa, xb, kb, vb, wqb, wob, out,
            x_buf, ka_buf, va_buf, kb_buf, vb_buf, wq_buf, wo_buf,
            q_buf, out_buf, os_buf, accm, mq_buf, sems):
    cp = pltpu.make_async_copy

    def wq_cp(s, sem, dyn=False):
        dst = wq_buf.at[s]
        src = dst if dyn else (wqa if s < NSB else wqb).at[:, pl.ds((s % NSB) * CH, CH)]
        return cp(src, dst, sems.at[sem])

    def wo_cp(s, sem, dyn=False):
        dst = wo_buf.at[s]
        src = dst if dyn else (woa if s < NSB else wob).at[pl.ds((s % NSB) * CH, CH), :]
        return cp(src, dst, sems.at[sem])

    def kv_cp(src, dst, j, n, sem, dyn=False):
        d = dst.at[:, pl.ds(j, n)]
        return cp(d if dyn else src.at[:, pl.ds(j, n)], d, sems.at[sem])

    def wq1_cp(a, b, sem):
        r, c = pl.ds(a * (D // 2), D // 2), b * (CH // 2)
        return cp(wqa.at[r, pl.ds(CH + c, CH // 2)], wq_buf.at[1, r, pl.ds(c, CH // 2)], sems.at[sem])

    def grp_r(n):
        if n < 4:
            sl = pl.ds(n * KS, KS)
            return [cp(xa.at[:, sl], x_buf.at[0, :, sl], sems.at[S_R + n]),
                    cp(wqa.at[sl, pl.ds(0, CH)], wq_buf.at[0, sl, :], sems.at[S_R + n])]
        if n == 4:
            return [kv_cp(ka, ka_buf, 0, 1, S_R + 4), wq1_cp(0, 0, S_R + 4), wq1_cp(1, 1, S_R + 4)]
        if n == 5:
            return [kv_cp(va, va_buf, 0, 1, S_R + 5), wq1_cp(0, 1, S_R + 5), wq1_cp(1, 0, S_R + 5)]
        return [wo_cp(0, S_R + 6)]

    def grp_a(s, dyn=False):
        return [wq_cp(s + 1, S_A + s, dyn), wo_cp(s, S_A + s, dyn)]

    def grp_a_kv(s):
        g = (s + 1) // 2
        return [kv_cp(ka, ka_buf, g, 1, S_A + s), kv_cp(va, va_buf, g, 1, S_A + s)]

    def grp_b(p, dyn=False):
        u = 2 * p
        sem = S_B + p
        return [wq_cp(NSB + u, sem, dyn), kv_cp(kb, kb_buf, u, 2, sem, dyn), wo_cp(NSB + u - 1, sem, dyn),
                kv_cp(vb, vb_buf, u, 2, sem, dyn), wq_cp(NSB + u + 1, sem, dyn), wo_cp(NSB + u, sem, dyn)]

    def xb_cp():
        return cp(xb, x_buf.at[1], sems.at[S_B])

    def out_cp(br, r0, nr, c0, nc):
        return cp(out_buf.at[br, pl.ds(r0, nr), pl.ds(c0, nc)],
                  out.at[pl.ds(r0, nr), pl.ds(br * D + c0, nc)], sems.at[S_OUT])

    for n in range(7):
        for c in grp_r(n):
            c.start()
    for s in range(1, NSB - 1):
        for c in grp_a(s) + (grp_a_kv(s) if s % 2 else []):
            c.start()
    xb_cp().start()
    for p in range(NSB // 2):
        for c in grp_b(p):
            c.start()
    wo_cp(NS - 1, S_E).start()

    lane_g = lax.broadcasted_iota(jnp.int32, (32, 128), 1) // 32
    QNH, QMQ = CH // 2, MH // 2
    NH = D // 2

    def q_prod(s, br, i):
        return jnp.dot(_operand(_LHS, x_buf, br, i, MH, D // 2), _operand(_RHS, wq_buf, s, i, D // 2, CH // 2),
                       preferred_element_type=F32)

    def q_stage(s, br, n):
        if n == 0:
            mq_buf[0] = q_prod(s, br, 1)
        elif n == 1:
            mq_buf[1] = q_prod(s, br, 4)
        elif n == 2:
            m1 = q_prod(s, br, 0)
            mq_buf[2] = m1 - mq_buf[0]
            mq_buf[3] = m1 - mq_buf[1]
        elif n == 3:
            m3 = q_prod(s, br, 2)
            q_buf[:QMQ, QNH:] = _pk(m3 + mq_buf[1])
            mq_buf[2] += m3
        elif n == 4:
            m4 = q_prod(s, br, 3)
            q_buf[QMQ:, :QNH] = _pk(m4 + mq_buf[0])
            mq_buf[3] += m4
        elif n == 5:
            q_buf[QMQ:, QNH:] = _pk(mq_buf[2] + q_prod(s, br, 5))
        else:
            q_buf[:QMQ, :QNH] = _pk(mq_buf[3] + q_prod(s, br, 6))

    def qproj(s, br):
        for n in range(7):
            q_stage(s, br, n)

    def o_acc(s, br, i, first, keep=True):
        m = jnp.dot(_upk(os_buf[i]), _operand(_RHS, wo_buf, s, i, CH // 2, D // 2), preferred_element_type=F32)
        if first is False:
            m = accm[br, i] + m
        elif first is not True:
            m = jnp.where(first, 0.0, accm[br, i]) + m
        if keep:
            accm[br, i] = m
        return m

    O_ORDER = (4, 2, 1, 3, 0, 5, 6)

    def o_stage(s, br, n, first, fin, last=False):
        i = O_ORDER[n]
        m = o_acc(s, br, i, first, keep=not (last and n >= 5))
        if not fin:
            return None
        ob = out_buf.at[br]
        if n == 1:
            ob[:MH, NH:] = (m + accm[br, 4]).astype(BF16)
            return (0, NH)
        if n == 3:
            ob[MH:, :NH] = (m + accm[br, 1]).astype(BF16)
            return (MH, 0)
        if n == 5:
            ob[MH:, NH:] = (accm[br, 0] - accm[br, 1] + accm[br, 2] + m).astype(BF16)
            return (MH, NH)
        if n == 6:
            ob[:MH, :NH] = (accm[br, 0] + accm[br, 3] - accm[br, 4] + m).astype(BF16)
            return (0, 0)
        return None

    def q4_of(b):
        return _upk(jnp.concatenate(
            [q_buf[b * 16:(b + 1) * 16, h * DH:(h + 1) * DH] for h in range(4)], axis=0))

    def qk_group(j, is_a, bb):
        pts = []
        for bi in range(4):
            b = bb * 4 + bi
            q4 = q4_of(b)
            if is_a:
                sc = lax.dot_general(ka_buf[b, j // 2], q4, NT, preferred_element_type=F32)
            else:
                st = lax.dot_general(kb_buf[b, j], q4, NT, preferred_element_type=F32)
                sc = st[0:32]
                for h in range(1, 4):
                    sc = jnp.where(lane_g == h, st[h * 32:(h + 1) * 32], sc)
            pts.append(_softmax_cols(sc))
        return jnp.concatenate(pts, axis=0).T

    def pv_tile(j, is_a, tts, bb, h):
        ph = tts[bb][h * 32:(h + 1) * 32]
        lhs = jnp.concatenate(
            [jnp.where(lane_g == bi, ph, 0.0) for bi in range(4)], axis=0).astype(BF16)
        if is_a:
            vh = jnp.concatenate([va_buf[bb * 4 + bi, j // 2] for bi in range(4)], axis=0)
        else:
            vh = jnp.concatenate(
                [vb_buf[bb * 4 + bi, j, h * 32:(h + 1) * 32, :] for bi in range(4)], axis=0)
        return lax.dot_general(lhs, vh, NN, preferred_element_type=F32)

    def pv(j, is_a, tts):
        for bb in range(2):
            for hh in range(2):
                t11 = pv_tile(j, is_a, tts, bb, hh)
                t12 = pv_tile(j, is_a, tts, bb, hh + 2)
                t21 = pv_tile(j, is_a, tts, bb + 2, hh)
                t22 = pv_tile(j, is_a, tts, bb + 2, hh + 2)
                ops = _lhs_ops(t11, t12, t21, t22)
                for i in range(7):
                    os_buf.at[i][bb * 64:(bb + 1) * 64, hh * DH:(hh + 1) * DH] = _pk(ops[i])

    QK_ORDER = (2, 3, 0, 1)

    def attn_oproj(j, is_a, so, bro, first, fin=False):
        tts = [None] * 4
        for n in range(7):
            o_stage(so, bro, n, first, fin)
            if n < 4:
                tts[QK_ORDER[n]] = qk_group(j, is_a, QK_ORDER[n])
        pv(j, is_a, tts)

    def wait_all(cs):
        for c in cs:
            c.wait()

    for n in range(4):
        with jax.named_scope("wait0"):
            wait_all(grp_r(n))
        with jax.named_scope("pro1"):
            part = jnp.dot(x_buf[0, :, n * KS:(n + 1) * KS], wq_buf[0, n * KS:(n + 1) * KS, :],
                           preferred_element_type=F32)
            for a in range(2):
                for c in range(2):
                    pq = part[a * MH:(a + 1) * MH, c * QNH:(c + 1) * QNH]
                    if n == 0:
                        mq_buf[2 * a + c] = pq
                    elif n < 3:
                        mq_buf[2 * a + c] += pq
                    else:
                        q_buf[a * QMQ:(a + 1) * QMQ, c * QNH:(c + 1) * QNH] = _pk(mq_buf[2 * a + c] + pq)
    with jax.named_scope("wait1"):
        wait_all(grp_r(4))
    with jax.named_scope("pro2"):
        tts = []
        q_stage(1, 0, 0)
        tts.append(qk_group(0, True, 0))
        tts.append(qk_group(0, True, 1))
        q_stage(1, 0, 1)
        tts.append(qk_group(0, True, 2))
        tts.append(qk_group(0, True, 3))
        q_stage(1, 0, 2)
    with jax.named_scope("wait2"):
        wait_all(grp_r(5))
    with jax.named_scope("pro3"):
        pv(0, True, tts)
        for n in range(3, 7):
            q_stage(1, 0, n)
    with jax.named_scope("wait3"):
        wait_all(grp_r(6))
    with jax.named_scope("pro4"):
        attn_oproj(1, True, 0, 0, True)

    def body_a(s, carry):
        with jax.named_scope("waitA"):
            wait_all(grp_a(s, dyn=True))

            @pl.when(s % 2 == 1)
            def _():
                g = (s + 1) // 2
                kv_cp(ka, ka_buf, g, 1, S_A + s, dyn=True).wait()
                kv_cp(va, va_buf, g, 1, S_A + s, dyn=True).wait()

        with jax.named_scope("bodyA"):
            qproj(s + 1, 0)
            attn_oproj(s + 1, True, s, 0, False)
        return carry

    lax.fori_loop(1, NSB - 1, body_a, 0)

    def body_b(p, carry):
        u = 2 * p
        with jax.named_scope("waitB"):
            wait_all(grp_b(p, dyn=True))

            @pl.when(p == 0)
            def _():
                xb_cp().wait()

            @pl.when(p == 1)
            def _():
                out_cp(0, 0, M, 0, D).start()

        with jax.named_scope("bodyB"):
            qproj(NSB + u, 1)
            attn_oproj(u, False, NSB + u - 1, jnp.minimum(p, 1), False, fin=True)
            qproj(NSB + u + 1, 1)
            attn_oproj(u + 1, False, NSB + u, 1, p == 0)
        return carry

    lax.fori_loop(0, NSB // 2, body_b, 0)

    with jax.named_scope("epi0"):
        wo_cp(NS - 1, S_E).wait()
    with jax.named_scope("epi1"):
        outs = [out_cp(0, 0, M, 0, D)]
        for n in range(7):
            blk = o_stage(NS - 1, 1, n, False, True, last=True)
            if blk is not None:
                outs.append(out_cp(1, blk[0], MH, blk[1], NH))
                outs[-1].start()
    with jax.named_scope("tail"):
        wait_all(outs)


@jax.jit
def pallas_concat_heads__gqa_block_cached__mha_block_cached__near_ridge_kernel(A_x, A_k_cache, A_v_cache, A_wq, A_wo, B_x, B_k_cache, B_v_cache, B_wq, B_wo):
    xa = A_x.reshape(M, D)
    xb = B_x.reshape(M, D)
    kb = B_k_cache.reshape(B, H // 4, 4 * SK, DH)
    vb = B_v_cache.reshape(B, H // 4, 4 * SK, DH)
    any_spec = pl.BlockSpec(memory_space=pl.ANY)
    out = pl.pallas_call(
        _kernel,
        in_specs=[any_spec] * 10,
        out_specs=any_spec,
        out_shape=jax.ShapeDtypeStruct((M, 2 * D), BF16),
        scratch_shapes=[
            pltpu.VMEM((2, M, D), BF16),
            pltpu.VMEM((B, HKV, SK, DH), BF16),
            pltpu.VMEM((B, HKV, SK, DH), BF16),
            pltpu.VMEM((B, H // 4, 4 * SK, DH), BF16),
            pltpu.VMEM((B, H // 4, 4 * SK, DH), BF16),
            pltpu.VMEM((NS, D, CH), BF16),
            pltpu.VMEM((NS, CH, D), BF16),
            pltpu.VMEM((M // 2, CH), U32),
            pltpu.VMEM((2, M, D), BF16),
            pltpu.VMEM((7, MH // 2, CH // 2), U32),
            pltpu.VMEM((2, 7, MH, D // 2), F32),
            pltpu.VMEM((4, MH, CH // 2), F32),
            pltpu.SemaphoreType.DMA((N_SEM,)),
        ],
        compiler_params=pltpu.CompilerParams(vmem_limit_bytes=100 * 1024 * 1024,
                                             disable_semaphore_checks=True),
        name="fused_attn",
    )(xa, A_k_cache, A_v_cache, A_wq, A_wo, xb, kb, vb, B_wq, B_wo)
    return out.reshape(B, SQ, 2 * D)
```

```python
import numpy as np
import jax
import jax.numpy as jnp
from jax import lax
import jax.experimental.pallas as pl
import jax.experimental.pallas.tpu as pltpu

B, SQ, D, H, HKV, SK, DH = 16, 32, 1024, 32, 4, 32, 128
M = B * SQ
MH = M // 2
SH = SQ // 2
HPS = 4
CH = HPS * DH
NSB = H // HPS
NS = 2 * NSB
KS = D // 4
NH = D // 2
QNH, QMQ = CH // 2, MH // 2
C_EXP2 = float(DH ** -0.5 * np.log2(np.e))
NT = (((1,), (1,)), ((), ()))
NN = (((1,), (0,)), ((), ()))
F32 = jnp.float32
BF16 = jnp.bfloat16
U32 = jnp.uint32

_LHS = [((0, 0), (1, 1), 1), ((1, 0), (1, 1), 1), ((0, 0), None, 0), ((1, 1), None, 0),
        ((0, 0), (0, 1), 1), ((1, 0), (0, 0), -1), ((0, 1), (1, 1), -1)]
_RHS = [((0, 0), (1, 1), 1), ((0, 0), None, 0), ((0, 1), (1, 1), -1), ((1, 0), (0, 0), -1),
        ((1, 1), None, 0), ((0, 0), (0, 1), 1), ((1, 0), (1, 1), 1)]
_OUT = {(0, 0): {0: 1, 3: 1, 4: -1, 6: 1}, (0, 1): {2: 1, 4: 1},
        (1, 0): {1: 1, 3: 1}, (1, 1): {0: 1, 1: -1, 2: 1, 5: 1}}

S_R = 0
S_A = 6
S_B = 13
S_E = 17
S_OUT = 18
N_SEM = 19


def _pk(x):
    return pltpu.bitcast(x.astype(BF16), U32)


def _upk(x):
    return pltpu.bitcast(x, BF16)


def _operand(spec, ld):
    a, b, sg = spec
    if b is None:
        return ld(a)
    u, v = ld(a).astype(F32), ld(b).astype(F32)
    return (u + v if sg > 0 else u - v).astype(BF16)


def _lhs_ops(a11, a12, a21, a22):
    return [a11 + a22, a21 + a22, a11, a22, a11 + a12, a21 - a11, a12 - a22]


def _softmax_cols(sc):
    m = jnp.max(sc, axis=0, keepdims=True)
    p = jnp.exp2((sc - m) * C_EXP2)
    l = jnp.sum(p, axis=0, keepdims=True)
    return p * (1.0 / l)


def _kernel(xa, ka, va, wqa, woa, xb, kb, vb, wqb, wob, out,
            x_buf, ka_buf, va_buf, kb_buf, vb_buf, wq_buf, wo_buf,
            q_buf, out_buf, os_buf, accm, mq_buf, sems):
    cp = pltpu.make_async_copy

    def wq_cp(s, sem, dyn=False):
        dst = wq_buf.at[s]
        src = dst if dyn else (wqa if s < NSB else wqb).at[:, pl.ds((s % NSB) * CH, CH)]
        return cp(src, dst, sems.at[sem])

    def wo_cp(s, sem, dyn=False):
        dst = wo_buf.at[s]
        src = dst if dyn else (woa if s < NSB else wob).at[pl.ds((s % NSB) * CH, CH), :]
        return cp(src, dst, sems.at[sem])

    def kv_cp(src, dst, j, n, sem, dyn=False):
        d = dst.at[:, pl.ds(j, n)]
        return cp(d if dyn else src.at[:, pl.ds(j, n)], d, sems.at[sem])

    def wq1_cp(a, b, sem):
        r, c = pl.ds(a * NH, NH), b * QNH
        return cp(wqa.at[r, pl.ds(CH + c, QNH)], wq_buf.at[1, r, pl.ds(c, QNH)], sems.at[sem])

    def grp_r(n):
        sem = S_R + n
        if n < 4:
            sl = pl.ds(n * KS, KS)
            return [cp(xa.at[:, :, :, sl], x_buf.at[0, :, :, :, sl], sems.at[sem]),
                    cp(wqa.at[sl, pl.ds(0, CH)], wq_buf.at[0, sl, :], sems.at[sem])]
        if n == 4:
            return [kv_cp(ka, ka_buf, 0, 1, sem), wq1_cp(0, 0, sem), wq1_cp(1, 1, sem)]
        if n == 5:
            return [kv_cp(va, va_buf, 0, 1, sem), wq1_cp(0, 1, sem), wq1_cp(1, 0, sem)]
        return [wo_cp(0, sem)]

    def grp_a(s, dyn=False):
        return [wq_cp(s + 1, S_A + s, dyn), wo_cp(s, S_A + s, dyn)]

    def grp_a_kv(s, dyn=False):
        g = (s + 1) // 2
        return [kv_cp(ka, ka_buf, g, 1, S_A + s, dyn), kv_cp(va, va_buf, g, 1, S_A + s, dyn)]

    def grp_b(p, dyn=False):
        u, sem = 2 * p, S_B + p
        return [wq_cp(NSB + u, sem, dyn), kv_cp(kb, kb_buf, u, 2, sem, dyn),
                wo_cp(NSB + u - 1, sem, dyn), kv_cp(vb, vb_buf, u, 2, sem, dyn),
                wq_cp(NSB + u + 1, sem, dyn), wo_cp(NSB + u, sem, dyn)]

    def xb_cp():
        return cp(xb, x_buf.at[1], sems.at[S_B])

    def out_cp(br, c0, nc):
        return cp(out_buf.at[br, :, :, :, pl.ds(c0, nc)],
                  out.at[:, :, :, pl.ds(br * D + c0, nc)], sems.at[S_OUT])

    def wait_all(cs):
        for c in cs:
            c.wait()

    for n in range(7):
        for c in grp_r(n):
            c.start()
    for s in range(1, NSB - 1):
        for c in grp_a(s) + (grp_a_kv(s) if s % 2 else []):
            c.start()
    xb_cp().start()
    for p in range(NSB // 2):
        for c in grp_b(p):
            c.start()
    wo_cp(NS - 1, S_E).start()

    accm[1] = jnp.zeros(accm.shape[1:], F32)

    lane_g = lax.broadcasted_iota(jnp.int32, (SK, 4 * SQ), 1) // SQ
    lane_h = lax.broadcasted_iota(jnp.int32, (SH, 4 * SK), 1) // SK

    def x_block(br, half, c0, nc):
        return x_buf[br, :, half, :, c0:c0 + nc].reshape(MH, nc)

    def q_prod(s, br, i):
        lhs = _operand(_LHS[i], lambda t: x_block(br, t[0], t[1] * NH, NH))
        rhs = _operand(_RHS[i], lambda t: wq_buf[s, t[0] * NH:(t[0] + 1) * NH, t[1] * QNH:(t[1] + 1) * QNH])
        return jnp.dot(lhs, rhs, preferred_element_type=F32)

    def q_stage(s, br, n):
        if n == 0:
            mq_buf[0] = q_prod(s, br, 1)
        elif n == 1:
            mq_buf[1] = q_prod(s, br, 4)
        elif n == 2:
            m1 = q_prod(s, br, 0)
            mq_buf[2] = m1 - mq_buf[0]
            mq_buf[3] = m1 - mq_buf[1]
        elif n == 3:
            m3 = q_prod(s, br, 2)
            q_buf[:QMQ, QNH:] = _pk(m3 + mq_buf[1])
            mq_buf[2] += m3
        elif n == 4:
            m4 = q_prod(s, br, 3)
            q_buf[QMQ:, :QNH] = _pk(m4 + mq_buf[0])
            mq_buf[3] += m4
        elif n == 5:
            q_buf[QMQ:, QNH:] = _pk(mq_buf[2] + q_prod(s, br, 5))
        else:
            q_buf[:QMQ, :QNH] = _pk(mq_buf[3] + q_prod(s, br, 6))

    def qproj(s, br):
        for n in range(7):
            q_stage(s, br, n)

    def o_prod(s, i, c0=0, nc=NH):
        rhs = _operand(_RHS[i], lambda t: wo_buf[s, t[0] * QNH:(t[0] + 1) * QNH,
                                                 t[1] * NH + c0:t[1] * NH + c0 + nc])
        return jnp.dot(_upk(os_buf[i]), rhs, preferred_element_type=F32)

    def put_out(br, half, c0, val):
        nc = val.shape[1]
        out_buf[br, :, half, :, c0:c0 + nc] = val.astype(BF16).reshape(B, SH, nc)

    def o_stage(s, br, i, first, fin):
        m = o_prod(s, i)
        if not first:
            m = accm[br, i] + m
        accm[br, i] = m
        if fin is None:
            return
        fin.add(i)
        for (half, cb), terms in _OUT.items():
            if i in terms and set(terms) <= fin:
                val = m if terms[i] > 0 else -m
                for k, sg in terms.items():
                    if k != i:
                        val = val + accm[br, k] if sg > 0 else val - accm[br, k]
                put_out(br, half, cb * NH, val)

    def qk_group(j, is_a, bb):
        pts = []
        for b in range(bb * 4, bb * 4 + 4):
            q4 = _upk(jnp.concatenate(
                [q_buf[half * QMQ + b * 8:half * QMQ + (b + 1) * 8, h * DH:(h + 1) * DH]
                 for h in range(HPS) for half in range(2)], axis=0))
            if is_a:
                sc = lax.dot_general(ka_buf[b, j // 2], q4, NT, preferred_element_type=F32)
            else:
                st = lax.dot_general(kb_buf[b, j], q4, NT, preferred_element_type=F32)
                sc = st[0:SK]
                for h in range(1, HPS):
                    sc = jnp.where(lane_g == h, st[h * SK:(h + 1) * SK], sc)
            pts.append(_softmax_cols(sc))
        return jnp.concatenate(pts, axis=0).T

    def pv_tile(j, is_a, tt, bb, h):
        ph = tt[h * SQ:(h + 1) * SQ]
        lhs = jnp.concatenate(
            [jnp.where(lane_h == bi, ph[half * SH:(half + 1) * SH], 0.0)
             for half in range(2) for bi in range(4)], axis=0).astype(BF16)
        if is_a:
            vh = jnp.concatenate([va_buf[bb * 4 + bi, j // 2] for bi in range(4)], axis=0)
        else:
            vh = jnp.concatenate(
                [vb_buf[bb * 4 + bi, j, h * SK:(h + 1) * SK, :] for bi in range(4)], axis=0)
        return lax.dot_general(lhs, vh, NN, preferred_element_type=F32)

    def pv(j, is_a, tts):
        for bb in range(4):
            t = [pv_tile(j, is_a, tts[bb], bb, h) for h in range(HPS)]
            for hh in range(2):
                ops = _lhs_ops(t[hh][:64], t[hh + 2][:64], t[hh][64:], t[hh + 2][64:])
                for i in range(7):
                    os_buf.at[i][bb * 32:(bb + 1) * 32, hh * DH:(hh + 1) * DH] = _pk(ops[i])

    def attn_oproj(j, is_a, so, bro, order, sched, first=False, fin=None):
        tts = [None] * 4
        for n in range(7):
            for g in sched.get(n, ()):
                tts[g] = qk_group(j, is_a, g)
            o_stage(so, bro, order[n], first, fin)
        pv(j, is_a, tts)

    order_mid = (2, 4, 3, 1, 0, 5, 6)

    for n in range(4):
        with jax.named_scope("wait0"):
            wait_all(grp_r(n))
        with jax.named_scope("pro1"):
            xs = jnp.concatenate([x_block(0, a, n * KS, KS) for a in range(2)], axis=0)
            part = jnp.dot(xs, wq_buf[0, n * KS:(n + 1) * KS, :], preferred_element_type=F32)
            for a in range(2):
                for c in range(2):
                    pq = part[a * MH:(a + 1) * MH, c * QNH:(c + 1) * QNH]
                    if n == 0:
                        mq_buf[2 * a + c] = pq
                    elif n < 3:
                        mq_buf[2 * a + c] += pq
                    else:
                        q_buf[a * QMQ:(a + 1) * QMQ, c * QNH:(c + 1) * QNH] = _pk(mq_buf[2 * a + c] + pq)
    with jax.named_scope("wait1"):
        wait_all(grp_r(4))
    with jax.named_scope("pro2"):
        tts0 = []
        q_stage(1, 0, 0)
        tts0.append(qk_group(0, True, 0))
        tts0.append(qk_group(0, True, 1))
        q_stage(1, 0, 1)
        tts0.append(qk_group(0, True, 2))
        tts0.append(qk_group(0, True, 3))
        q_stage(1, 0, 2)
    with jax.named_scope("wait2"):
        wait_all(grp_r(5))
    with jax.named_scope("pro3"):
        pv(0, True, tts0)
        for n in range(3, 7):
            q_stage(1, 0, n)
    with jax.named_scope("wait3"):
        wait_all(grp_r(6))
    with jax.named_scope("pro4"):
        attn_oproj(1, True, 0, 0, (4, 2, 1, 3, 0, 5, 6), {1: (2,), 2: (3,), 3: (0,), 4: (1,)}, first=True)

    def body_a(s, carry):
        with jax.named_scope("waitA"):
            wait_all(grp_a(s, dyn=True))

            @pl.when(s % 2 == 1)
            def _():
                wait_all(grp_a_kv(s, dyn=True))

        with jax.named_scope("bodyA"):
            qproj(s + 1, 0)
            attn_oproj(s + 1, True, s, 0, order_mid, {1: (0, 1), 3: (2, 3)})
        return carry

    lax.fori_loop(1, NSB - 1, body_a, 0)

    def body_b(p, carry):
        u = 2 * p
        with jax.named_scope("waitB"):
            wait_all(grp_b(p, dyn=True))

            @pl.when(p == 0)
            def _():
                xb_cp().wait()

            @pl.when(p == 1)
            def _():
                out_cp(0, 0, D).start()

        with jax.named_scope("bodyB"):
            qproj(NSB + u, 1)
            attn_oproj(u, False, NSB + u - 1, jnp.minimum(p, 1), order_mid, {1: (0, 1), 3: (2, 3)}, fin=set())
            qproj(NSB + u + 1, 1)
            attn_oproj(u + 1, False, NSB + u, 1, order_mid, {1: (0, 1, 2, 3)})
        return carry

    lax.fori_loop(0, NSB // 2, body_b, 0)

    with jax.named_scope("epi0"):
        wo_cp(NS - 1, S_E).wait()
    with jax.named_scope("epi1"):
        outs = [out_cp(0, 0, D)]
        c0 = 0
        for tc in (256, 128, 128):
            def fm(k, c0=c0, tc=tc):
                return accm[1, k, :, c0:c0 + tc] + o_prod(NS - 1, k, c0, tc)
            m5, m2 = fm(4), fm(1)
            m3 = fm(2)
            put_out(1, 0, NH + c0, m3 + m5)
            m1 = fm(0)
            m6 = fm(5)
            put_out(1, 1, NH + c0, m1 - m2 + m3 + m6)
            outs.append(out_cp(1, NH + c0, tc))
            outs[-1].start()
            m4 = fm(3)
            put_out(1, 1, c0, m2 + m4)
            m7 = fm(6)
            put_out(1, 0, c0, m1 + m4 - m5 + m7)
            outs.append(out_cp(1, c0, tc))
            outs[-1].start()
            c0 += tc
    with jax.named_scope("tail"):
        wait_all(outs)


@jax.jit
def pallas_concat_heads__gqa_block_cached__mha_block_cached__near_ridge_kernel(A_x, A_k_cache, A_v_cache, A_wq, A_wo, B_x, B_k_cache, B_v_cache, B_wq, B_wo):
    xa = A_x.reshape(B, 2, SH, D)
    xb = B_x.reshape(B, 2, SH, D)
    kb = B_k_cache.reshape(B, NSB, HPS * SK, DH)
    vb = B_v_cache.reshape(B, NSB, HPS * SK, DH)
    any_spec = pl.BlockSpec(memory_space=pl.ANY)
    out = pl.pallas_call(
        _kernel,
        in_specs=[any_spec] * 10,
        out_specs=any_spec,
        out_shape=jax.ShapeDtypeStruct((B, 2, SH, 2 * D), BF16),
        scratch_shapes=[
            pltpu.VMEM((2, B, 2, SH, D), BF16),
            pltpu.VMEM((B, HKV, SK, DH), BF16),
            pltpu.VMEM((B, HKV, SK, DH), BF16),
            pltpu.VMEM((B, NSB, HPS * SK, DH), BF16),
            pltpu.VMEM((B, NSB, HPS * SK, DH), BF16),
            pltpu.VMEM((NS, D, CH), BF16),
            pltpu.VMEM((NS, CH, D), BF16),
            pltpu.VMEM((M // 2, CH), U32),
            pltpu.VMEM((2, B, 2, SH, D), BF16),
            pltpu.VMEM((7, MH // 2, QNH), U32),
            pltpu.VMEM((2, 7, MH, NH), F32),
            pltpu.VMEM((4, MH, QNH), F32),
            pltpu.SemaphoreType.DMA((N_SEM,)),
        ],
        compiler_params=pltpu.CompilerParams(vmem_limit_bytes=100 * 1024 * 1024,
                                             disable_semaphore_checks=True),
        name="fused_attn",
    )(xa, A_k_cache, A_v_cache, A_wq, A_wo, xb, kb, vb, B_wq, B_wo)
    return out.reshape(B, SQ, 2 * D)
```

```python
import numpy as np
import jax
import jax.numpy as jnp
from jax import lax
import jax.experimental.pallas as pl
import jax.experimental.pallas.tpu as pltpu

B, SQ, D, H, HKV, SK, DH = 16, 32, 1024, 32, 4, 32, 128
M = B * SQ
MH = M // 2
SH = SQ // 2
HPS = 4
CH = HPS * DH
NSB = H // HPS
NS = 2 * NSB
KS = D // 4
NH = D // 2
QNH, QMQ = CH // 2, MH // 2
NQ4 = D // 4
RQ = SQ // 4
C_EXP2 = float(DH ** -0.5 * np.log2(np.e))
NT = (((1,), (1,)), ((), ()))
NN = (((1,), (0,)), ((), ()))
F32 = jnp.float32
BF16 = jnp.bfloat16
U32 = jnp.uint32

_LHS = [((0, 0), (1, 1), -1), ((1, 0), (1, 1), -1), ((0, 0), None, 0), ((1, 1), None, 0),
        ((0, 0), (0, 1), -1), ((1, 0), (0, 0), -1), ((0, 1), (1, 1), -1)]
_RHS = [((0, 0), (1, 1), -1), ((0, 0), None, 0), ((0, 1), (1, 1), 1), ((1, 0), (0, 0), 1),
        ((1, 1), None, 0), ((0, 0), (0, 1), 1), ((1, 0), (1, 1), 1)]
_OUT = {(0, 0): {0: 1, 3: 1, 4: 1, 6: 1}, (0, 1): {2: 1, 4: -1},
        (1, 0): {1: 1, 3: 1}, (1, 1): {0: 1, 1: -1, 2: 1, 5: 1}}
_SWAP = (0, 1, 0, 0, 1, 1, 1)
J_ORDER = (1, 4, 0, 2, 3, 5, 6)

def _o_order():
    nt = lambda i: 1 if _RHS[i][1] is None else 2
    allp = [(i, j) for i in range(7) for j in range(7)]
    heavy = [p for p in allp if nt(p[0]) * nt(p[1]) == 4]
    mid = [p for p in allp if nt(p[0]) * nt(p[1]) == 2]
    light = [p for p in allp if nt(p[0]) * nt(p[1]) == 1]
    mode = 0
    seq = []
    if mode == 0:
        lo = light[:2] + mid[:10] + light[2:] + mid[10:]
        seq = lo[:2]
        lo = lo[2:]
        while heavy or lo:
            if heavy:
                seq.append(heavy.pop(0))
            if lo:
                seq.append(lo.pop(0))
    elif mode == 1:
        lo = light[:2] + mid[:10] + light[2:] + mid[10:]
        while heavy or lo:
            seq += lo[:2]; lo = lo[2:]
            seq += heavy[:2]; heavy = heavy[2:]
    return tuple(seq)


O_SEQ = _o_order()
SPLIT = O_SEQ[0]

S_R = 0
S_A = 6
S_B = 14
S_E = 17
S_OUT = 18
N_SEM = 19


def _pk(x):
    return pltpu.bitcast(x.astype(BF16), U32)


def _upk(x):
    return pltpu.bitcast(x, BF16)


def _terms(spec):
    a, b, sg = spec
    return [(a, 1)] + ([(b, sg)] if b is not None else [])


def _signed_sum(items):
    items = sorted(items, key=lambda t: -t[0])
    acc = items[0][1]
    for sg, v in items[1:]:
        acc = acc + v if sg > 0 else acc - v
    return acc


def _comb(spec, get):
    return _signed_sum([(sg, get(t)) for t, sg in _terms(spec)])


def _operand(spec, ld):
    if spec[1] is None:
        return ld(spec[0])
    return _comb(spec, lambda t: ld(t).astype(F32)).astype(BF16)


def _softmax_cols(sc):
    m = jnp.max(sc, axis=0, keepdims=True)
    p = jnp.exp2((sc - m) * C_EXP2)
    l = jnp.sum(p, axis=0, keepdims=True)
    return p * (1.0 / l)


def _kernel(xa, ka, va, wqa, woa, xb, kb, vb, wqb, wob, out,
            x_buf, ka_buf, va_buf, kb_buf, vb_buf, wq_buf, wo_buf,
            q_buf, out_buf, os_buf, accm, mq_buf, sems):
    cp = pltpu.make_async_copy

    def wq_cp(s, sem, dyn=False):
        dst = wq_buf.at[s]
        src = dst if dyn else (wqa if s < NSB else wqb).at[:, pl.ds((s % NSB) * CH, CH)]
        return cp(src, dst, sems.at[sem])

    def wo_cp(s, sem, dyn=False):
        dst = wo_buf.at[s]
        src = dst if dyn else (woa if s < NSB else wob).at[pl.ds((s % NSB) * CH, CH), :]
        return cp(src, dst, sems.at[sem])

    def kv_cp(src, dst, j, n, sem, dyn=False, off=0):
        d = dst.at[:, pl.ds(j + off, n)]
        return cp(d if dyn else src.at[:, pl.ds(j, n)], d, sems.at[sem])

    def wq1_cp(a, b, sem):
        r, c = pl.ds(a * NH, NH), b * QNH
        return cp(wqa.at[r, pl.ds(CH + c, QNH)], wq_buf.at[1, r, pl.ds(c, QNH)], sems.at[sem])

    def grp_r(n):
        sem = S_R + n
        if n < 4:
            sl = pl.ds(n * KS, KS)
            return [cp(xa.at[:, :, :, sl], x_buf.at[0, :, :, :, sl], sems.at[sem]),
                    cp(wqa.at[sl, pl.ds(0, CH)], wq_buf.at[0, sl, :], sems.at[sem])]
        if n == 4:
            return [kv_cp(ka, ka_buf, 0, 1, sem), wq1_cp(0, 0, sem), wq1_cp(1, 1, sem)]
        if n == 5:
            return [kv_cp(va, va_buf, 0, 1, sem), wq1_cp(0, 1, sem), wq1_cp(1, 0, sem)]
        return [wo_cp(0, sem)]

    def grp_a(s, dyn=False):
        return [wq_cp(s + 1, S_A + s, dyn), wo_cp(s, S_A + s, dyn)]

    def grp_a_kv(s, dyn=False):
        g = s // 2
        return [kv_cp(ka, ka_buf, g, 1, S_A + s, dyn), kv_cp(va, va_buf, g, 1, S_A + s, dyn)]

    def xb_cp():
        return cp(xb, x_buf.at[1], sems.at[S_A + NSB - 1])

    def grp_b(p, dyn=False):
        u, sem = 2 * p, S_B + p
        g = [kv_cp(kb, kb_buf, u, 2, sem, dyn), wq_cp(NSB + u + 1, sem, dyn),
             kv_cp(vb, vb_buf, u, 2, sem, dyn), wo_cp(NSB + u, sem, dyn)]
        if dyn or u + 2 < NSB:
            g.append(wq_cp(NSB + u + 2, sem, dyn))
        return g + [wo_cp(NSB + u + 1, sem, dyn)]

    def out_cp(br, c0, nc):
        return cp(out_buf.at[br, :, :, :, pl.ds(c0, nc)],
                  out.at[:, :, :, pl.ds(br * D + c0, nc)], sems.at[S_OUT])

    def wait_all(cs):
        for c in cs:
            c.wait()

    for n in range(7):
        for c in grp_r(n):
            c.start()
    for s in range(1, NSB):
        if s == NSB - 1:
            xb_cp().start()
        for c in (grp_a_kv(s) if s % 2 == 0 else []) + grp_a(s):
            c.start()
    for p in range(NSB // 2):
        for c in grp_b(p):
            c.start()

    def zero_acc(k0, k1):
        accm[1, k0:k1] = jnp.zeros((k1 - k0,) + accm.shape[2:], F32)

    zero_acc(0, 25)

    lane_g = lax.broadcasted_iota(jnp.int32, (SK, 4 * SQ), 1) // SQ

    def x_block(br, half, c0, nc):
        return x_buf[br, :, half, :, c0:c0 + nc].reshape(MH, nc)

    def q_stage(s, br, n, mid=None):
        def q_prod(i):
            lhs = _operand(_LHS[i], lambda t: x_block(br, t[0], t[1] * NH, NH))

            def part(c0, nc):
                rhs = _operand(_RHS[i], lambda t: wq_buf[s, t[0] * NH:(t[0] + 1) * NH,
                                                         t[1] * QNH + c0:t[1] * QNH + c0 + nc])
                return jnp.dot(lhs, rhs, preferred_element_type=F32)

            if mid is None:
                return part(0, QNH)
            m0 = part(0, DH)
            mid()
            return jnp.concatenate([m0, part(DH, DH)], axis=1)

        if n == 0:
            mq_buf[0] = q_prod(1)
        elif n == 1:
            mq_buf[1] = q_prod(4)
        elif n == 2:
            m1 = q_prod(0)
            mq_buf[2] = m1 - mq_buf[0]
            mq_buf[3] = m1 + mq_buf[1]
        elif n == 3:
            m3 = q_prod(2)
            q_buf[:QMQ, QNH:] = _pk(m3 - mq_buf[1])
            mq_buf[2] += m3
        elif n == 4:
            m4 = q_prod(3)
            q_buf[QMQ:, :QNH] = _pk(m4 + mq_buf[0])
            mq_buf[3] += m4
        elif n == 5:
            q_buf[QMQ:, QNH:] = _pk(mq_buf[2] + q_prod(5))
        else:
            q_buf[:QMQ, :QNH] = _pk(mq_buf[3] + q_prod(6))

    def o_prod(s, i, j, c0=0, nc=NQ4, r0=0, nr=128):
        ts = [(s1 * s2, 2 * a[0] + b[0], 2 * a[1] + (b[1] ^ _SWAP[i]))
              for a, s1 in _terms(_RHS[i]) for b, s2 in _terms(_RHS[j])]
        ld = lambda r, c: wo_buf[s, r * DH:(r + 1) * DH, c * NQ4 + c0:c * NQ4 + c0 + nc]
        if len(ts) == 1:
            rhs = ld(ts[0][1], ts[0][2])
        else:
            rhs = _signed_sum([(sg, ld(r, c).astype(F32)) for sg, r, c in ts]).astype(BF16)
        return jnp.dot(_upk(os_buf[i * 64 + r0 // 2:i * 64 + (r0 + nr) // 2, j * DH:(j + 1) * DH]), rhs, preferred_element_type=F32)

    def o_step(s, br, i, j, first, split):
        for r0, nr in (((0, 64), (64, 64)) if split and (i, j) == SPLIT else ((0, 128),)):
            m = o_prod(s, i, j, r0=r0, nr=nr)
            if not first:
                m = accm[br, i * 7 + j, r0:r0 + nr] + m
            accm[br, i * 7 + j, r0:r0 + nr] = m

    def inner(i, get):
        return {(r2, c2 ^ _SWAP[i]): _signed_sum([(sg, get(j)) for j, sg in terms.items()])
                for (r2, c2), terms in _OUT.items()}

    def finalize_a(b, carry):
        rows = pl.ds(pl.multiple_of(b * RQ, RQ), RQ)
        res = {}
        for i in range(7):
            vals = [accm[0, i * 7 + j, rows, :] for j in range(7)]
            d = inner(i, lambda j: vals[j])
            for (r1, c1), terms in _OUT.items():
                if i in terms:
                    for k, v in d.items():
                        key = (r1, c1) + k
                        if key not in res:
                            assert terms[i] > 0
                            res[key] = v
                        else:
                            res[key] = res[key] + v if terms[i] > 0 else res[key] - v
        for (r1, c1, r2, c2), v in res.items():
            c = (2 * c1 + c2) * NQ4
            out_buf[0, b, r1, r2 * RQ:(r2 + 1) * RQ, c:c + NQ4] = v.astype(BF16)
        return carry

    def put_out(br, r1, r2, c0, val):
        nc = val.shape[1]
        out_buf[br, :, r1, r2 * RQ:(r2 + 1) * RQ, c0:c0 + nc] = val.reshape(B, RQ, nc).astype(BF16)

    def qk_group(j, is_a, bb):
        pts = []
        for b in range(bb * 4, bb * 4 + 4):
            q4 = _upk(jnp.concatenate(
                [q_buf[half * QMQ + b * 8:half * QMQ + (b + 1) * 8, h * DH:(h + 1) * DH]
                 for h in range(HPS) for half in range(2)], axis=0))
            if is_a:
                sc = lax.dot_general(ka_buf[b, j // 2], q4, NT, preferred_element_type=F32)
            else:
                st = lax.dot_general(kb_buf[b, j], q4, NT, preferred_element_type=F32)
                sc = st[0:SK]
                for h in range(1, HPS):
                    sc = jnp.where(lane_g == h, st[h * SK:(h + 1) * SK], sc)
            pts.append(_softmax_cols(sc))
        return jnp.concatenate(pts, axis=0).T

    def pv_tile(j, is_a, tt, bb, h):
        ph = tt[h * SQ:(h + 1) * SQ]
        lhs = jnp.concatenate([jnp.where(lane_g == bi, ph, 0.0) for bi in range(4)], axis=0).astype(BF16)
        if is_a:
            vh = jnp.concatenate([va_buf[bb * 4 + bi, j // 2] for bi in range(4)], axis=0)
        else:
            vh = jnp.concatenate(
                [vb_buf[bb * 4 + bi, j, h * SK:(h + 1) * SK, :] for bi in range(4)], axis=0)
        return lax.dot_general(lhs, vh, NN, preferred_element_type=F32)

    def pv_group(j, is_a, tt, bb, levels=2):
        t = [pv_tile(j, is_a, tt, bb, h) for h in range(HPS)]
        for pr in range(2):
            base = {(r, h): jnp.concatenate(
                [t[h][bi * SQ + r * RQ:bi * SQ + (r + 1) * RQ] for bi in (2 * pr, 2 * pr + 1)], axis=0)
                for r in range(4) for h in range(HPS)}
            r0 = (bb * 2 + pr) * 8
            for i in range(7):
                l1 = {(b0, b1): _comb(_LHS[i], lambda a: base[(2 * a[0] + b0, 2 * a[1] + b1)])
                      for b0 in range(2) for b1 in range(2)}
                if levels == 1:
                    for (b0, b1), v in l1.items():
                        jj = 2 * b0 + b1
                        os_buf[i * 64 + r0:i * 64 + r0 + 8, jj * DH:(jj + 1) * DH] = _pk(v)
                    continue
                for jj in range(7):
                    os_buf[i * 64 + r0:i * 64 + r0 + 8, jj * DH:(jj + 1) * DH] = _pk(_comb(_LHS[jj], lambda t2: l1[t2]))

    def attn_qproj(j, is_a, s, br, qs, ps, stages=range(7), tts=None):
        tts = [None] * 4 if tts is None else tts

        def run(pos):
            for g in qs.get(pos, ()):
                tts[g] = qk_group(j, is_a, g)
            for g in ps.get(pos, ()):
                pv_group(j, is_a, tts[g], g)

        for n in stages:
            run(n)
            has_mid = (n + 0.5) in qs or (n + 0.5) in ps
            q_stage(s, br, n, (lambda: run(n + 0.5)) if has_mid else None)
        run(7)
        return tts

    def oproj(so, bro, first=False, j=None, qs={}, split=False):
        tts = [None] * 4
        for n, (oi, oj) in enumerate(O_SEQ):
            for g in qs.get(n, ()):
                tts[g] = qk_group(j, False, g)
            o_step(so, bro, oi, oj, first, split)
        return tts

    SPA = False
    SPB = False
    P2Q = {0.5: (0, 1), 1.5: (2, 3)}
    P3P = {3: (0,), 3.5: (1,), 4.5: (2,), 5.5: (3,)}
    QSA = {0.5: (0, 1), 1.5: (2, 3)}
    QSB = {0.5: (0, 1), 1.5: (2, 3)}
    PSA = {2.5: (0,), 3.5: (1,), 4.5: (2,), 5.5: (3,)}
    PSB = {2.5: (0,), 3.5: (1,), 4.5: (2,), 5.5: (3,)}

    for n in range(4):
        with jax.named_scope("wait0"):
            wait_all(grp_r(n))
        with jax.named_scope("pro1"):
            xs = jnp.concatenate([x_block(0, a, n * KS, KS) for a in range(2)], axis=0)
            part = jnp.dot(xs, wq_buf[0, n * KS:(n + 1) * KS, :], preferred_element_type=F32)
            for a in range(2):
                for c in range(2):
                    pq = part[a * MH:(a + 1) * MH, c * QNH:(c + 1) * QNH]
                    if n == 0:
                        mq_buf[2 * a + c] = pq
                    elif n < 3:
                        mq_buf[2 * a + c] += pq
                    else:
                        q_buf[a * QMQ:(a + 1) * QMQ, c * QNH:(c + 1) * QNH] = _pk(mq_buf[2 * a + c] + pq)
            zero_acc(25 + 6 * n, 31 + 6 * n)
    with jax.named_scope("wait1"):
        wait_all(grp_r(4))
    with jax.named_scope("pro2"):
        tts0 = attn_qproj(0, True, 1, 0, P2Q, {}, stages=range(3))
    with jax.named_scope("wait2"):
        wait_all(grp_r(5))
    with jax.named_scope("pro3"):
        attn_qproj(0, True, 1, 0, {}, P3P, stages=range(3, 7), tts=tts0)
    with jax.named_scope("wait3"):
        wait_all(grp_r(6))
    with jax.named_scope("pro4"):
        oproj(0, 0, first=True, split=True)

    def body_a(s, carry):
        with jax.named_scope("waitA"):
            wait_all(grp_a(s, dyn=True))

            @pl.when(s % 2 == 0)
            def _():
                wait_all(grp_a_kv(s, dyn=True))

            @pl.when(s == NSB - 1)
            def _():
                xb_cp().wait()

        with jax.named_scope("bodyA"):
            attn_qproj(s, True, s + 1, (s + 1) // NSB, QSA, PSA)
            oproj(s, 0, split=SPA)
        return carry

    lax.fori_loop(1, NSB, body_a, 0)

    with jax.named_scope("finA"):
        lax.fori_loop(0, B, finalize_a, 0, unroll=4)
        out_cp(0, 0, D).start()

    def body_b(p, carry):
        u = 2 * p
        with jax.named_scope("waitB"):
            wait_all(grp_b(p, dyn=True))
        with jax.named_scope("bodyB"):
            attn_qproj(u, False, NSB + u + 1, 1, QSB, PSB)
            oproj(NSB + u, 1, split=SPB)
            attn_qproj(u + 1, False, NSB + u + 2, 1, QSB, PSB)
            oproj(NSB + u + 1, 1, split=SPB)
        return carry

    lax.fori_loop(0, NSB // 2 - 1, body_b, 0)

    with jax.named_scope("epi0"):
        wait_all(grp_b(NSB // 2 - 1))
    with jax.named_scope("epi1"):
        attn_qproj(NSB - 2, False, NS - 1, 1, QSB, PSB)
        tts = oproj(NS - 2, 1, j=NSB - 1, qs={4: (0, 1, 2, 3)}, split=True)
        for g in range(4):
            pv_group(NSB - 1, False, tts[g], g, levels=1)
        outs = [out_cp(0, 0, D)]
        for c2, c0, tc in ((0, 0, 256), (1, 0, 128), (1, 128, 128)):
            cc = c2 * NQ4 + c0

            def fm(i):
                lhs = _upk(jnp.concatenate(
                    [os_buf[i * 64:(i + 1) * 64, b0 * QNH:(b0 + 1) * QNH] for b0 in range(2)], axis=0))
                rhs = _operand(_RHS[i], lambda t: wo_buf[NS - 1, t[0] * QNH:(t[0] + 1) * QNH,
                                                         t[1] * NH + cc:t[1] * NH + cc + tc])
                m = jnp.dot(lhs, rhs, preferred_element_type=F32)
                return [_signed_sum([(1, m[r2 * 128:(r2 + 1) * 128])] +
                                    [(sg, accm[1, i * 7 + j, :, c0:c0 + tc])
                                     for j, sg in _OUT[(r2, c2 ^ _SWAP[i])].items()]) for r2 in range(2)]

            d = {}
            for i in (4, 1, 2, 0, 5, 3, 6):
                d[i] = fm(i)
                for (r1, c1), terms in _OUT.items():
                    if i in terms and set(terms) <= set(d):
                        for r2 in range(2):
                            put_out(1, r1, r2, c1 * NH + cc,
                                    _signed_sum([(sg, d[k][r2]) for k, sg in terms.items()]))
                if i in (5, 6):
                    outs.append(out_cp(1, (1 if i == 5 else 0) * NH + cc, tc))
                    outs[-1].start()
    with jax.named_scope("tail"):
        wait_all(outs)


@jax.jit
def pallas_concat_heads__gqa_block_cached__mha_block_cached__near_ridge_kernel(A_x, A_k_cache, A_v_cache, A_wq, A_wo, B_x, B_k_cache, B_v_cache, B_wq, B_wo):
    xa = A_x.reshape(B, 2, SH, D)
    xb = B_x.reshape(B, 2, SH, D)
    kb = B_k_cache.reshape(B, NSB, HPS * SK, DH)
    vb = B_v_cache.reshape(B, NSB, HPS * SK, DH)
    any_spec = pl.BlockSpec(memory_space=pl.ANY)
    out = pl.pallas_call(
        _kernel,
        in_specs=[any_spec] * 10,
        out_specs=any_spec,
        out_shape=jax.ShapeDtypeStruct((B, 2, SH, 2 * D), BF16),
        scratch_shapes=[
            pltpu.VMEM((2, B, 2, SH, D), BF16),
            pltpu.VMEM((B, HKV, SK, DH), BF16),
            pltpu.VMEM((B, HKV, SK, DH), BF16),
            pltpu.VMEM((B, NSB, HPS * SK, DH), BF16),
            pltpu.VMEM((B, NSB, HPS * SK, DH), BF16),
            pltpu.VMEM((NS, D, CH), BF16),
            pltpu.VMEM((NS, CH, D), BF16),
            pltpu.VMEM((M // 2, CH), U32),
            pltpu.VMEM((2, B, 2, SH, D), BF16),
            pltpu.VMEM((7 * B * RQ // 2, 7 * DH), U32),
            pltpu.VMEM((2, 49, B * RQ, NQ4), F32),
            pltpu.VMEM((4, MH, QNH), F32),
            pltpu.SemaphoreType.DMA((N_SEM,)),
        ],
        compiler_params=pltpu.CompilerParams(vmem_limit_bytes=100 * 1024 * 1024,
                                             disable_semaphore_checks=True),
        name="fused_attn",
    )(xa, A_k_cache, A_v_cache, A_wq, A_wo, xb, kb, vb, B_wq, B_wo)
    return out.reshape(B, SQ, 2 * D)
```

```python
import numpy as np
import jax
import jax.numpy as jnp
from jax import lax
import jax.experimental.pallas as pl
import jax.experimental.pallas.tpu as pltpu

B, SQ, D, H, HKV, SK, DH = 16, 32, 1024, 32, 4, 32, 128
M = B * SQ
MH = M // 2
SH = SQ // 2
HPS = 4
CH = HPS * DH
NSB = H // HPS
NS = 2 * NSB
KS = D // 4
NH = D // 2
QNH, QMQ = CH // 2, MH // 2
NQ4 = D // 4
RQ = SQ // 4
C_EXP2 = float(DH ** -0.5 * np.log2(np.e))
NT = (((1,), (1,)), ((), ()))
NN = (((1,), (0,)), ((), ()))
F32 = jnp.float32
BF16 = jnp.bfloat16
U32 = jnp.uint32

_LHS = [((0, 0), (1, 1), -1), ((1, 0), (1, 1), -1), ((0, 0), None, 0), ((1, 1), None, 0),
        ((0, 0), (0, 1), -1), ((1, 0), (0, 0), -1), ((0, 1), (1, 1), -1)]
_RHS = [((0, 0), (1, 1), -1), ((0, 0), None, 0), ((0, 1), (1, 1), 1), ((1, 0), (0, 0), 1),
        ((1, 1), None, 0), ((0, 0), (0, 1), 1), ((1, 0), (1, 1), 1)]
_OUT = {(0, 0): {0: 1, 3: 1, 4: 1, 6: 1}, (0, 1): {2: 1, 4: -1},
        (1, 0): {1: 1, 3: 1}, (1, 1): {0: 1, 1: -1, 2: 1, 5: 1}}
_SWAP = (0, 1, 0, 0, 1, 1, 1)
J_ORDER = (1, 4, 0, 2, 3, 5, 6)

def _o_order():
    nt = lambda i: 1 if _RHS[i][1] is None else 2
    allp = [(i, j) for i in range(7) for j in range(7)]
    heavy = [p for p in allp if nt(p[0]) * nt(p[1]) == 4]
    mid = [p for p in allp if nt(p[0]) * nt(p[1]) == 2]
    light = [p for p in allp if nt(p[0]) * nt(p[1]) == 1]
    mode = 0
    seq = []
    if mode == 0:
        lo = light[:2] + mid[:10] + light[2:] + mid[10:]
        seq = lo[:2]
        lo = lo[2:]
        while heavy or lo:
            if heavy:
                seq.append(heavy.pop(0))
            if lo:
                seq.append(lo.pop(0))
    elif mode == 1:
        lo = light[:2] + mid[:10] + light[2:] + mid[10:]
        while heavy or lo:
            seq += lo[:2]; lo = lo[2:]
            seq += heavy[:2]; heavy = heavy[2:]
    return tuple(seq)


O_SEQ = _o_order()
SPLIT = O_SEQ[0]

S_R = 0
S_A = 6
S_B = 13
S_E = 16
S_OUT = 17
N_SEM = 18
LA = NSB - 1


def _pk(x):
    return pltpu.bitcast(x.astype(BF16), U32)


def _upk(x):
    return pltpu.bitcast(x, BF16)


def _terms(spec):
    a, b, sg = spec
    return [(a, 1)] + ([(b, sg)] if b is not None else [])


def _signed_sum(items):
    items = sorted(items, key=lambda t: -t[0])
    acc = items[0][1]
    for sg, v in items[1:]:
        acc = acc + v if sg > 0 else acc - v
    return acc


def _comb(spec, get):
    return _signed_sum([(sg, get(t)) for t, sg in _terms(spec)])


def _operand(spec, ld):
    if spec[1] is None:
        return ld(spec[0])
    return _comb(spec, lambda t: ld(t).astype(F32)).astype(BF16)


def _softmax_cols(sc):
    m = jnp.max(sc, axis=0, keepdims=True)
    p = jnp.exp2((sc - m) * C_EXP2)
    l = jnp.sum(p, axis=0, keepdims=True)
    return p * (1.0 / l)


def _kernel(xa, ka, va, wqa, woa, xb, kb, vb, wqb, wob, out,
            x_buf, ka_buf, va_buf, kb_buf, vb_buf, wq_buf, wo_buf,
            q_buf, out_buf, os_buf, accm, mq_buf, sems):
    cp = pltpu.make_async_copy

    def wq_cp(s, sem, dyn=False):
        dst = wq_buf.at[s]
        src = dst if dyn else (wqa if s < NSB else wqb).at[:, pl.ds((s % NSB) * CH, CH)]
        return cp(src, dst, sems.at[sem])

    def wo_cp(s, sem, dyn=False):
        dst = wo_buf.at[s]
        src = dst if dyn else (woa if s < NSB else wob).at[pl.ds((s % NSB) * CH, CH), :]
        return cp(src, dst, sems.at[sem])

    def kv_cp(src, dst, j, n, sem, dyn=False, off=0):
        d = dst.at[:, pl.ds(j + off, n)]
        return cp(d if dyn else src.at[:, pl.ds(j, n)], d, sems.at[sem])

    def wq1_cp(a, b, sem):
        r, c = pl.ds(a * NH, NH), b * QNH
        return cp(wqa.at[r, pl.ds(CH + c, QNH)], wq_buf.at[1, r, pl.ds(c, QNH)], sems.at[sem])

    def grp_r(n):
        sem = S_R + n
        if n < 4:
            sl = pl.ds(n * KS, KS)
            return [cp(xa.at[:, :, :, sl], x_buf.at[0, :, :, :, sl], sems.at[sem]),
                    cp(wqa.at[sl, pl.ds(0, CH)], wq_buf.at[0, sl, :], sems.at[sem])]
        if n == 4:
            return [kv_cp(ka, ka_buf, 0, 1, sem), wq1_cp(0, 0, sem), wq1_cp(1, 1, sem)]
        if n == 5:
            return [kv_cp(va, va_buf, 0, 1, sem), wq1_cp(0, 1, sem), wq1_cp(1, 0, sem)]
        return [wo_cp(0, sem)]

    def next_a(s):
        return s + 1 + (s == LA - 1) * 1

    def grp_a(s, dyn=False):
        return [wq_cp(next_a(s), S_A + s, dyn), wo_cp(s, S_A + s, dyn)]

    def grp_a_kv(s, dyn=False):
        g = s // 2
        return [kv_cp(ka, ka_buf, g, 1, S_A + s, dyn), kv_cp(va, va_buf, g, 1, S_A + s, dyn)]

    def xb_cp():
        return cp(xb, x_buf.at[1], sems.at[S_A + LA - 1])

    def grp_b(p, dyn=False):
        u, sem = 2 * p, S_B + p
        return [kv_cp(kb, kb_buf, u, 2, sem, dyn), wq_cp(NSB + u + 1, sem, dyn),
                kv_cp(vb, vb_buf, u, 2, sem, dyn), wo_cp(NSB + u, sem, dyn),
                wq_cp(NSB + u + 2, sem, dyn), wo_cp(NSB + u + 1, sem, dyn)]

    def grp_e():
        return [kv_cp(kb, kb_buf, NSB - 2, 2, S_E), wq_cp(LA, S_E), kv_cp(vb, vb_buf, NSB - 2, 2, S_E),
                wo_cp(NS - 2, S_E), wq_cp(NS - 1, S_E), wo_cp(LA, S_E), wo_cp(NS - 1, S_E)]

    def out_cp(br, c0, nc):
        return cp(out_buf.at[br, :, :, :, pl.ds(c0, nc)],
                  out.at[:, :, :, pl.ds(br * D + c0, nc)], sems.at[S_OUT])

    def wait_all(cs):
        for c in cs:
            c.wait()

    for n in range(7):
        for c in grp_r(n):
            c.start()
    for s in range(1, LA):
        if s == LA - 1:
            xb_cp().start()
        for c in (grp_a_kv(s) if s % 2 == 0 else []) + grp_a(s):
            c.start()
    for p in range(NSB // 2 - 1):
        for c in grp_b(p):
            c.start()
    for c in grp_e():
        c.start()

    def zero_acc(k0, k1):
        accm[1, k0:k1] = jnp.zeros((k1 - k0,) + accm.shape[2:], F32)

    zero_acc(0, 25)

    lane_g = lax.broadcasted_iota(jnp.int32, (SK, 4 * SQ), 1) // SQ

    def x_block(br, half, c0, nc):
        return x_buf[br, :, half, :, c0:c0 + nc].reshape(MH, nc)

    def q_stage(s, br, n, mid=None):
        def q_prod(i):
            lhs = _operand(_LHS[i], lambda t: x_block(br, t[0], t[1] * NH, NH))

            def part(c0, nc):
                rhs = _operand(_RHS[i], lambda t: wq_buf[s, t[0] * NH:(t[0] + 1) * NH,
                                                         t[1] * QNH + c0:t[1] * QNH + c0 + nc])
                return jnp.dot(lhs, rhs, preferred_element_type=F32)

            if mid is None:
                return part(0, QNH)
            m0 = part(0, DH)
            mid()
            return jnp.concatenate([m0, part(DH, DH)], axis=1)

        if n == 0:
            mq_buf[0] = q_prod(1)
        elif n == 1:
            mq_buf[1] = q_prod(4)
        elif n == 2:
            m1 = q_prod(0)
            mq_buf[2] = m1 - mq_buf[0]
            mq_buf[3] = m1 + mq_buf[1]
        elif n == 3:
            m3 = q_prod(2)
            q_buf[:QMQ, QNH:] = _pk(m3 - mq_buf[1])
            mq_buf[2] += m3
        elif n == 4:
            m4 = q_prod(3)
            q_buf[QMQ:, :QNH] = _pk(m4 + mq_buf[0])
            mq_buf[3] += m4
        elif n == 5:
            q_buf[QMQ:, QNH:] = _pk(mq_buf[2] + q_prod(5))
        else:
            q_buf[:QMQ, :QNH] = _pk(mq_buf[3] + q_prod(6))

    def o_prod(s, i, j, c0=0, nc=NQ4, r0=0, nr=128):
        ts = [(s1 * s2, 2 * a[0] + b[0], 2 * a[1] + (b[1] ^ _SWAP[i]))
              for a, s1 in _terms(_RHS[i]) for b, s2 in _terms(_RHS[j])]
        ld = lambda r, c: wo_buf[s, r * DH:(r + 1) * DH, c * NQ4 + c0:c * NQ4 + c0 + nc]
        if len(ts) == 1:
            rhs = ld(ts[0][1], ts[0][2])
        else:
            rhs = _signed_sum([(sg, ld(r, c).astype(F32)) for sg, r, c in ts]).astype(BF16)
        return jnp.dot(_upk(os_buf[i * 64 + r0 // 2:i * 64 + (r0 + nr) // 2, j * DH:(j + 1) * DH]), rhs, preferred_element_type=F32)

    def o_step(s, br, i, j, first, split):
        for r0, nr in (((0, 64), (64, 64)) if split and (i, j) == SPLIT else ((0, 128),)):
            m = o_prod(s, i, j, r0=r0, nr=nr)
            if not first:
                m = accm[br, i * 7 + j, r0:r0 + nr] + m
            accm[br, i * 7 + j, r0:r0 + nr] = m

    def put_out(br, r1, r2, c0, val):
        nc = val.shape[1]
        out_buf[br, :, r1, r2 * RQ:(r2 + 1) * RQ, c0:c0 + nc] = val.reshape(B, RQ, nc).astype(BF16)

    def qk_group(j, is_a, bb):
        pts = []
        for b in range(bb * 4, bb * 4 + 4):
            q4 = _upk(jnp.concatenate(
                [q_buf[half * QMQ + b * 8:half * QMQ + (b + 1) * 8, h * DH:(h + 1) * DH]
                 for h in range(HPS) for half in range(2)], axis=0))
            if is_a:
                sc = lax.dot_general(ka_buf[b, j // 2], q4, NT, preferred_element_type=F32)
            else:
                st = lax.dot_general(kb_buf[b, j], q4, NT, preferred_element_type=F32)
                sc = st[0:SK]
                for h in range(1, HPS):
                    sc = jnp.where(lane_g == h, st[h * SK:(h + 1) * SK], sc)
            pts.append(_softmax_cols(sc))
        return jnp.concatenate(pts, axis=0).T

    def pv_tile(j, is_a, tt, bb, h):
        ph = tt[h * SQ:(h + 1) * SQ]
        lhs = jnp.concatenate([jnp.where(lane_g == bi, ph, 0.0) for bi in range(4)], axis=0).astype(BF16)
        if is_a:
            vh = jnp.concatenate([va_buf[bb * 4 + bi, j // 2] for bi in range(4)], axis=0)
        else:
            vh = jnp.concatenate(
                [vb_buf[bb * 4 + bi, j, h * SK:(h + 1) * SK, :] for bi in range(4)], axis=0)
        return lax.dot_general(lhs, vh, NN, preferred_element_type=F32)

    def pv_group(j, is_a, tt, bb, levels=2):
        t = [pv_tile(j, is_a, tt, bb, h) for h in range(HPS)]
        for pr in range(2):
            base = {(r, h): jnp.concatenate(
                [t[h][bi * SQ + r * RQ:bi * SQ + (r + 1) * RQ] for bi in (2 * pr, 2 * pr + 1)], axis=0)
                for r in range(4) for h in range(HPS)}
            r0 = (bb * 2 + pr) * 8
            for i in range(7):
                l1 = {(b0, b1): _comb(_LHS[i], lambda a: base[(2 * a[0] + b0, 2 * a[1] + b1)])
                      for b0 in range(2) for b1 in range(2)}
                if levels == 1:
                    for (b0, b1), v in l1.items():
                        jj = 2 * b0 + b1
                        os_buf[i * 64 + r0:i * 64 + r0 + 8, jj * DH:(jj + 1) * DH] = _pk(v)
                    continue
                for jj in range(7):
                    os_buf[i * 64 + r0:i * 64 + r0 + 8, jj * DH:(jj + 1) * DH] = _pk(_comb(_LHS[jj], lambda t2: l1[t2]))

    def attn_qproj(j, is_a, s, br, qs, ps, stages=range(7), tts=None, levels=2):
        tts = [None] * 4 if tts is None else tts

        def run(pos):
            for g in qs.get(pos, ()):
                tts[g] = qk_group(j, is_a, g)
            for g in ps.get(pos, ()):
                pv_group(j, is_a, tts[g], g, levels)

        for n in stages:
            run(n)
            has_mid = (n + 0.5) in qs or (n + 0.5) in ps
            q_stage(s, br, n, (lambda: run(n + 0.5)) if has_mid else None)
        run(7)
        return tts

    def oproj(so, bro, first=False, j=None, qs={}, split=False):
        tts = [None] * 4
        for n, (oi, oj) in enumerate(O_SEQ):
            for g in qs.get(n, ()):
                tts[g] = qk_group(j, False, g)
            o_step(so, bro, oi, oj, first, split)
        return tts

    SPA = False
    SPB = False
    P2Q = {0.5: (0, 1), 1.5: (2, 3)}
    P3P = {3: (0,), 3.5: (1,), 4.5: (2,), 5.5: (3,)}
    QSA = {0.5: (0,), 1: (1,), 1.5: (2,), 2.5: (3,)}
    QSB = {0.5: (0, 1), 1.5: (2, 3)}
    PSA = {3.5: (0,), 4.5: (1,), 5.5: (2,), 6.5: (3,)}
    PSB = {2.5: (0,), 3.5: (1,), 4.5: (2,), 5.5: (3,)}

    for n in range(4):
        with jax.named_scope("wait0"):
            wait_all(grp_r(n))
        with jax.named_scope("pro1"):
            xs = jnp.concatenate([x_block(0, a, n * KS, KS) for a in range(2)], axis=0)
            part = jnp.dot(xs, wq_buf[0, n * KS:(n + 1) * KS, :], preferred_element_type=F32)
            for a in range(2):
                for c in range(2):
                    pq = part[a * MH:(a + 1) * MH, c * QNH:(c + 1) * QNH]
                    if n == 0:
                        mq_buf[2 * a + c] = pq
                    elif n < 3:
                        mq_buf[2 * a + c] += pq
                    else:
                        q_buf[a * QMQ:(a + 1) * QMQ, c * QNH:(c + 1) * QNH] = _pk(mq_buf[2 * a + c] + pq)
            zero_acc(25 + 6 * n, 31 + 6 * n)
    with jax.named_scope("wait1"):
        wait_all(grp_r(4))
    with jax.named_scope("pro2"):
        tts0 = attn_qproj(0, True, 1, 0, P2Q, {}, stages=range(3))
    with jax.named_scope("wait2"):
        wait_all(grp_r(5))
    with jax.named_scope("pro3"):
        attn_qproj(0, True, 1, 0, {}, P3P, stages=range(3, 7), tts=tts0)
    with jax.named_scope("wait3"):
        wait_all(grp_r(6))
    with jax.named_scope("pro4"):
        oproj(0, 0, first=True, split=True)

    def body_a(s, carry):
        with jax.named_scope("waitA"):
            wait_all(grp_a(s, dyn=True))

            @pl.when(s % 2 == 0)
            def _():
                wait_all(grp_a_kv(s, dyn=True))

            @pl.when(s == LA - 1)
            def _():
                xb_cp().wait()

        with jax.named_scope("bodyA"):
            attn_qproj(s, True, next_a(s), (s + 1) // LA, QSA, PSA)
            oproj(s, 0, split=SPA)
        return carry

    lax.fori_loop(1, LA, body_a, 0)

    def body_b(p, carry):
        u = 2 * p
        with jax.named_scope("waitB"):
            wait_all(grp_b(p, dyn=True))
        with jax.named_scope("bodyB"):
            attn_qproj(u, False, NSB + u + 1, 1, QSB, PSB)
            oproj(NSB + u, 1, split=SPB)
            attn_qproj(u + 1, False, NSB + u + 2, 1, QSB, PSB)
            oproj(NSB + u + 1, 1, split=SPB)
        return carry

    lax.fori_loop(0, NSB // 2 - 1, body_b, 0)

    outs = []

    def final_oproj(s, br, chunks, qs={}):
        tts = [None] * 4
        n = 0
        for c2, c0, tc in chunks:
            cc = c2 * NQ4 + c0

            def fm(i):
                lhs = _upk(jnp.concatenate(
                    [os_buf[i * 64:(i + 1) * 64, b0 * QNH:(b0 + 1) * QNH] for b0 in range(2)], axis=0))
                rhs = _operand(_RHS[i], lambda t: wo_buf[s, t[0] * QNH:(t[0] + 1) * QNH,
                                                         t[1] * NH + cc:t[1] * NH + cc + tc])
                m = jnp.dot(lhs, rhs, preferred_element_type=F32)
                return [_signed_sum([(1, m[r2 * 128:(r2 + 1) * 128])] +
                                    [(sg, accm[br, i * 7 + j, :, c0:c0 + tc])
                                     for j, sg in _OUT[(r2, c2 ^ _SWAP[i])].items()]) for r2 in range(2)]

            d = {}
            for i in (4, 1, 2, 0, 5, 3, 6):
                for g in qs.get(n, ()):
                    tts[g] = qk_group(NSB - 1, False, g)
                n += 1
                d[i] = fm(i)
                for (r1, c1), terms in _OUT.items():
                    if i in terms and set(terms) <= set(d):
                        for r2 in range(2):
                            put_out(br, r1, r2, c1 * NH + cc,
                                    _signed_sum([(sg, d[k][r2]) for k, sg in terms.items()]))
                if i in (5, 6):
                    outs.append(out_cp(br, (1 if i == 5 else 0) * NH + cc, tc))
                    outs[-1].start()
        return tts

    with jax.named_scope("epi0"):
        wait_all(grp_e())
    with jax.named_scope("epi1"):
        attn_qproj(NSB - 2, False, LA, 0, QSB, PSB)
        oproj(NS - 2, 1, split=True)
        attn_qproj(LA, True, NS - 1, 1, QSB, PSB, levels=1)
        tts = final_oproj(LA, 0, ((0, 0, 256), (1, 0, 256)), qs={1: (0, 1, 2, 3)})
        for g in range(4):
            pv_group(NSB - 1, False, tts[g], g, levels=1)
        final_oproj(NS - 1, 1, ((0, 0, 256), (1, 0, 128), (1, 128, 128)))
    with jax.named_scope("tail"):
        wait_all(outs)


@jax.jit
def pallas_concat_heads__gqa_block_cached__mha_block_cached__near_ridge_kernel(A_x, A_k_cache, A_v_cache, A_wq, A_wo, B_x, B_k_cache, B_v_cache, B_wq, B_wo):
    xa = A_x.reshape(B, 2, SH, D)
    xb = B_x.reshape(B, 2, SH, D)
    kb = B_k_cache.reshape(B, NSB, HPS * SK, DH)
    vb = B_v_cache.reshape(B, NSB, HPS * SK, DH)
    any_spec = pl.BlockSpec(memory_space=pl.ANY)
    out = pl.pallas_call(
        _kernel,
        in_specs=[any_spec] * 10,
        out_specs=any_spec,
        out_shape=jax.ShapeDtypeStruct((B, 2, SH, 2 * D), BF16),
        scratch_shapes=[
            pltpu.VMEM((2, B, 2, SH, D), BF16),
            pltpu.VMEM((B, HKV, SK, DH), BF16),
            pltpu.VMEM((B, HKV, SK, DH), BF16),
            pltpu.VMEM((B, NSB, HPS * SK, DH), BF16),
            pltpu.VMEM((B, NSB, HPS * SK, DH), BF16),
            pltpu.VMEM((NS, D, CH), BF16),
            pltpu.VMEM((NS, CH, D), BF16),
            pltpu.VMEM((M // 2, CH), U32),
            pltpu.VMEM((2, B, 2, SH, D), BF16),
            pltpu.VMEM((7 * B * RQ // 2, 7 * DH), U32),
            pltpu.VMEM((2, 49, B * RQ, NQ4), F32),
            pltpu.VMEM((4, MH, QNH), F32),
            pltpu.SemaphoreType.DMA((N_SEM,)),
        ],
        compiler_params=pltpu.CompilerParams(vmem_limit_bytes=100 * 1024 * 1024,
                                             disable_semaphore_checks=True),
        name="fused_attn",
    )(xa, A_k_cache, A_v_cache, A_wq, A_wo, xb, kb, vb, B_wq, B_wo)
    return out.reshape(B, SQ, 2 * D)
```

```python
import numpy as np
import jax
import jax.numpy as jnp
from jax import lax
import jax.experimental.pallas as pl
import jax.experimental.pallas.tpu as pltpu

B, SQ, D, H, HKV, SK, DH = 16, 32, 1024, 32, 4, 32, 128
M = B * SQ
MH = M // 2
SH = SQ // 2
HPS = 4
CH = HPS * DH
NSB = H // HPS
NS = 2 * NSB
KS = D // 4
NH = D // 2
QNH, QMQ = CH // 2, MH // 2
NQ4 = D // 4
RQ = SQ // 4
C_EXP2 = float(DH ** -0.5 * np.log2(np.e))
NT = (((1,), (1,)), ((), ()))
NN = (((1,), (0,)), ((), ()))
F32 = jnp.float32
BF16 = jnp.bfloat16
U32 = jnp.uint32

_LHS = [((0, 0), (1, 1), -1), ((1, 0), (1, 1), -1), ((0, 0), None, 0), ((1, 1), None, 0),
        ((0, 0), (0, 1), -1), ((1, 0), (0, 0), -1), ((0, 1), (1, 1), -1)]
_RHS = [((0, 0), (1, 1), -1), ((0, 0), None, 0), ((0, 1), (1, 1), 1), ((1, 0), (0, 0), 1),
        ((1, 1), None, 0), ((0, 0), (0, 1), 1), ((1, 0), (1, 1), 1)]
_OUT = {(0, 0): {0: 1, 3: 1, 4: 1, 6: 1}, (0, 1): {2: 1, 4: -1},
        (1, 0): {1: 1, 3: 1}, (1, 1): {0: 1, 1: -1, 2: 1, 5: 1}}
_SWAP = (0, 1, 0, 0, 1, 1, 1)
J_ORDER = (1, 4, 0, 2, 3, 5, 6)

def _o_order():
    nt = lambda i: 1 if _RHS[i][1] is None else 2
    allp = [(i, j) for i in range(7) for j in range(7)]
    heavy = [p for p in allp if nt(p[0]) * nt(p[1]) == 4]
    mid = [p for p in allp if nt(p[0]) * nt(p[1]) == 2]
    light = [p for p in allp if nt(p[0]) * nt(p[1]) == 1]
    mode = 0
    seq = []
    if mode == 0:
        lo = light[:2] + mid[:10] + light[2:] + mid[10:]
        seq = lo[:2]
        lo = lo[2:]
        while heavy or lo:
            if heavy:
                seq.append(heavy.pop(0))
            if lo:
                seq.append(lo.pop(0))
    elif mode == 1:
        lo = light[:2] + mid[:10] + light[2:] + mid[10:]
        while heavy or lo:
            seq += lo[:2]; lo = lo[2:]
            seq += heavy[:2]; heavy = heavy[2:]
    return tuple(seq)


O_SEQ = _o_order()
SPLIT = O_SEQ[0]

KSL = (128, 128, 256, 256, 256)
NK = len(KSL)
S_R = 18
S_A = 6
S_B = 13
S_E = 16
S_OUT = 17
N_SEM = 18 + NK + 3
LA = NSB - 1


def _pk(x):
    return pltpu.bitcast(x.astype(BF16), U32)


def _upk(x):
    return pltpu.bitcast(x, BF16)


def _terms(spec):
    a, b, sg = spec
    return [(a, 1)] + ([(b, sg)] if b is not None else [])


def _signed_sum(items):
    items = sorted(items, key=lambda t: -t[0])
    acc = items[0][1]
    for sg, v in items[1:]:
        acc = acc + v if sg > 0 else acc - v
    return acc


def _comb(spec, get):
    return _signed_sum([(sg, get(t)) for t, sg in _terms(spec)])


def _operand(spec, ld):
    if spec[1] is None:
        return ld(spec[0])
    return _comb(spec, lambda t: ld(t).astype(F32)).astype(BF16)


def _softmax_cols(sc):
    m = jnp.max(sc, axis=0, keepdims=True)
    p = jnp.exp2((sc - m) * C_EXP2)
    l = jnp.sum(p, axis=0, keepdims=True)
    return p * (1.0 / l)


def _kernel(xa, ka, va, wqa, woa, xb, kb, vb, wqb, wob, out,
            x_buf, ka_buf, va_buf, kb_buf, vb_buf, wq_buf, wo_buf,
            q_buf, out_buf, os_buf, accm, mq_buf, sems):
    cp = pltpu.make_async_copy

    def wq_cp(s, sem, dyn=False):
        dst = wq_buf.at[s]
        src = dst if dyn else (wqa if s < NSB else wqb).at[:, pl.ds((s % NSB) * CH, CH)]
        return cp(src, dst, sems.at[sem])

    def wo_cp(s, sem, dyn=False):
        dst = wo_buf.at[s]
        src = dst if dyn else (woa if s < NSB else wob).at[pl.ds((s % NSB) * CH, CH), :]
        return cp(src, dst, sems.at[sem])

    def kv_cp(src, dst, j, n, sem, dyn=False, off=0):
        d = dst.at[:, pl.ds(j + off, n)]
        return cp(d if dyn else src.at[:, pl.ds(j, n)], d, sems.at[sem])

    def wq1_cp(a, b, sem):
        r, c = pl.ds(a * NH, NH), b * QNH
        return cp(wqa.at[r, pl.ds(CH + c, QNH)], wq_buf.at[1, r, pl.ds(c, QNH)], sems.at[sem])

    def grp_r(n):
        sem = S_R + n
        if n < NK:
            sl = pl.ds(sum(KSL[:n]), KSL[n])
            return [cp(xa.at[:, :, :, sl], x_buf.at[0, :, :, :, sl], sems.at[sem]),
                    cp(wqa.at[sl, pl.ds(0, CH)], wq_buf.at[0, sl, :], sems.at[sem])]
        if n == NK:
            return [kv_cp(ka, ka_buf, 0, 1, sem), wq1_cp(0, 0, sem), wq1_cp(1, 1, sem)]
        if n == NK + 1:
            return [kv_cp(va, va_buf, 0, 1, sem), wq1_cp(0, 1, sem), wq1_cp(1, 0, sem)]
        return [wo_cp(0, sem)]

    def next_a(s):
        return s + 1 + (s == LA - 1) * 1

    def grp_a(s, dyn=False):
        return [wq_cp(next_a(s), S_A + s, dyn), wo_cp(s, S_A + s, dyn)]

    def grp_a_kv(s, dyn=False):
        g = s // 2
        return [kv_cp(ka, ka_buf, g, 1, S_A + s, dyn), kv_cp(va, va_buf, g, 1, S_A + s, dyn)]

    def xb_cp():
        return cp(xb, x_buf.at[1], sems.at[S_A + LA - 1])

    def grp_b(p, dyn=False):
        u, sem = 2 * p, S_B + p
        return [kv_cp(kb, kb_buf, u, 2, sem, dyn), wq_cp(NSB + u + 1, sem, dyn),
                kv_cp(vb, vb_buf, u, 2, sem, dyn), wo_cp(NSB + u, sem, dyn),
                wq_cp(NSB + u + 2, sem, dyn), wo_cp(NSB + u + 1, sem, dyn)]

    def grp_e():
        return [kv_cp(kb, kb_buf, NSB - 2, 2, S_E), wq_cp(LA, S_E), kv_cp(vb, vb_buf, NSB - 2, 2, S_E),
                wo_cp(NS - 2, S_E), wq_cp(NS - 1, S_E), wo_cp(LA, S_E), wo_cp(NS - 1, S_E)]

    def out_cp(br, c0, nc):
        return cp(out_buf.at[br, :, :, :, pl.ds(c0, nc)],
                  out.at[:, :, :, pl.ds(br * D + c0, nc)], sems.at[S_OUT])

    def wait_all(cs):
        for c in cs:
            c.wait()

    for n in range(NK + 3):
        for c in grp_r(n):
            c.start()
    for s in range(1, LA):
        if s == LA - 1:
            xb_cp().start()
        for c in (grp_a_kv(s) if s % 2 == 0 else []) + grp_a(s):
            c.start()
    for p in range(NSB // 2 - 1):
        for c in grp_b(p):
            c.start()
    for c in grp_e():
        c.start()

    def zero_acc(k0, k1):
        accm[1, k0:k1] = jnp.zeros((k1 - k0,) + accm.shape[2:], F32)

    zero_acc(0, 25)

    lane_g = lax.broadcasted_iota(jnp.int32, (SK, 4 * SQ), 1) // SQ

    def x_block(br, half, c0, nc):
        return x_buf[br, :, half, :, c0:c0 + nc].reshape(MH, nc)

    def q_stage(s, br, n, mid=None):
        def q_prod(i):
            lhs = _operand(_LHS[i], lambda t: x_block(br, t[0], t[1] * NH, NH))

            def part(c0, nc):
                rhs = _operand(_RHS[i], lambda t: wq_buf[s, t[0] * NH:(t[0] + 1) * NH,
                                                         t[1] * QNH + c0:t[1] * QNH + c0 + nc])
                return jnp.dot(lhs, rhs, preferred_element_type=F32)

            if mid is None:
                return part(0, QNH)
            m0 = part(0, DH)
            mid()
            return jnp.concatenate([m0, part(DH, DH)], axis=1)

        if n == 0:
            mq_buf[0] = q_prod(1)
        elif n == 1:
            mq_buf[1] = q_prod(4)
        elif n == 2:
            m1 = q_prod(0)
            mq_buf[2] = m1 - mq_buf[0]
            mq_buf[3] = m1 + mq_buf[1]
        elif n == 3:
            m3 = q_prod(2)
            q_buf[:QMQ, QNH:] = _pk(m3 - mq_buf[1])
            mq_buf[2] += m3
        elif n == 4:
            m4 = q_prod(3)
            q_buf[QMQ:, :QNH] = _pk(m4 + mq_buf[0])
            mq_buf[3] += m4
        elif n == 5:
            q_buf[QMQ:, QNH:] = _pk(mq_buf[2] + q_prod(5))
        else:
            q_buf[:QMQ, :QNH] = _pk(mq_buf[3] + q_prod(6))

    def o_prod(s, i, j, c0=0, nc=NQ4, r0=0, nr=128):
        ts = [(s1 * s2, 2 * a[0] + b[0], 2 * a[1] + (b[1] ^ _SWAP[i]))
              for a, s1 in _terms(_RHS[i]) for b, s2 in _terms(_RHS[j])]
        ld = lambda r, c: wo_buf[s, r * DH:(r + 1) * DH, c * NQ4 + c0:c * NQ4 + c0 + nc]
        if len(ts) == 1:
            rhs = ld(ts[0][1], ts[0][2])
        else:
            rhs = _signed_sum([(sg, ld(r, c).astype(F32)) for sg, r, c in ts]).astype(BF16)
        return jnp.dot(_upk(os_buf[i * 64 + r0 // 2:i * 64 + (r0 + nr) // 2, j * DH:(j + 1) * DH]), rhs, preferred_element_type=F32)

    def o_step(s, br, i, j, first, split):
        for r0, nr in (((0, 64), (64, 64)) if split and (i, j) == SPLIT else ((0, 128),)):
            m = o_prod(s, i, j, r0=r0, nr=nr)
            if not first:
                m = accm[br, i * 7 + j, r0:r0 + nr] + m
            accm[br, i * 7 + j, r0:r0 + nr] = m

    def put_out(br, r1, r2, c0, val):
        nc = val.shape[1]
        out_buf[br, :, r1, r2 * RQ:(r2 + 1) * RQ, c0:c0 + nc] = val.reshape(B, RQ, nc).astype(BF16)

    def qk_group(j, is_a, bb):
        pts = []
        for b in range(bb * 4, bb * 4 + 4):
            q4 = _upk(jnp.concatenate(
                [q_buf[half * QMQ + b * 8:half * QMQ + (b + 1) * 8, h * DH:(h + 1) * DH]
                 for h in range(HPS) for half in range(2)], axis=0))
            if is_a:
                sc = lax.dot_general(ka_buf[b, j // 2], q4, NT, preferred_element_type=F32)
            else:
                st = lax.dot_general(kb_buf[b, j], q4, NT, preferred_element_type=F32)
                sc = st[0:SK]
                for h in range(1, HPS):
                    sc = jnp.where(lane_g == h, st[h * SK:(h + 1) * SK], sc)
            pts.append(_softmax_cols(sc))
        return jnp.concatenate(pts, axis=0).T

    def pv_tile(j, is_a, tt, bb, h):
        ph = tt[h * SQ:(h + 1) * SQ]
        lhs = jnp.concatenate([jnp.where(lane_g == bi, ph, 0.0) for bi in range(4)], axis=0).astype(BF16)
        if is_a:
            vh = jnp.concatenate([va_buf[bb * 4 + bi, j // 2] for bi in range(4)], axis=0)
        else:
            vh = jnp.concatenate(
                [vb_buf[bb * 4 + bi, j, h * SK:(h + 1) * SK, :] for bi in range(4)], axis=0)
        return lax.dot_general(lhs, vh, NN, preferred_element_type=F32)

    def pv_group(j, is_a, tt, bb, levels=2):
        t = [pv_tile(j, is_a, tt, bb, h) for h in range(HPS)]
        for pr in range(2):
            base = {(r, h): jnp.concatenate(
                [t[h][bi * SQ + r * RQ:bi * SQ + (r + 1) * RQ] for bi in (2 * pr, 2 * pr + 1)], axis=0)
                for r in range(4) for h in range(HPS)}
            r0 = (bb * 2 + pr) * 8
            for i in range(7):
                l1 = {(b0, b1): _comb(_LHS[i], lambda a: base[(2 * a[0] + b0, 2 * a[1] + b1)])
                      for b0 in range(2) for b1 in range(2)}
                if levels == 1:
                    for (b0, b1), v in l1.items():
                        jj = 2 * b0 + b1
                        os_buf[i * 64 + r0:i * 64 + r0 + 8, jj * DH:(jj + 1) * DH] = _pk(v)
                    continue
                for jj in range(7):
                    os_buf[i * 64 + r0:i * 64 + r0 + 8, jj * DH:(jj + 1) * DH] = _pk(_comb(_LHS[jj], lambda t2: l1[t2]))

    def attn_qproj(j, is_a, s, br, qs, ps, stages=range(7), tts=None, levels=2):
        tts = [None] * 4 if tts is None else tts

        def run(pos):
            for g in qs.get(pos, ()):
                tts[g] = qk_group(j, is_a, g)
            for g in ps.get(pos, ()):
                pv_group(j, is_a, tts[g], g, levels)

        for n in stages:
            run(n)
            has_mid = (n + 0.5) in qs or (n + 0.5) in ps
            q_stage(s, br, n, (lambda: run(n + 0.5)) if has_mid else None)
        run(7)
        return tts

    def oproj(so, bro, first=False, j=None, qs={}, split=False):
        tts = [None] * 4
        for n, (oi, oj) in enumerate(O_SEQ):
            for g in qs.get(n, ()):
                tts[g] = qk_group(j, False, g)
            o_step(so, bro, oi, oj, first, split)
        return tts

    SPA = False
    SPB = False
    P2Q = {0.5: (0, 1), 1.5: (2, 3)}
    P3P = {3: (0,), 3.5: (1,), 4.5: (2,), 5.5: (3,)}
    QSA = {0.5: (0,), 1: (1,), 1.5: (2,), 2.5: (3,)}
    QSB = {0.5: (0, 1), 1.5: (2, 3)}
    PSA = {3.5: (0,), 4.5: (1,), 5.5: (2,), 6.5: (3,)}
    PSB = {2.5: (0,), 3.5: (1,), 4.5: (2,), 5.5: (3,)}

    for n in range(NK):
        with jax.named_scope("wait0"):
            wait_all(grp_r(n))
        with jax.named_scope("pro1"):
            k0, kn = sum(KSL[:n]), KSL[n]
            xs = jnp.concatenate([x_block(0, a, k0, kn) for a in range(2)], axis=0)
            part = jnp.dot(xs, wq_buf[0, k0:k0 + kn, :], preferred_element_type=F32)
            for a in range(2):
                for c in range(2):
                    pq = part[a * MH:(a + 1) * MH, c * QNH:(c + 1) * QNH]
                    if n == 0:
                        mq_buf[2 * a + c] = pq
                    elif n < NK - 1:
                        mq_buf[2 * a + c] += pq
                    else:
                        q_buf[a * QMQ:(a + 1) * QMQ, c * QNH:(c + 1) * QNH] = _pk(mq_buf[2 * a + c] + pq)
            if n >= NK - 3:
                zero_acc(25 + 8 * (n - NK + 3), 33 + 8 * (n - NK + 3))
    with jax.named_scope("wait1"):
        wait_all(grp_r(NK))
    with jax.named_scope("pro2"):
        tts0 = attn_qproj(0, True, 1, 0, P2Q, {}, stages=range(3))
    with jax.named_scope("wait2"):
        wait_all(grp_r(NK + 1))
    with jax.named_scope("pro3"):
        attn_qproj(0, True, 1, 0, {}, P3P, stages=range(3, 7), tts=tts0)
    with jax.named_scope("wait3"):
        wait_all(grp_r(NK + 2))
    with jax.named_scope("pro4"):
        oproj(0, 0, first=True, split=True)

    def body_a(s, carry):
        with jax.named_scope("waitA"):
            wait_all(grp_a(s, dyn=True))

            @pl.when(s % 2 == 0)
            def _():
                wait_all(grp_a_kv(s, dyn=True))

            @pl.when(s == LA - 1)
            def _():
                xb_cp().wait()

        with jax.named_scope("bodyA"):
            attn_qproj(s, True, next_a(s), (s + 1) // LA, QSA, PSA)
            oproj(s, 0, split=SPA)
        return carry

    lax.fori_loop(1, LA, body_a, 0)

    def body_b(p, carry):
        u = 2 * p
        with jax.named_scope("waitB"):
            wait_all(grp_b(p, dyn=True))
        with jax.named_scope("bodyB"):
            attn_qproj(u, False, NSB + u + 1, 1, QSB, PSB)
            oproj(NSB + u, 1, split=SPB)
            attn_qproj(u + 1, False, NSB + u + 2, 1, QSB, PSB)
            oproj(NSB + u + 1, 1, split=SPB)
        return carry

    lax.fori_loop(0, NSB // 2 - 1, body_b, 0)

    outs = []

    def final_oproj(s, br, chunks, qs={}):
        tts = [None] * 4
        n = 0
        for c2, c0, tc in chunks:
            cc = c2 * NQ4 + c0

            def fm(i):
                lhs = _upk(jnp.concatenate(
                    [os_buf[i * 64:(i + 1) * 64, b0 * QNH:(b0 + 1) * QNH] for b0 in range(2)], axis=0))
                rhs = _operand(_RHS[i], lambda t: wo_buf[s, t[0] * QNH:(t[0] + 1) * QNH,
                                                         t[1] * NH + cc:t[1] * NH + cc + tc])
                m = jnp.dot(lhs, rhs, preferred_element_type=F32)
                return [_signed_sum([(1, m[r2 * 128:(r2 + 1) * 128])] +
                                    [(sg, accm[br, i * 7 + j, :, c0:c0 + tc])
                                     for j, sg in _OUT[(r2, c2 ^ _SWAP[i])].items()]) for r2 in range(2)]

            d = {}
            for i in (4, 1, 2, 0, 5, 3, 6):
                for g in qs.get(n, ()):
                    tts[g] = qk_group(NSB - 1, False, g)
                n += 1
                d[i] = fm(i)
                for (r1, c1), terms in _OUT.items():
                    if i in terms and set(terms) <= set(d):
                        for r2 in range(2):
                            put_out(br, r1, r2, c1 * NH + cc,
                                    _signed_sum([(sg, d[k][r2]) for k, sg in terms.items()]))
                if i in (5, 6):
                    outs.append(out_cp(br, (1 if i == 5 else 0) * NH + cc, tc))
                    outs[-1].start()
        return tts

    with jax.named_scope("epi0"):
        wait_all(grp_e())
    with jax.named_scope("epi1"):
        attn_qproj(NSB - 2, False, LA, 0, QSB, PSB)
        oproj(NS - 2, 1, split=True)
        attn_qproj(LA, True, NS - 1, 1, QSB, PSB, levels=1)
        tts = final_oproj(LA, 0, ((0, 0, 256), (1, 0, 256)), qs={1: (0, 1, 2, 3)})
        for g in range(4):
            pv_group(NSB - 1, False, tts[g], g, levels=1)
        final_oproj(NS - 1, 1, ((0, 0, 256), (1, 0, 128), (1, 128, 128)))
    with jax.named_scope("tail"):
        wait_all(outs)


@jax.jit
def pallas_concat_heads__gqa_block_cached__mha_block_cached__near_ridge_kernel(A_x, A_k_cache, A_v_cache, A_wq, A_wo, B_x, B_k_cache, B_v_cache, B_wq, B_wo):
    xa = A_x.reshape(B, 2, SH, D)
    xb = B_x.reshape(B, 2, SH, D)
    kb = B_k_cache.reshape(B, NSB, HPS * SK, DH)
    vb = B_v_cache.reshape(B, NSB, HPS * SK, DH)
    any_spec = pl.BlockSpec(memory_space=pl.ANY)
    out = pl.pallas_call(
        _kernel,
        in_specs=[any_spec] * 10,
        out_specs=any_spec,
        out_shape=jax.ShapeDtypeStruct((B, 2, SH, 2 * D), BF16),
        scratch_shapes=[
            pltpu.VMEM((2, B, 2, SH, D), BF16),
            pltpu.VMEM((B, HKV, SK, DH), BF16),
            pltpu.VMEM((B, HKV, SK, DH), BF16),
            pltpu.VMEM((B, NSB, HPS * SK, DH), BF16),
            pltpu.VMEM((B, NSB, HPS * SK, DH), BF16),
            pltpu.VMEM((NS, D, CH), BF16),
            pltpu.VMEM((NS, CH, D), BF16),
            pltpu.VMEM((M // 2, CH), U32),
            pltpu.VMEM((2, B, 2, SH, D), BF16),
            pltpu.VMEM((7 * B * RQ // 2, 7 * DH), U32),
            pltpu.VMEM((2, 49, B * RQ, NQ4), F32),
            pltpu.VMEM((4, MH, QNH), F32),
            pltpu.SemaphoreType.DMA((N_SEM,)),
        ],
        compiler_params=pltpu.CompilerParams(vmem_limit_bytes=100 * 1024 * 1024,
                                             disable_semaphore_checks=True),
        name="fused_attn",
    )(xa, A_k_cache, A_v_cache, A_wq, A_wo, xb, kb, vb, B_wq, B_wo)
    return out.reshape(B, SQ, 2 * D)
```

```python
import numpy as np
import jax
import jax.numpy as jnp
from jax import lax
import jax.experimental.pallas as pl
import jax.experimental.pallas.tpu as pltpu

B, SQ, D, H, HKV, SK, DH = 16, 32, 1024, 32, 4, 32, 128
M = B * SQ
MH = M // 2
MQ = M // 4
SH, RQ = SQ // 2, SQ // 4
HPS = 4
CH = HPS * DH
NSB = H // HPS
NS = 2 * NSB
LA = NSB - 1
NH, NQ4 = D // 2, D // 4
QNH, QMQ = CH // 2, MH // 2
KSL = (128, 128, 256, 256, 256)
NK = len(KSL)
C_EXP2 = float(DH ** -0.5 * np.log2(np.e))
NT = (((1,), (1,)), ((), ()))
NN = (((1,), (0,)), ((), ()))
F32 = jnp.float32
BF16 = jnp.bfloat16
U32 = jnp.uint32

_LHS = [((0, 0), (1, 1), -1), ((1, 0), (1, 1), -1), ((0, 0), None, 0), ((1, 1), None, 0),
        ((0, 0), (0, 1), -1), ((1, 0), (0, 0), -1), ((0, 1), (1, 1), -1)]
_RHS = [((0, 0), (1, 1), -1), ((0, 0), None, 0), ((0, 1), (1, 1), 1), ((1, 0), (0, 0), 1),
        ((1, 1), None, 0), ((0, 0), (0, 1), 1), ((1, 0), (1, 1), 1)]
_OUT = {(0, 0): {0: 1, 3: 1, 4: 1, 6: 1}, (0, 1): {2: 1, 4: -1},
        (1, 0): {1: 1, 3: 1}, (1, 1): {0: 1, 1: -1, 2: 1, 5: 1}}
_SWAP = (0, 1, 0, 0, 1, 1, 1)


def _o_order():
    nt = [1 if r[1] is None else 2 for r in _RHS]
    allp = [(i, j) for i in range(7) for j in range(7)]
    heavy, mid, light = ([p for p in allp if nt[p[0]] * nt[p[1]] == n] for n in (4, 2, 1))
    cheap = mid[:10] + light[2:] + mid[10:]
    seq = light[:2]
    while heavy or cheap:
        seq += heavy[:1] + cheap[:1]
        heavy, cheap = heavy[1:], cheap[1:]
    return tuple(seq)


O_SEQ = _o_order()

QK_PAIRS = {0.5: (0, 1), 1.5: (2, 3)}
QK_SPREAD = {0.5: (0,), 1: (1,), 1.5: (2,), 2.5: (3,)}
PV_FIRST = {3: (0,), 3.5: (1,), 4.5: (2,), 5.5: (3,)}
PV_EARLY = {2.5: (0,), 3.5: (1,), 4.5: (2,), 5.5: (3,)}
PV_LATE = {3.5: (0,), 4.5: (1,), 5.5: (2,), 6.5: (3,)}

S_OUT = 0
S_A = 0
S_B = LA
S_E = S_B + NSB // 2 - 1
S_R = S_E + 1
N_SEM = S_R + NK + 3


def _pk(x):
    return pltpu.bitcast(x.astype(BF16), U32)


def _upk(x):
    return pltpu.bitcast(x, BF16)


def _terms(spec):
    a, b, sg = spec
    return [(a, 1)] + ([(b, sg)] if b is not None else [])


def _signed_sum(items):
    items = sorted(items, key=lambda t: -t[0])
    acc = items[0][1]
    for sg, v in items[1:]:
        acc = acc + v if sg > 0 else acc - v
    return acc


def _comb(spec, get):
    return _signed_sum([(sg, get(t)) for t, sg in _terms(spec)])


def _operand(spec, ld):
    if spec[1] is None:
        return ld(spec[0])
    return _comb(spec, lambda t: ld(t).astype(F32)).astype(BF16)


def _softmax_cols(sc):
    m = jnp.max(sc, axis=0, keepdims=True)
    p = jnp.exp2((sc - m) * C_EXP2)
    l = jnp.sum(p, axis=0, keepdims=True)
    return p * (1.0 / l)


def _kernel(xa, ka, va, wqa, woa, xb, kb, vb, wqb, wob, out,
            x_buf, ka_buf, va_buf, kb_buf, vb_buf, wq_buf, wo_buf,
            q_buf, out_buf, os_buf, accm, mq_buf, sems):
    cp = pltpu.make_async_copy

    def wq_cp(s, sem, dyn=False):
        dst = wq_buf.at[s]
        src = dst if dyn else (wqa if s < NSB else wqb).at[:, pl.ds((s % NSB) * CH, CH)]
        return cp(src, dst, sems.at[sem])

    def wo_cp(s, sem, dyn=False):
        dst = wo_buf.at[s]
        src = dst if dyn else (woa if s < NSB else wob).at[pl.ds((s % NSB) * CH, CH), :]
        return cp(src, dst, sems.at[sem])

    def kv_cp(src, dst, j, n, sem, dyn=False):
        d = dst.at[:, pl.ds(j, n)]
        return cp(d if dyn else src.at[:, pl.ds(j, n)], d, sems.at[sem])

    def wq1_cp(a, b, sem):
        r, c = pl.ds(a * NH, NH), b * QNH
        return cp(wqa.at[r, pl.ds(CH + c, QNH)], wq_buf.at[1, r, pl.ds(c, QNH)], sems.at[sem])

    def grp_r(n):
        sem = S_R + n
        if n < NK:
            sl = pl.ds(sum(KSL[:n]), KSL[n])
            return [cp(xa.at[:, :, :, sl], x_buf.at[0, :, :, :, sl], sems.at[sem]),
                    cp(wqa.at[sl, pl.ds(0, CH)], wq_buf.at[0, sl, :], sems.at[sem])]
        if n == NK:
            return [kv_cp(ka, ka_buf, 0, 1, sem), wq1_cp(0, 0, sem), wq1_cp(1, 1, sem)]
        if n == NK + 1:
            return [kv_cp(va, va_buf, 0, 1, sem), wq1_cp(0, 1, sem), wq1_cp(1, 0, sem)]
        return [wo_cp(0, sem)]

    def next_a(s):
        return s + 1 + (s == LA - 1) * 1

    def grp_a(s, dyn=False):
        return [wq_cp(next_a(s), S_A + s, dyn), wo_cp(s, S_A + s, dyn)]

    def grp_a_kv(s, dyn=False):
        g = s // 2
        return [kv_cp(ka, ka_buf, g, 1, S_A + s, dyn), kv_cp(va, va_buf, g, 1, S_A + s, dyn)]

    def xb_cp():
        return cp(xb, x_buf.at[1], sems.at[S_A + LA - 1])

    def grp_b(p, dyn=False):
        u, sem = 2 * p, S_B + p
        return [kv_cp(kb, kb_buf, u, 2, sem, dyn), wq_cp(NSB + u + 1, sem, dyn),
                kv_cp(vb, vb_buf, u, 2, sem, dyn), wo_cp(NSB + u, sem, dyn),
                wq_cp(NSB + u + 2, sem, dyn), wo_cp(NSB + u + 1, sem, dyn)]

    def grp_e():
        return [kv_cp(kb, kb_buf, NSB - 2, 2, S_E), wq_cp(LA, S_E), kv_cp(vb, vb_buf, NSB - 2, 2, S_E),
                wo_cp(NS - 2, S_E), wq_cp(NS - 1, S_E), wo_cp(LA, S_E), wo_cp(NS - 1, S_E)]

    def out_cp(br, c0, nc):
        return cp(out_buf.at[br, :, :, :, pl.ds(c0, nc)],
                  out.at[:, :, :, pl.ds(br * D + c0, nc)], sems.at[S_OUT])

    def wait_all(cs):
        for c in cs:
            c.wait()

    for n in range(NK + 3):
        for c in grp_r(n):
            c.start()
    for s in range(1, LA):
        if s == LA - 1:
            xb_cp().start()
        for c in (grp_a_kv(s) if s % 2 == 0 else []) + grp_a(s):
            c.start()
    for p in range(NSB // 2 - 1):
        for c in grp_b(p):
            c.start()
    for c in grp_e():
        c.start()

    def zero_acc(k0, k1):
        accm[1, k0:k1] = jnp.zeros((k1 - k0,) + accm.shape[2:], F32)

    zero_acc(0, 25)

    lane_g = lax.broadcasted_iota(jnp.int32, (SK, 4 * SQ), 1) // SQ

    def x_block(br, half, c0, nc):
        return x_buf[br, :, half, :, c0:c0 + nc].reshape(MH, nc)

    def q_stage(s, br, n, mid=None):
        def q_prod(i):
            lhs = _operand(_LHS[i], lambda t: x_block(br, t[0], t[1] * NH, NH))

            def part(c0, nc):
                rhs = _operand(_RHS[i], lambda t: wq_buf[s, t[0] * NH:(t[0] + 1) * NH,
                                                         t[1] * QNH + c0:t[1] * QNH + c0 + nc])
                return jnp.dot(lhs, rhs, preferred_element_type=F32)

            if mid is None:
                return part(0, QNH)
            m0 = part(0, DH)
            mid()
            return jnp.concatenate([m0, part(DH, DH)], axis=1)

        if n == 0:
            mq_buf[0] = q_prod(1)
        elif n == 1:
            mq_buf[1] = q_prod(4)
        elif n == 2:
            p0 = q_prod(0)
            mq_buf[2] = p0 - mq_buf[0]
            mq_buf[3] = p0 + mq_buf[1]
        elif n == 3:
            p2 = q_prod(2)
            q_buf[:QMQ, QNH:] = _pk(p2 - mq_buf[1])
            mq_buf[2] += p2
        elif n == 4:
            p3 = q_prod(3)
            q_buf[QMQ:, :QNH] = _pk(p3 + mq_buf[0])
            mq_buf[3] += p3
        elif n == 5:
            q_buf[QMQ:, QNH:] = _pk(mq_buf[2] + q_prod(5))
        else:
            q_buf[:QMQ, :QNH] = _pk(mq_buf[3] + q_prod(6))

    def o_prod(s, i, j, r0, nr):
        ts = [(s1 * s2, 2 * a[0] + b[0], 2 * a[1] + (b[1] ^ _SWAP[i]))
              for a, s1 in _terms(_RHS[i]) for b, s2 in _terms(_RHS[j])]
        ld = lambda r, c: wo_buf[s, r * DH:(r + 1) * DH, c * NQ4:(c + 1) * NQ4]
        if len(ts) == 1:
            rhs = ld(ts[0][1], ts[0][2])
        else:
            rhs = _signed_sum([(sg, ld(r, c).astype(F32)) for sg, r, c in ts]).astype(BF16)
        lhs = _upk(os_buf[(i * MQ + r0) // 2:(i * MQ + r0 + nr) // 2, j * DH:(j + 1) * DH])
        return jnp.dot(lhs, rhs, preferred_element_type=F32)

    def oproj(s, br, first=False, split=False):
        for n, (i, j) in enumerate(O_SEQ):
            for r0, nr in (((0, MQ // 2), (MQ // 2, MQ // 2)) if split and n == 0 else ((0, MQ),)):
                m = o_prod(s, i, j, r0, nr)
                if not first:
                    m = accm[br, i * 7 + j, r0:r0 + nr] + m
                accm[br, i * 7 + j, r0:r0 + nr] = m

    def qk_group(j, is_a, bb):
        pts = []
        for b in range(bb * 4, bb * 4 + 4):
            q4 = _upk(jnp.concatenate(
                [q_buf[half * QMQ + b * 8:half * QMQ + (b + 1) * 8, h * DH:(h + 1) * DH]
                 for h in range(HPS) for half in range(2)], axis=0))
            if is_a:
                sc = lax.dot_general(ka_buf[b, j // 2], q4, NT, preferred_element_type=F32)
            else:
                st = lax.dot_general(kb_buf[b, j], q4, NT, preferred_element_type=F32)
                sc = st[0:SK]
                for h in range(1, HPS):
                    sc = jnp.where(lane_g == h, st[h * SK:(h + 1) * SK], sc)
            pts.append(_softmax_cols(sc))
        return jnp.concatenate(pts, axis=0).T

    def pv_tile(j, is_a, tt, bb, h):
        ph = tt[h * SQ:(h + 1) * SQ]
        lhs = jnp.concatenate([jnp.where(lane_g == bi, ph, 0.0) for bi in range(4)], axis=0).astype(BF16)
        if is_a:
            vh = jnp.concatenate([va_buf[bb * 4 + bi, j // 2] for bi in range(4)], axis=0)
        else:
            vh = jnp.concatenate(
                [vb_buf[bb * 4 + bi, j, h * SK:(h + 1) * SK, :] for bi in range(4)], axis=0)
        return lax.dot_general(lhs, vh, NN, preferred_element_type=F32)

    def pv_group(j, is_a, tt, bb, levels):
        t = [pv_tile(j, is_a, tt, bb, h) for h in range(HPS)]
        for pr in range(2):
            base = {(r, h): jnp.concatenate(
                [t[h][bi * SQ + r * RQ:bi * SQ + (r + 1) * RQ] for bi in (2 * pr, 2 * pr + 1)], axis=0)
                for r in range(4) for h in range(HPS)}
            for i in range(7):
                r0 = i * MQ // 2 + (bb * 2 + pr) * RQ
                l1 = {(b0, b1): _comb(_LHS[i], lambda a: base[(2 * a[0] + b0, 2 * a[1] + b1)])
                      for b0 in range(2) for b1 in range(2)}
                if levels == 1:
                    ops = list(l1.values())
                else:
                    ops = [None] * 7
                for jj, v in enumerate(ops):
                    v = _comb(_LHS[jj], lambda t2: l1[t2]) if v is None else v
                    os_buf[r0:r0 + RQ, jj * DH:(jj + 1) * DH] = _pk(v)

    def attn_qproj(j, is_a, s, br, qs, ps, stages=range(7), tts=None, levels=2):
        tts = [None] * 4 if tts is None else tts

        def run(pos):
            for g in qs.get(pos, ()):
                tts[g] = qk_group(j, is_a, g)
            for g in ps.get(pos, ()):
                pv_group(j, is_a, tts[g], g, levels)

        for n in stages:
            run(n)
            has_mid = (n + 0.5) in qs or (n + 0.5) in ps
            q_stage(s, br, n, (lambda: run(n + 0.5)) if has_mid else None)
        return tts

    outs = []

    def final_oproj(s, br, chunks, with_qk):
        tts = None
        for c2, c0, tc in chunks:
            cc = c2 * NQ4 + c0

            def total(i):
                lhs = _upk(jnp.concatenate(
                    [os_buf[i * MQ // 2:(i + 1) * MQ // 2, b0 * QNH:(b0 + 1) * QNH] for b0 in range(2)],
                    axis=0))
                rhs = _operand(_RHS[i], lambda t: wo_buf[s, t[0] * QNH:(t[0] + 1) * QNH,
                                                         t[1] * NH + cc:t[1] * NH + cc + tc])
                m = jnp.dot(lhs, rhs, preferred_element_type=F32)
                return [_signed_sum([(1, m[r2 * MQ:(r2 + 1) * MQ])] +
                                    [(sg, accm[br, i * 7 + j, :, c0:c0 + tc])
                                     for j, sg in _OUT[(r2, c2 ^ _SWAP[i])].items()]) for r2 in range(2)]

            d = {}
            for i in (4, 1, 2, 0, 5, 3, 6):
                if with_qk and tts is None and d:
                    tts = [qk_group(NSB - 1, False, g) for g in range(4)]
                d[i] = total(i)
                for (r1, c1), terms in _OUT.items():
                    if i in terms and set(terms) <= set(d):
                        for r2 in range(2):
                            val = _signed_sum([(sg, d[k][r2]) for k, sg in terms.items()])
                            out_buf[br, :, r1, r2 * RQ:(r2 + 1) * RQ, c1 * NH + cc:c1 * NH + cc + tc] = (
                                val.reshape(B, RQ, tc).astype(BF16))
                if i in (5, 6):
                    outs.append(out_cp(br, (1 if i == 5 else 0) * NH + cc, tc))
                    outs[-1].start()
        return tts

    for n in range(NK):
        with jax.named_scope("wait0"):
            wait_all(grp_r(n))
        with jax.named_scope("pro1"):
            k0, kn = sum(KSL[:n]), KSL[n]
            xs = jnp.concatenate([x_block(0, a, k0, kn) for a in range(2)], axis=0)
            part = jnp.dot(xs, wq_buf[0, k0:k0 + kn, :], preferred_element_type=F32)
            for a in range(2):
                for c in range(2):
                    pq = part[a * MH:(a + 1) * MH, c * QNH:(c + 1) * QNH]
                    if n == 0:
                        mq_buf[2 * a + c] = pq
                    elif n < NK - 1:
                        mq_buf[2 * a + c] += pq
                    else:
                        q_buf[a * QMQ:(a + 1) * QMQ, c * QNH:(c + 1) * QNH] = _pk(mq_buf[2 * a + c] + pq)
            if n >= NK - 3:
                zero_acc(25 + 8 * (n - NK + 3), 33 + 8 * (n - NK + 3))
    with jax.named_scope("wait1"):
        wait_all(grp_r(NK))
    with jax.named_scope("pro2"):
        tts0 = attn_qproj(0, True, 1, 0, QK_PAIRS, {}, stages=range(3))
    with jax.named_scope("wait2"):
        wait_all(grp_r(NK + 1))
    with jax.named_scope("pro3"):
        attn_qproj(0, True, 1, 0, {}, PV_FIRST, stages=range(3, 7), tts=tts0)
    with jax.named_scope("wait3"):
        wait_all(grp_r(NK + 2))
    with jax.named_scope("pro4"):
        oproj(0, 0, first=True, split=True)

    def body_a(s, carry):
        with jax.named_scope("waitA"):
            wait_all(grp_a(s, dyn=True))

            @pl.when(s % 2 == 0)
            def _():
                wait_all(grp_a_kv(s, dyn=True))

            @pl.when(s == LA - 1)
            def _():
                xb_cp().wait()

        with jax.named_scope("bodyA"):
            attn_qproj(s, True, next_a(s), (s + 1) // LA, QK_SPREAD, PV_LATE)
            oproj(s, 0)
        return carry

    lax.fori_loop(1, LA, body_a, 0)

    def body_b(p, carry):
        u = 2 * p
        with jax.named_scope("waitB"):
            wait_all(grp_b(p, dyn=True))
        with jax.named_scope("bodyB"):
            attn_qproj(u, False, NSB + u + 1, 1, QK_PAIRS, PV_EARLY)
            oproj(NSB + u, 1)
            attn_qproj(u + 1, False, NSB + u + 2, 1, QK_PAIRS, PV_EARLY)
            oproj(NSB + u + 1, 1)
        return carry

    lax.fori_loop(0, NSB // 2 - 1, body_b, 0)

    with jax.named_scope("epi0"):
        wait_all(grp_e())
    with jax.named_scope("epi1"):
        attn_qproj(NSB - 2, False, LA, 0, QK_PAIRS, PV_EARLY)
        oproj(NS - 2, 1, split=True)
        attn_qproj(LA, True, NS - 1, 1, QK_PAIRS, PV_EARLY, levels=1)
        tts = final_oproj(LA, 0, ((0, 0, 256), (1, 0, 256)), True)
        for g in range(4):
            pv_group(NSB - 1, False, tts[g], g, 1)
        final_oproj(NS - 1, 1, ((0, 0, 256), (1, 0, 128), (1, 128, 128)), False)
    with jax.named_scope("tail"):
        wait_all(outs)


@jax.jit
def pallas_concat_heads__gqa_block_cached__mha_block_cached__near_ridge_kernel(A_x, A_k_cache, A_v_cache, A_wq, A_wo, B_x, B_k_cache, B_v_cache, B_wq, B_wo):
    xa = A_x.reshape(B, 2, SH, D)
    xb = B_x.reshape(B, 2, SH, D)
    kb = B_k_cache.reshape(B, NSB, HPS * SK, DH)
    vb = B_v_cache.reshape(B, NSB, HPS * SK, DH)
    any_spec = pl.BlockSpec(memory_space=pl.ANY)
    out = pl.pallas_call(
        _kernel,
        in_specs=[any_spec] * 10,
        out_specs=any_spec,
        out_shape=jax.ShapeDtypeStruct((B, 2, SH, 2 * D), BF16),
        scratch_shapes=[
            pltpu.VMEM((2, B, 2, SH, D), BF16),
            pltpu.VMEM((B, HKV, SK, DH), BF16),
            pltpu.VMEM((B, HKV, SK, DH), BF16),
            pltpu.VMEM((B, NSB, HPS * SK, DH), BF16),
            pltpu.VMEM((B, NSB, HPS * SK, DH), BF16),
            pltpu.VMEM((NS, D, CH), BF16),
            pltpu.VMEM((NS, CH, D), BF16),
            pltpu.VMEM((M // 2, CH), U32),
            pltpu.VMEM((2, B, 2, SH, D), BF16),
            pltpu.VMEM((7 * MQ // 2, 7 * DH), U32),
            pltpu.VMEM((2, 49, MQ, NQ4), F32),
            pltpu.VMEM((4, MH, QNH), F32),
            pltpu.SemaphoreType.DMA((N_SEM,)),
        ],
        compiler_params=pltpu.CompilerParams(vmem_limit_bytes=100 * 1024 * 1024,
                                             disable_semaphore_checks=True),
        name="fused_attn",
    )(xa, A_k_cache, A_v_cache, A_wq, A_wo, xb, kb, vb, B_wq, B_wo)
    return out.reshape(B, SQ, 2 * D)
```

```python
import numpy as np
import jax
import jax.numpy as jnp
from jax import lax
import jax.experimental.pallas as pl
import jax.experimental.pallas.tpu as pltpu

B, SQ, D, H, HKV, SK, DH = 16, 32, 1024, 32, 4, 32, 128
M = B * SQ
MH = M // 2
MQ = M // 4
SH, RQ = SQ // 2, SQ // 4
HPS = 4
CH = HPS * DH
NSB = H // HPS
NS = 2 * NSB
LA = NSB - 1
NH, NQ4 = D // 2, D // 4
QNH, QMQ = CH // 2, MH // 2
KSL = (128, 128, 256, 256, 256)
NK = len(KSL)
C_EXP2 = float(DH ** -0.5 * np.log2(np.e))
NT = (((1,), (1,)), ((), ()))
NN = (((1,), (0,)), ((), ()))
F32 = jnp.float32
BF16 = jnp.bfloat16
U32 = jnp.uint32

_LHS = [((0, 0), (1, 1), -1), ((1, 0), (1, 1), -1), ((0, 0), None, 0), ((1, 1), None, 0),
        ((0, 0), (0, 1), -1), ((1, 0), (0, 0), -1), ((0, 1), (1, 1), -1)]
_RHS = [((0, 0), (1, 1), -1), ((0, 0), None, 0), ((0, 1), (1, 1), 1), ((1, 0), (0, 0), 1),
        ((1, 1), None, 0), ((0, 0), (0, 1), 1), ((1, 0), (1, 1), 1)]
_OUT = {(0, 0): {0: 1, 3: 1, 4: 1, 6: 1}, (0, 1): {2: 1, 4: -1},
        (1, 0): {1: 1, 3: 1}, (1, 1): {0: 1, 1: -1, 2: 1, 5: 1}}
_SWAP = (0, 1, 0, 0, 1, 1, 1)


def _o_order():
    nt = [1 if r[1] is None else 2 for r in _RHS]
    allp = [(i, j) for i in range(7) for j in range(7)]
    heavy, mid, light = ([p for p in allp if nt[p[0]] * nt[p[1]] == n] for n in (4, 2, 1))
    cheap = mid[:10] + light[2:] + mid[10:]
    seq = light[:2]
    while heavy or cheap:
        seq += heavy[:1] + cheap[:1]
        heavy, cheap = heavy[1:], cheap[1:]
    return tuple(seq)


O_SEQ = _o_order()

QK_PAIRS = {0.5: (0, 1), 1.5: (2, 3)}
QK_SPREAD = {0.5: (0,), 1: (1,), 1.5: (2,), 2.5: (3,)}
PV_FIRST = {3: (0,), 3.5: (1,), 4.5: (2,), 5.5: (3,)}
PV_EARLY = {2.5: (0,), 3.5: (1,), 4.5: (2,), 5.5: (3,)}
PV_LATE = {3.5: (0,), 4.5: (1,), 5.5: (2,), 6.5: (3,)}

S_OUT = 0
S_A = 0
S_B = LA
S_E = S_B + NSB // 2 - 1
S_R = S_E + 1
N_SEM = S_R + NK + 3


def _pk(x):
    return pltpu.bitcast(x.astype(BF16), U32)


def _upk(x):
    return pltpu.bitcast(x, BF16)


def _terms(spec):
    a, b, sg = spec
    return [(a, 1)] + ([(b, sg)] if b is not None else [])


def _signed_sum(items):
    items = sorted(items, key=lambda t: -t[0])
    acc = items[0][1]
    for sg, v in items[1:]:
        acc = acc + v if sg > 0 else acc - v
    return acc


def _comb(spec, get):
    return _signed_sum([(sg, get(t)) for t, sg in _terms(spec)])


def _operand(spec, ld):
    if spec[1] is None:
        return ld(spec[0])
    return _comb(spec, lambda t: ld(t).astype(F32)).astype(BF16)


def _softmax_cols(sc):
    m = jnp.max(sc, axis=0, keepdims=True)
    p = jnp.exp2((sc - m) * C_EXP2)
    l = jnp.sum(p, axis=0, keepdims=True)
    return p * (1.0 / l)


def _kernel(xa, ka, va, wqa, woa, xb, kb, vb, wqb, wob, out,
            x_buf, ka_buf, va_buf, kb_buf, vb_buf, wq_buf, wo_buf,
            q_buf, out_buf, os_buf, accm, mq_buf, sems):
    cp = pltpu.make_async_copy

    def wq_cp(s, sem, dyn=False):
        dst = wq_buf.at[s]
        src = dst if dyn else (wqa if s < NSB else wqb).at[:, pl.ds((s % NSB) * CH, CH)]
        return cp(src, dst, sems.at[sem])

    def wo_cp(s, sem, dyn=False):
        dst = wo_buf.at[s]
        src = dst if dyn else (woa if s < NSB else wob).at[pl.ds((s % NSB) * CH, CH), :]
        return cp(src, dst, sems.at[sem])

    def kv_cp(src, dst, j, n, sem, dyn=False):
        d = dst.at[:, pl.ds(j, n)]
        return cp(d if dyn else src.at[:, pl.ds(j, n)], d, sems.at[sem])

    def wq1_cp(a, b, sem):
        r, c = pl.ds(a * NH, NH), b * QNH
        return cp(wqa.at[r, pl.ds(CH + c, QNH)], wq_buf.at[1, r, pl.ds(c, QNH)], sems.at[sem])

    def grp_r(n):
        sem = S_R + n
        if n < NK:
            sl = pl.ds(sum(KSL[:n]), KSL[n])
            return [cp(xa.at[:, :, :, sl], x_buf.at[0, :, :, :, sl], sems.at[sem]),
                    cp(wqa.at[sl, pl.ds(0, CH)], wq_buf.at[0, sl, :], sems.at[sem])]
        if n == NK:
            return [kv_cp(ka, ka_buf, 0, 1, sem), wq1_cp(0, 0, sem), wq1_cp(1, 1, sem)]
        if n == NK + 1:
            return [kv_cp(va, va_buf, 0, 1, sem), wq1_cp(0, 1, sem), wq1_cp(1, 0, sem)]
        return [wo_cp(0, sem)]

    def next_a(s):
        return s + 1 + (s == LA - 1) * 1

    def grp_a(s, dyn=False):
        return [wq_cp(next_a(s), S_A + s, dyn), wo_cp(s, S_A + s, dyn)]

    def grp_a_kv(s, dyn=False):
        g = s >> 1
        return [kv_cp(ka, ka_buf, g, 1, S_A + s, dyn), kv_cp(va, va_buf, g, 1, S_A + s, dyn)]

    def xb_cp():
        return cp(xb, x_buf.at[1], sems.at[S_A + LA - 1])

    def grp_b(p, dyn=False):
        u, sem = 2 * p, S_B + p
        return [kv_cp(kb, kb_buf, u, 2, sem, dyn), wq_cp(NSB + u + 1, sem, dyn),
                kv_cp(vb, vb_buf, u, 2, sem, dyn), wo_cp(NSB + u, sem, dyn),
                wq_cp(NSB + u + 2, sem, dyn), wo_cp(NSB + u + 1, sem, dyn)]

    def grp_e():
        return [kv_cp(kb, kb_buf, NSB - 2, 2, S_E), wq_cp(LA, S_E), kv_cp(vb, vb_buf, NSB - 2, 2, S_E),
                wo_cp(NS - 2, S_E), wq_cp(NS - 1, S_E), wo_cp(LA, S_E), wo_cp(NS - 1, S_E)]

    def out_cp(br, c0, nc):
        return cp(out_buf.at[br, :, :, :, pl.ds(c0, nc)],
                  out.at[:, :, :, pl.ds(br * D + c0, nc)], sems.at[S_OUT])

    def wait_all(cs):
        for c in cs:
            c.wait()

    for n in range(NK + 3):
        for c in grp_r(n):
            c.start()
    for s in range(1, LA):
        if s == LA - 1:
            xb_cp().start()
        for c in (grp_a_kv(s) if s % 2 == 0 else []) + grp_a(s):
            c.start()
    for p in range(NSB // 2 - 1):
        for c in grp_b(p):
            c.start()
    for c in grp_e():
        c.start()

    def zero_acc(k0, k1):
        accm[1, k0:k1] = jnp.zeros((k1 - k0,) + accm.shape[2:], F32)

    zero_acc(0, 25)

    lane_g = lax.broadcasted_iota(jnp.int32, (SK, 4 * SQ), 1) // SQ

    def x_block(br, half, c0, nc):
        return x_buf[br, :, half, :, c0:c0 + nc].reshape(MH, nc)

    def q_stage(s, br, n, mid=None):
        def q_prod(i):
            lhs = _operand(_LHS[i], lambda t: x_block(br, t[0], t[1] * NH, NH))

            def part(c0, nc):
                rhs = _operand(_RHS[i], lambda t: wq_buf[s, t[0] * NH:(t[0] + 1) * NH,
                                                         t[1] * QNH + c0:t[1] * QNH + c0 + nc])
                return jnp.dot(lhs, rhs, preferred_element_type=F32)

            if mid is None:
                return part(0, QNH)
            m0 = part(0, DH)
            mid()
            return jnp.concatenate([m0, part(DH, DH)], axis=1)

        if n == 0:
            mq_buf[0] = q_prod(1)
        elif n == 1:
            mq_buf[1] = q_prod(4)
        elif n == 2:
            p0 = q_prod(0)
            mq_buf[2] = p0 - mq_buf[0]
            mq_buf[3] = p0 + mq_buf[1]
        elif n == 3:
            p2 = q_prod(2)
            q_buf[:QMQ, QNH:] = _pk(p2 - mq_buf[1])
            mq_buf[2] += p2
        elif n == 4:
            p3 = q_prod(3)
            q_buf[QMQ:, :QNH] = _pk(p3 + mq_buf[0])
            mq_buf[3] += p3
        elif n == 5:
            q_buf[QMQ:, QNH:] = _pk(mq_buf[2] + q_prod(5))
        else:
            q_buf[:QMQ, :QNH] = _pk(mq_buf[3] + q_prod(6))

    def o_prod(s, i, j, r0, nr):
        ts = [(s1 * s2, 2 * a[0] + b[0], 2 * a[1] + (b[1] ^ _SWAP[i]))
              for a, s1 in _terms(_RHS[i]) for b, s2 in _terms(_RHS[j])]
        ld = lambda r, c: wo_buf[s, r * DH:(r + 1) * DH, c * NQ4:(c + 1) * NQ4]
        if len(ts) == 1:
            rhs = ld(ts[0][1], ts[0][2])
        else:
            rhs = _signed_sum([(sg, ld(r, c).astype(F32)) for sg, r, c in ts]).astype(BF16)
        lhs = _upk(os_buf[(i * MQ + r0) // 2:(i * MQ + r0 + nr) // 2, j * DH:(j + 1) * DH])
        return jnp.dot(lhs, rhs, preferred_element_type=F32)

    def oproj(s, br, first=False, split=False):
        for n, (i, j) in enumerate(O_SEQ):
            for r0, nr in (((0, MQ // 2), (MQ // 2, MQ // 2)) if split and n == 0 else ((0, MQ),)):
                m = o_prod(s, i, j, r0, nr)
                if not first:
                    m = accm[br, i * 7 + j, r0:r0 + nr] + m
                accm[br, i * 7 + j, r0:r0 + nr] = m

    def qk_group(j, is_a, bb):
        pts = []
        for b in range(bb * 4, bb * 4 + 4):
            q4 = _upk(jnp.concatenate(
                [q_buf[half * QMQ + b * 8:half * QMQ + (b + 1) * 8, h * DH:(h + 1) * DH]
                 for h in range(HPS) for half in range(2)], axis=0))
            if is_a:
                sc = lax.dot_general(ka_buf[b, j >> 1], q4, NT, preferred_element_type=F32)
            else:
                st = lax.dot_general(kb_buf[b, j], q4, NT, preferred_element_type=F32)
                sc = st[0:SK]
                for h in range(1, HPS):
                    sc = jnp.where(lane_g == h, st[h * SK:(h + 1) * SK], sc)
            pts.append(_softmax_cols(sc))
        return jnp.concatenate(pts, axis=0).T

    def pv_tile(j, is_a, tt, bb, h):
        ph = tt[h * SQ:(h + 1) * SQ]
        lhs = jnp.concatenate([jnp.where(lane_g == bi, ph, 0.0) for bi in range(4)], axis=0).astype(BF16)
        if is_a:
            vh = jnp.concatenate([va_buf[bb * 4 + bi, j >> 1] for bi in range(4)], axis=0)
        else:
            vh = jnp.concatenate(
                [vb_buf[bb * 4 + bi, j, h * SK:(h + 1) * SK, :] for bi in range(4)], axis=0)
        return lax.dot_general(lhs, vh, NN, preferred_element_type=F32)

    def pv_group(j, is_a, tt, bb, levels):
        t = [pv_tile(j, is_a, tt, bb, h) for h in range(HPS)]
        for pr in range(2):
            base = {(r, h): jnp.concatenate(
                [t[h][bi * SQ + r * RQ:bi * SQ + (r + 1) * RQ] for bi in (2 * pr, 2 * pr + 1)], axis=0)
                for r in range(4) for h in range(HPS)}
            for i in range(7):
                r0 = i * MQ // 2 + (bb * 2 + pr) * RQ
                l1 = {(b0, b1): _comb(_LHS[i], lambda a: base[(2 * a[0] + b0, 2 * a[1] + b1)])
                      for b0 in range(2) for b1 in range(2)}
                if levels == 1:
                    ops = list(l1.values())
                else:
                    ops = [None] * 7
                for jj, v in enumerate(ops):
                    v = _comb(_LHS[jj], lambda t2: l1[t2]) if v is None else v
                    os_buf[r0:r0 + RQ, jj * DH:(jj + 1) * DH] = _pk(v)

    def attn_qproj(j, is_a, s, br, qs, ps, stages=range(7), tts=None, levels=2):
        tts = [None] * 4 if tts is None else tts

        def run(pos):
            for g in qs.get(pos, ()):
                tts[g] = qk_group(j, is_a, g)
            for g in ps.get(pos, ()):
                pv_group(j, is_a, tts[g], g, levels)

        for n in stages:
            run(n)
            has_mid = (n + 0.5) in qs or (n + 0.5) in ps
            q_stage(s, br, n, (lambda: run(n + 0.5)) if has_mid else None)
        return tts

    outs = []

    def final_oproj(s, br, chunks, with_qk):
        tts = None
        for c2, c0, tc in chunks:
            cc = c2 * NQ4 + c0

            def total(i):
                lhs = _upk(jnp.concatenate(
                    [os_buf[i * MQ // 2:(i + 1) * MQ // 2, b0 * QNH:(b0 + 1) * QNH] for b0 in range(2)],
                    axis=0))
                rhs = _operand(_RHS[i], lambda t: wo_buf[s, t[0] * QNH:(t[0] + 1) * QNH,
                                                         t[1] * NH + cc:t[1] * NH + cc + tc])
                m = jnp.dot(lhs, rhs, preferred_element_type=F32)
                return [_signed_sum([(1, m[r2 * MQ:(r2 + 1) * MQ])] +
                                    [(sg, accm[br, i * 7 + j, :, c0:c0 + tc])
                                     for j, sg in _OUT[(r2, c2 ^ _SWAP[i])].items()]) for r2 in range(2)]

            d = {}
            for i in (4, 1, 2, 0, 5, 3, 6):
                if with_qk and tts is None and d:
                    tts = [qk_group(NSB - 1, False, g) for g in range(4)]
                d[i] = total(i)
                for (r1, c1), terms in _OUT.items():
                    if i in terms and set(terms) <= set(d):
                        for r2 in range(2):
                            val = _signed_sum([(sg, d[k][r2]) for k, sg in terms.items()])
                            out_buf[br, :, r1, r2 * RQ:(r2 + 1) * RQ, c1 * NH + cc:c1 * NH + cc + tc] = (
                                val.reshape(B, RQ, tc).astype(BF16))
                if i in (5, 6):
                    outs.append(out_cp(br, (1 if i == 5 else 0) * NH + cc, tc))
                    outs[-1].start()
        return tts

    for n in range(NK):
        with jax.named_scope("wait0"):
            wait_all(grp_r(n))
        with jax.named_scope("pro1"):
            k0, kn = sum(KSL[:n]), KSL[n]
            xs = jnp.concatenate([x_block(0, a, k0, kn) for a in range(2)], axis=0)
            part = jnp.dot(xs, wq_buf[0, k0:k0 + kn, :], preferred_element_type=F32)
            for a in range(2):
                for c in range(2):
                    pq = part[a * MH:(a + 1) * MH, c * QNH:(c + 1) * QNH]
                    if n == 0:
                        mq_buf[2 * a + c] = pq
                    elif n < NK - 1:
                        mq_buf[2 * a + c] += pq
                    else:
                        q_buf[a * QMQ:(a + 1) * QMQ, c * QNH:(c + 1) * QNH] = _pk(mq_buf[2 * a + c] + pq)
            z0 = 25 + sum(k // 128 * 3 for k in KSL[:n])
            zero_acc(z0, z0 + kn // 128 * 3)
    with jax.named_scope("wait1"):
        wait_all(grp_r(NK))
    with jax.named_scope("pro2"):
        tts0 = attn_qproj(0, True, 1, 0, QK_PAIRS, {}, stages=range(3))
    with jax.named_scope("wait2"):
        wait_all(grp_r(NK + 1))
    with jax.named_scope("pro3"):
        attn_qproj(0, True, 1, 0, {}, PV_FIRST, stages=range(3, 7), tts=tts0)
    with jax.named_scope("wait3"):
        wait_all(grp_r(NK + 2))
    with jax.named_scope("pro4"):
        oproj(0, 0, first=True, split=True)

    def body_a(s, carry):
        with jax.named_scope("waitA"):
            @pl.when((s & 1) == 0)
            def _():
                wait_all(grp_a_kv(s, dyn=True))

            @pl.when(s == LA - 1)
            def _():
                xb_cp().wait()

            wait_all(grp_a(s, dyn=True))

        with jax.named_scope("bodyA"):
            attn_qproj(s, True, next_a(s), (s == LA - 1) * 1, QK_SPREAD, PV_LATE)
            oproj(s, 0)
        return carry

    lax.fori_loop(1, LA, body_a, 0)

    def body_b(p, carry):
        u = 2 * p
        with jax.named_scope("waitB"):
            wait_all(grp_b(p, dyn=True))
        with jax.named_scope("bodyB"):
            attn_qproj(u, False, NSB + u + 1, 1, QK_PAIRS, PV_EARLY)
            oproj(NSB + u, 1)
            attn_qproj(u + 1, False, NSB + u + 2, 1, QK_PAIRS, PV_EARLY)
            oproj(NSB + u + 1, 1)
        return carry

    lax.fori_loop(0, NSB // 2 - 1, body_b, 0)

    with jax.named_scope("epi0"):
        wait_all(grp_e())
    with jax.named_scope("epi1"):
        attn_qproj(NSB - 2, False, LA, 0, QK_PAIRS, PV_EARLY)
        oproj(NS - 2, 1, split=True)
        attn_qproj(LA, True, NS - 1, 1, QK_PAIRS, PV_EARLY, levels=1)
        tts = final_oproj(LA, 0, ((0, 0, 256), (1, 0, 256)), True)
        for g in range(4):
            pv_group(NSB - 1, False, tts[g], g, 1)
        final_oproj(NS - 1, 1, ((0, 0, 256), (1, 0, 128), (1, 128, 128)), False)
    with jax.named_scope("tail"):
        wait_all(outs)


@jax.jit
def pallas_concat_heads__gqa_block_cached__mha_block_cached__near_ridge_kernel(A_x, A_k_cache, A_v_cache, A_wq, A_wo, B_x, B_k_cache, B_v_cache, B_wq, B_wo):
    xa = A_x.reshape(B, 2, SH, D)
    xb = B_x.reshape(B, 2, SH, D)
    kb = B_k_cache.reshape(B, NSB, HPS * SK, DH)
    vb = B_v_cache.reshape(B, NSB, HPS * SK, DH)
    any_spec = pl.BlockSpec(memory_space=pl.ANY)
    out = pl.pallas_call(
        _kernel,
        in_specs=[any_spec] * 10,
        out_specs=any_spec,
        out_shape=jax.ShapeDtypeStruct((B, 2, SH, 2 * D), BF16),
        scratch_shapes=[
            pltpu.VMEM((2, B, 2, SH, D), BF16),
            pltpu.VMEM((B, HKV, SK, DH), BF16),
            pltpu.VMEM((B, HKV, SK, DH), BF16),
            pltpu.VMEM((B, NSB, HPS * SK, DH), BF16),
            pltpu.VMEM((B, NSB, HPS * SK, DH), BF16),
            pltpu.VMEM((NS, D, CH), BF16),
            pltpu.VMEM((NS, CH, D), BF16),
            pltpu.VMEM((M // 2, CH), U32),
            pltpu.VMEM((2, B, 2, SH, D), BF16),
            pltpu.VMEM((7 * MQ // 2, 7 * DH), U32),
            pltpu.VMEM((2, 49, MQ, NQ4), F32),
            pltpu.VMEM((4, MH, QNH), F32),
            pltpu.SemaphoreType.DMA((N_SEM,)),
        ],
        compiler_params=pltpu.CompilerParams(vmem_limit_bytes=100 * 1024 * 1024,
                                             disable_semaphore_checks=True),
        name="fused_attn",
    )(xa, A_k_cache, A_v_cache, A_wq, A_wo, xb, kb, vb, B_wq, B_wo)
    return out.reshape(B, SQ, 2 * D)
```

```python
import numpy as np
import jax
import jax.numpy as jnp
from jax import lax
import jax.experimental.pallas as pl
import jax.experimental.pallas.tpu as pltpu

B, SQ, D, H, HKV, SK, DH = 16, 32, 1024, 32, 4, 32, 128
M = B * SQ
MH = M // 2
MQ = M // 4
SH, RQ = SQ // 2, SQ // 4
HPS = 4
CH = HPS * DH
NSB = H // HPS
NS = 2 * NSB
LA = NSB - 1
NH, NQ4 = D // 2, D // 4
QNH, QMQ = CH // 2, MH // 2
KSL = (128, 128, 256)
NK = len(KSL)
C_EXP2 = float(DH ** -0.5 * np.log2(np.e))
NT = (((1,), (1,)), ((), ()))
NN = (((1,), (0,)), ((), ()))
F32 = jnp.float32
BF16 = jnp.bfloat16
U32 = jnp.uint32

_LHS = [((0, 0), (1, 1), -1), ((1, 0), (1, 1), -1), ((0, 0), None, 0), ((1, 1), None, 0),
        ((0, 0), (0, 1), -1), ((1, 0), (0, 0), -1), ((0, 1), (1, 1), -1)]
_RHS = [((0, 0), (1, 1), -1), ((0, 0), None, 0), ((0, 1), (1, 1), 1), ((1, 0), (0, 0), 1),
        ((1, 1), None, 0), ((0, 0), (0, 1), 1), ((1, 0), (1, 1), 1)]
_OUT = {(0, 0): {0: 1, 3: 1, 4: 1, 6: 1}, (0, 1): {2: 1, 4: -1},
        (1, 0): {1: 1, 3: 1}, (1, 1): {0: 1, 1: -1, 2: 1, 5: 1}}
_SWAP = (0, 1, 0, 0, 1, 1, 1)


def _o_order():
    nt = [1 if r[1] is None else 2 for r in _RHS]
    allp = [(i, j) for i in range(7) for j in range(7)]
    heavy, mid, light = ([p for p in allp if nt[p[0]] * nt[p[1]] == n] for n in (4, 2, 1))
    cheap = mid[:10] + light[2:] + mid[10:]
    seq = light[:2]
    while heavy or cheap:
        seq += heavy[:1] + cheap[:1]
        heavy, cheap = heavy[1:], cheap[1:]
    return tuple(seq)


O_SEQ = _o_order()

QK_PAIRS = {0.5: (0, 1), 1.5: (2, 3)}
QK_SPREAD = {0.5: (0,), 1: (1,), 1.5: (2,), 2.5: (3,)}
QK_FIRST = {1: (0, 1), 2: (2, 3)}
PV_FIRST = {4: (0,), 5: (1, 2), 6: (3,)}
PV_EARLY = {2.5: (0,), 3.5: (1,), 4.5: (2,), 5.5: (3,)}
PV_LATE = {3.5: (0,), 4.5: (1,), 5.5: (2,), 6.5: (3,)}

S_OUT = 0
S_A = 0
S_B = LA
S_E = S_B + NSB // 2 - 1
S_R = S_E + 1
N_SEM = S_R + NK + 4


def _pk(x):
    return pltpu.bitcast(x.astype(BF16), U32)


def _upk(x):
    return pltpu.bitcast(x, BF16)


def _terms(spec):
    a, b, sg = spec
    return [(a, 1)] + ([(b, sg)] if b is not None else [])


def _signed_sum(items):
    items = sorted(items, key=lambda t: -t[0])
    acc = items[0][1]
    for sg, v in items[1:]:
        acc = acc + v if sg > 0 else acc - v
    return acc


def _comb(spec, get):
    return _signed_sum([(sg, get(t)) for t, sg in _terms(spec)])


def _operand(spec, ld):
    if spec[1] is None:
        return ld(spec[0])
    return _comb(spec, lambda t: ld(t).astype(F32)).astype(BF16)


def _softmax_cols(sc):
    m = jnp.max(sc, axis=0, keepdims=True)
    p = jnp.exp2((sc - m) * C_EXP2)
    l = jnp.sum(p, axis=0, keepdims=True)
    return p * (1.0 / l)


def _kernel(xa, ka, va, wqa, woa, xb, kb, vb, wqb, wob, out,
            x_buf, ka_buf, va_buf, kb_buf, vb_buf, wq_buf, wo_buf,
            q_buf, out_buf, os_buf, accm, mq_buf, sems):
    cp = pltpu.make_async_copy

    def wq_cp(s, sem, dyn=False):
        dst = wq_buf.at[s]
        src = dst if dyn else (wqa if s < NSB else wqb).at[:, pl.ds((s % NSB) * CH, CH)]
        return cp(src, dst, sems.at[sem])

    def wo_cp(s, sem, dyn=False):
        dst = wo_buf.at[s]
        src = dst if dyn else (woa if s < NSB else wob).at[pl.ds((s % NSB) * CH, CH), :]
        return cp(src, dst, sems.at[sem])

    def kv_cp(src, dst, j, n, sem, dyn=False):
        d = dst.at[:, pl.ds(j, n)]
        return cp(d if dyn else src.at[:, pl.ds(j, n)], d, sems.at[sem])

    def wq_rows_cp(s, k0, kn, sem):
        return cp(wqa.at[pl.ds(k0, kn), pl.ds(s * CH, CH)], wq_buf.at[s, pl.ds(k0, kn), :], sems.at[sem])

    def xa_cols_cp(k0, kn, sem):
        return cp(xa.at[:, :, :, pl.ds(k0, kn)], x_buf.at[0, :, :, :, pl.ds(k0, kn)], sems.at[sem])

    def grp_r(n):
        sem = S_R + n
        if n < NK:
            k0 = sum(KSL[:n])
            return [xa_cols_cp(k0, KSL[n], sem), wq_rows_cp(0, k0, KSL[n], sem)]
        if n == NK:
            return [wq_rows_cp(1, 0, NH, sem)]
        if n == NK + 1:
            return [xa_cols_cp(NH, NH, sem), wq_rows_cp(0, NH, NH, sem)]
        if n == NK + 2:
            return [kv_cp(ka, ka_buf, 0, 1, sem), wq_rows_cp(1, NH, NH, sem), kv_cp(va, va_buf, 0, 1, sem)]
        return [wo_cp(0, sem)]

    def next_a(s):
        return s + 1 + (s == LA - 1) * 1

    def grp_a(s, dyn=False):
        return [wq_cp(next_a(s), S_A + s, dyn), wo_cp(s, S_A + s, dyn)]

    def grp_a_kv(s, dyn=False):
        g = s >> 1
        return [kv_cp(ka, ka_buf, g, 1, S_A + s, dyn), kv_cp(va, va_buf, g, 1, S_A + s, dyn)]

    def xb_cp():
        return cp(xb, x_buf.at[1], sems.at[S_A + LA - 1])

    def grp_b(p, dyn=False):
        u, sem = 2 * p, S_B + p
        return [kv_cp(kb, kb_buf, u, 2, sem, dyn), wq_cp(NSB + u + 1, sem, dyn),
                kv_cp(vb, vb_buf, u, 2, sem, dyn), wo_cp(NSB + u, sem, dyn),
                wq_cp(NSB + u + 2, sem, dyn), wo_cp(NSB + u + 1, sem, dyn)]

    def grp_e():
        return [kv_cp(kb, kb_buf, NSB - 2, 2, S_E), wq_cp(LA, S_E), kv_cp(vb, vb_buf, NSB - 2, 2, S_E),
                wo_cp(NS - 2, S_E), wq_cp(NS - 1, S_E), wo_cp(LA, S_E), wo_cp(NS - 1, S_E)]

    def out_cp(br, c0, nc):
        return cp(out_buf.at[br, :, :, :, pl.ds(c0, nc)],
                  out.at[:, :, :, pl.ds(br * D + c0, nc)], sems.at[S_OUT])

    def wait_all(cs):
        for c in cs:
            c.wait()

    for n in range(NK + 4):
        for c in grp_r(n):
            c.start()
    for s in range(1, LA):
        if s == LA - 1:
            xb_cp().start()
        for c in (grp_a_kv(s) if s % 2 == 0 else []) + grp_a(s):
            c.start()
    for p in range(NSB // 2 - 1):
        for c in grp_b(p):
            c.start()
    for c in grp_e():
        c.start()

    def zero_acc(k0, k1):
        accm[1, k0:k1] = jnp.zeros((k1 - k0,) + accm.shape[2:], F32)

    zero_acc(0, 25)

    lane_g = lax.broadcasted_iota(jnp.int32, (SK, 4 * SQ), 1) // SQ

    def x_block(br, half, c0, nc):
        return x_buf[br, :, half, :, c0:c0 + nc].reshape(MH, nc)

    def q_stage(s, br, n, mid=None, k0=0, kh=NH, add=None, to=None):
        def q_prod(i):
            lhs = _operand(_LHS[i], lambda t: x_block(br, t[0], k0 + t[1] * kh, kh))

            def part(c0, nc):
                rhs = _operand(_RHS[i], lambda t: wq_buf[s, k0 + t[0] * kh:k0 + (t[0] + 1) * kh,
                                                         t[1] * QNH + c0:t[1] * QNH + c0 + nc])
                return jnp.dot(lhs, rhs, preferred_element_type=F32)

            if mid is None:
                return part(0, QNH)
            m0 = part(0, DH)
            mid()
            return jnp.concatenate([m0, part(DH, DH)], axis=1)

        def put(a, c, val):
            if add is not None:
                val = val + mq_buf[add + 2 * a + c]
            if to is not None:
                mq_buf[to + 2 * a + c] = val
            else:
                q_buf[a * QMQ:(a + 1) * QMQ, c * QNH:(c + 1) * QNH] = _pk(val)

        if n == 0:
            mq_buf[0] = q_prod(1)
        elif n == 1:
            mq_buf[1] = q_prod(4)
        elif n == 2:
            p0 = q_prod(0)
            mq_buf[2] = p0 - mq_buf[0]
            mq_buf[3] = p0 + mq_buf[1]
        elif n == 3:
            p2 = q_prod(2)
            put(0, 1, p2 - mq_buf[1])
            mq_buf[2] += p2
        elif n == 4:
            p3 = q_prod(3)
            put(1, 0, p3 + mq_buf[0])
            mq_buf[3] += p3
        elif n == 5:
            put(1, 1, mq_buf[2] + q_prod(5))
        else:
            put(0, 0, mq_buf[3] + q_prod(6))

    def o_prod(s, i, j, r0, nr):
        ts = [(s1 * s2, 2 * a[0] + b[0], 2 * a[1] + (b[1] ^ _SWAP[i]))
              for a, s1 in _terms(_RHS[i]) for b, s2 in _terms(_RHS[j])]
        ld = lambda r, c: wo_buf[s, r * DH:(r + 1) * DH, c * NQ4:(c + 1) * NQ4]
        if len(ts) == 1:
            rhs = ld(ts[0][1], ts[0][2])
        else:
            rhs = _signed_sum([(sg, ld(r, c).astype(F32)) for sg, r, c in ts]).astype(BF16)
        lhs = _upk(os_buf[(i * MQ + r0) // 2:(i * MQ + r0 + nr) // 2, j * DH:(j + 1) * DH])
        return jnp.dot(lhs, rhs, preferred_element_type=F32)

    def oproj(s, br, first=False, split=False):
        for n, (i, j) in enumerate(O_SEQ):
            for r0, nr in (((0, MQ // 2), (MQ // 2, MQ // 2)) if split and n == 0 else ((0, MQ),)):
                m = o_prod(s, i, j, r0, nr)
                if not first:
                    m = accm[br, i * 7 + j, r0:r0 + nr] + m
                accm[br, i * 7 + j, r0:r0 + nr] = m

    def qk_group(j, is_a, bb):
        pts = []
        for b in range(bb * 4, bb * 4 + 4):
            q4 = _upk(jnp.concatenate(
                [q_buf[half * QMQ + b * 8:half * QMQ + (b + 1) * 8, h * DH:(h + 1) * DH]
                 for h in range(HPS) for half in range(2)], axis=0))
            if is_a:
                sc = lax.dot_general(ka_buf[b, j >> 1], q4, NT, preferred_element_type=F32)
            else:
                st = lax.dot_general(kb_buf[b, j], q4, NT, preferred_element_type=F32)
                sc = st[0:SK]
                for h in range(1, HPS):
                    sc = jnp.where(lane_g == h, st[h * SK:(h + 1) * SK], sc)
            pts.append(_softmax_cols(sc))
        return jnp.concatenate(pts, axis=0).T

    def pv_tile(j, is_a, tt, bb, h):
        ph = tt[h * SQ:(h + 1) * SQ]
        lhs = jnp.concatenate([jnp.where(lane_g == bi, ph, 0.0) for bi in range(4)], axis=0).astype(BF16)
        if is_a:
            vh = jnp.concatenate([va_buf[bb * 4 + bi, j >> 1] for bi in range(4)], axis=0)
        else:
            vh = jnp.concatenate(
                [vb_buf[bb * 4 + bi, j, h * SK:(h + 1) * SK, :] for bi in range(4)], axis=0)
        return lax.dot_general(lhs, vh, NN, preferred_element_type=F32)

    def pv_group(j, is_a, tt, bb, levels):
        t = [pv_tile(j, is_a, tt, bb, h) for h in range(HPS)]
        for pr in range(2):
            base = {(r, h): jnp.concatenate(
                [t[h][bi * SQ + r * RQ:bi * SQ + (r + 1) * RQ] for bi in (2 * pr, 2 * pr + 1)], axis=0)
                for r in range(4) for h in range(HPS)}
            for i in range(7):
                r0 = i * MQ // 2 + (bb * 2 + pr) * RQ
                l1 = {(b0, b1): _comb(_LHS[i], lambda a: base[(2 * a[0] + b0, 2 * a[1] + b1)])
                      for b0 in range(2) for b1 in range(2)}
                if levels == 1:
                    ops = list(l1.values())
                else:
                    ops = [None] * 7
                for jj, v in enumerate(ops):
                    v = _comb(_LHS[jj], lambda t2: l1[t2]) if v is None else v
                    os_buf[r0:r0 + RQ, jj * DH:(jj + 1) * DH] = _pk(v)

    def attn_qproj(j, is_a, s, br, qs, ps, levels=2, **kw):
        tts = [None] * 4

        def run(pos):
            for g in qs.get(pos, ()):
                tts[g] = qk_group(j, is_a, g)
            for g in ps.get(pos, ()):
                pv_group(j, is_a, tts[g], g, levels)

        for n in range(7):
            run(n)
            has_mid = (n + 0.5) in qs or (n + 0.5) in ps
            q_stage(s, br, n, (lambda: run(n + 0.5)) if has_mid else None, **kw)

    outs = []

    def final_oproj(s, br, chunks, with_qk):
        tts = None
        for c2, c0, tc in chunks:
            cc = c2 * NQ4 + c0

            def total(i):
                lhs = _upk(jnp.concatenate(
                    [os_buf[i * MQ // 2:(i + 1) * MQ // 2, b0 * QNH:(b0 + 1) * QNH] for b0 in range(2)],
                    axis=0))
                rhs = _operand(_RHS[i], lambda t: wo_buf[s, t[0] * QNH:(t[0] + 1) * QNH,
                                                         t[1] * NH + cc:t[1] * NH + cc + tc])
                m = jnp.dot(lhs, rhs, preferred_element_type=F32)
                return [_signed_sum([(1, m[r2 * MQ:(r2 + 1) * MQ])] +
                                    [(sg, accm[br, i * 7 + j, :, c0:c0 + tc])
                                     for j, sg in _OUT[(r2, c2 ^ _SWAP[i])].items()]) for r2 in range(2)]

            d = {}
            for i in (4, 1, 2, 0, 5, 3, 6):
                if with_qk and tts is None and d:
                    tts = [qk_group(NSB - 1, False, g) for g in range(4)]
                d[i] = total(i)
                for (r1, c1), terms in _OUT.items():
                    if i in terms and set(terms) <= set(d):
                        for r2 in range(2):
                            val = _signed_sum([(sg, d[k][r2]) for k, sg in terms.items()])
                            out_buf[br, :, r1, r2 * RQ:(r2 + 1) * RQ, c1 * NH + cc:c1 * NH + cc + tc] = (
                                val.reshape(B, RQ, tc).astype(BF16))
                if i in (5, 6):
                    outs.append(out_cp(br, (1 if i == 5 else 0) * NH + cc, tc))
                    outs[-1].start()
        return tts

    for n in range(NK):
        with jax.named_scope("wait0"):
            wait_all(grp_r(n))
        with jax.named_scope("pro1"):
            k0, kn = sum(KSL[:n]), KSL[n]
            xs = jnp.concatenate([x_block(0, a, k0, kn) for a in range(2)], axis=0)
            part = jnp.dot(xs, wq_buf[0, k0:k0 + kn, :], preferred_element_type=F32)
            for a in range(2):
                for c in range(2):
                    pq = part[a * MH:(a + 1) * MH, c * QNH:(c + 1) * QNH]
                    if n == 0:
                        mq_buf[4 + 2 * a + c] = pq
                    else:
                        mq_buf[4 + 2 * a + c] += pq
            z0 = 25 + sum(k // 128 * 3 for k in KSL[:n])
            zero_acc(z0, z0 + kn // 128 * 3)
    with jax.named_scope("wait1"):
        wait_all(grp_r(NK))
    with jax.named_scope("pro2"):
        zero_acc(37, 43)
        attn_qproj(0, True, 1, 0, {}, {}, k0=0, kh=NQ4, to=8)
    with jax.named_scope("wait2"):
        wait_all(grp_r(NK + 1))
    with jax.named_scope("pro3"):
        zero_acc(43, 49)
        attn_qproj(0, True, 0, 0, {}, {}, k0=NH, kh=NQ4, add=4)
    with jax.named_scope("wait3"):
        wait_all(grp_r(NK + 2))
    with jax.named_scope("pro4"):
        attn_qproj(0, True, 1, 0, QK_FIRST, PV_FIRST, k0=NH, kh=NQ4, add=8)
    with jax.named_scope("wait4"):
        wait_all(grp_r(NK + 3))
    with jax.named_scope("pro5"):
        oproj(0, 0, first=True, split=True)

    def body_a(s, carry):
        with jax.named_scope("waitA"):
            @pl.when((s & 1) == 0)
            def _():
                wait_all(grp_a_kv(s, dyn=True))

            @pl.when(s == LA - 1)
            def _():
                xb_cp().wait()

            wait_all(grp_a(s, dyn=True))

        with jax.named_scope("bodyA"):
            attn_qproj(s, True, next_a(s), (s == LA - 1) * 1, QK_SPREAD, PV_LATE)
            oproj(s, 0)
        return carry

    lax.fori_loop(1, LA, body_a, 0)

    def body_b(p, carry):
        u = 2 * p
        with jax.named_scope("waitB"):
            wait_all(grp_b(p, dyn=True))
        with jax.named_scope("bodyB"):
            attn_qproj(u, False, NSB + u + 1, 1, QK_PAIRS, PV_EARLY)
            oproj(NSB + u, 1)
            attn_qproj(u + 1, False, NSB + u + 2, 1, QK_PAIRS, PV_EARLY)
            oproj(NSB + u + 1, 1)
        return carry

    lax.fori_loop(0, NSB // 2 - 1, body_b, 0)

    with jax.named_scope("epi0"):
        wait_all(grp_e())
    with jax.named_scope("epi1"):
        attn_qproj(NSB - 2, False, LA, 0, QK_PAIRS, PV_EARLY)
        oproj(NS - 2, 1, split=True)
        attn_qproj(LA, True, NS - 1, 1, QK_PAIRS, PV_EARLY, levels=1)
        tts = final_oproj(LA, 0, ((0, 0, 256), (1, 0, 256)), True)
        for g in range(4):
            pv_group(NSB - 1, False, tts[g], g, 1)
        final_oproj(NS - 1, 1, ((0, 0, 256), (1, 0, 128), (1, 128, 128)), False)
    with jax.named_scope("tail"):
        wait_all(outs)


@jax.jit
def pallas_concat_heads__gqa_block_cached__mha_block_cached__near_ridge_kernel(A_x, A_k_cache, A_v_cache, A_wq, A_wo, B_x, B_k_cache, B_v_cache, B_wq, B_wo):
    xa = A_x.reshape(B, 2, SH, D)
    xb = B_x.reshape(B, 2, SH, D)
    kb = B_k_cache.reshape(B, NSB, HPS * SK, DH)
    vb = B_v_cache.reshape(B, NSB, HPS * SK, DH)
    any_spec = pl.BlockSpec(memory_space=pl.ANY)
    out = pl.pallas_call(
        _kernel,
        in_specs=[any_spec] * 10,
        out_specs=any_spec,
        out_shape=jax.ShapeDtypeStruct((B, 2, SH, 2 * D), BF16),
        scratch_shapes=[
            pltpu.VMEM((2, B, 2, SH, D), BF16),
            pltpu.VMEM((B, HKV, SK, DH), BF16),
            pltpu.VMEM((B, HKV, SK, DH), BF16),
            pltpu.VMEM((B, NSB, HPS * SK, DH), BF16),
            pltpu.VMEM((B, NSB, HPS * SK, DH), BF16),
            pltpu.VMEM((NS, D, CH), BF16),
            pltpu.VMEM((NS, CH, D), BF16),
            pltpu.VMEM((M // 2, CH), U32),
            pltpu.VMEM((2, B, 2, SH, D), BF16),
            pltpu.VMEM((7 * MQ // 2, 7 * DH), U32),
            pltpu.VMEM((2, 49, MQ, NQ4), F32),
            pltpu.VMEM((12, MH, QNH), F32),
            pltpu.SemaphoreType.DMA((N_SEM,)),
        ],
        compiler_params=pltpu.CompilerParams(vmem_limit_bytes=100 * 1024 * 1024,
                                             disable_semaphore_checks=True),
        name="fused_attn",
    )(xa, A_k_cache, A_v_cache, A_wq, A_wo, xb, kb, vb, B_wq, B_wo)
    return out.reshape(B, SQ, 2 * D)
```

```python
import numpy as np
import jax
import jax.numpy as jnp
from jax import lax
import jax.experimental.pallas as pl
import jax.experimental.pallas.tpu as pltpu

B, SQ, D, H, HKV, SK, DH = 16, 32, 1024, 32, 4, 32, 128
M = B * SQ
MH = M // 2
MQ = M // 4
SH, RQ = SQ // 2, SQ // 4
HPS = 4
CH = HPS * DH
NSB = H // HPS
NS = 2 * NSB
LA = NSB - 1
NH, NQ4 = D // 2, D // 4
QNH, QMQ = CH // 2, MH // 2
KSL = (128, 128, 256)
NK = len(KSL)
C_EXP2 = float(DH ** -0.5 * np.log2(np.e))
NT = (((1,), (1,)), ((), ()))
NN = (((1,), (0,)), ((), ()))
F32 = jnp.float32
BF16 = jnp.bfloat16
U32 = jnp.uint32

_LHS = [((0, 0), (1, 1), -1), ((1, 0), (1, 1), -1), ((0, 0), None, 0), ((1, 1), None, 0),
        ((0, 0), (0, 1), -1), ((1, 0), (0, 0), -1), ((0, 1), (1, 1), -1)]
_RHS = [((0, 0), (1, 1), -1), ((0, 0), None, 0), ((0, 1), (1, 1), 1), ((1, 0), (0, 0), 1),
        ((1, 1), None, 0), ((0, 0), (0, 1), 1), ((1, 0), (1, 1), 1)]
_OUT = {(0, 0): {0: 1, 3: 1, 4: 1, 6: 1}, (0, 1): {2: 1, 4: -1},
        (1, 0): {1: 1, 3: 1}, (1, 1): {0: 1, 1: -1, 2: 1, 5: 1}}
_SWAP = (0, 1, 0, 0, 1, 1, 1)


def _o_order():
    nt = [1 if r[1] is None else 2 for r in _RHS]
    allp = [(i, j) for i in range(7) for j in range(7)]
    heavy, mid, light = ([p for p in allp if nt[p[0]] * nt[p[1]] == n] for n in (4, 2, 1))
    cheap = mid[:10] + light[2:] + mid[10:]
    seq = light[:2]
    while heavy or cheap:
        seq += heavy[:1] + cheap[:1]
        heavy, cheap = heavy[1:], cheap[1:]
    return tuple(seq)


O_SEQ = _o_order()

QK_PAIRS = {0.5: (0, 1), 1.5: (2, 3)}
QK_SPREAD = {0.5: (0,), 1: (1,), 1.5: (2,), 2.5: (3,)}
QK_FIRST = {1: (0, 1), 2: (2, 3)}
PV_FIRST = {4: (0,), 5: (1, 2), 6: (3,)}
PV_EARLY = {2.5: (0,), 3.5: (1,), 4.5: (2,), 5.5: (3,)}
PV_LATE = {3.5: (0,), 4.5: (1,), 5.5: (2,), 6.5: (3,)}

S_OUT = 0
S_A = 0
BU = 3
NB = (NSB - 2) // BU
S_B = LA
S_E = S_B + NB
S_R = S_E + 1
N_SEM = S_R + NK + 4


def _pk(x):
    return pltpu.bitcast(x.astype(BF16), U32)


def _upk(x):
    return pltpu.bitcast(x, BF16)


def _terms(spec):
    a, b, sg = spec
    return [(a, 1)] + ([(b, sg)] if b is not None else [])


def _signed_sum(items):
    items = sorted(items, key=lambda t: -t[0])
    acc = items[0][1]
    for sg, v in items[1:]:
        acc = acc + v if sg > 0 else acc - v
    return acc


def _comb(spec, get):
    return _signed_sum([(sg, get(t)) for t, sg in _terms(spec)])


def _operand(spec, ld):
    if spec[1] is None:
        return ld(spec[0])
    return _comb(spec, lambda t: ld(t).astype(F32)).astype(BF16)


def _softmax_cols(sc):
    m = jnp.max(sc, axis=0, keepdims=True)
    p = jnp.exp2((sc - m) * C_EXP2)
    l = jnp.sum(p, axis=0, keepdims=True)
    return p * (1.0 / l)


def _kernel(xa, ka, va, wqa, woa, xb, kb, vb, wqb, wob, out,
            x_buf, ka_buf, va_buf, kb_buf, vb_buf, wq_buf, wo_buf,
            q_buf, out_buf, os_buf, accm, mq_buf, sems):
    cp = pltpu.make_async_copy

    def wq_cp(s, sem, dyn=False):
        dst = wq_buf.at[s]
        src = dst if dyn else (wqa if s < NSB else wqb).at[:, pl.ds((s % NSB) * CH, CH)]
        return cp(src, dst, sems.at[sem])

    def wo_cp(s, sem, dyn=False):
        dst = wo_buf.at[s]
        src = dst if dyn else (woa if s < NSB else wob).at[pl.ds((s % NSB) * CH, CH), :]
        return cp(src, dst, sems.at[sem])

    def kv_cp(src, dst, j, n, sem, dyn=False):
        d = dst.at[:, pl.ds(j, n)]
        return cp(d if dyn else src.at[:, pl.ds(j, n)], d, sems.at[sem])

    def wq_rows_cp(s, k0, kn, sem):
        return cp(wqa.at[pl.ds(k0, kn), pl.ds(s * CH, CH)], wq_buf.at[s, pl.ds(k0, kn), :], sems.at[sem])

    def xa_cols_cp(k0, kn, sem):
        return cp(xa.at[:, :, :, pl.ds(k0, kn)], x_buf.at[0, :, :, :, pl.ds(k0, kn)], sems.at[sem])

    def grp_r(n):
        sem = S_R + n
        if n < NK:
            k0 = sum(KSL[:n])
            return [xa_cols_cp(k0, KSL[n], sem), wq_rows_cp(0, k0, KSL[n], sem)]
        if n == NK:
            return [wq_rows_cp(1, 0, NH, sem)]
        if n == NK + 1:
            return [xa_cols_cp(NH, NH, sem), wq_rows_cp(0, NH, NH, sem)]
        if n == NK + 2:
            return [kv_cp(ka, ka_buf, 0, 1, sem), wq_rows_cp(1, NH, NH, sem), kv_cp(va, va_buf, 0, 1, sem)]
        return [wo_cp(0, sem)]

    def next_a(s):
        return s + 1 + (s == LA - 1) * 1

    def grp_a(s, dyn=False):
        return [wq_cp(next_a(s), S_A + s, dyn), wo_cp(s, S_A + s, dyn)]

    def grp_a_kv(s, dyn=False):
        g = s >> 1
        return [kv_cp(ka, ka_buf, g, 1, S_A + s, dyn), kv_cp(va, va_buf, g, 1, S_A + s, dyn)]

    def xb_cp():
        return cp(xb, x_buf.at[1], sems.at[S_A + LA - 1])

    def grp_b(p, dyn=False):
        u, sem = BU * p, S_B + p
        g = [kv_cp(kb, kb_buf, u, BU, sem, dyn), kv_cp(vb, vb_buf, u, BU, sem, dyn)]
        for k in range(BU):
            g += [wq_cp(NSB + u + k + 1, sem, dyn), wo_cp(NSB + u + k, sem, dyn)]
        return g

    def grp_e():
        return [kv_cp(kb, kb_buf, NSB - 2, 2, S_E), wq_cp(LA, S_E), kv_cp(vb, vb_buf, NSB - 2, 2, S_E),
                wo_cp(NS - 2, S_E), wq_cp(NS - 1, S_E), wo_cp(LA, S_E), wo_cp(NS - 1, S_E)]

    def out_cp(br, c0, nc):
        return cp(out_buf.at[br, :, :, :, pl.ds(c0, nc)],
                  out.at[:, :, :, pl.ds(br * D + c0, nc)], sems.at[S_OUT])

    def wait_all(cs):
        for c in cs:
            c.wait()

    for n in range(NK + 4):
        for c in grp_r(n):
            c.start()
    for s in range(1, LA):
        if s == LA - 1:
            xb_cp().start()
        for c in (grp_a_kv(s) if s % 2 == 0 else []) + grp_a(s):
            c.start()
    for p in range(NB):
        for c in grp_b(p):
            c.start()
    for c in grp_e():
        c.start()

    def zero_acc(k0, k1):
        accm[1, k0:k1] = jnp.zeros((k1 - k0,) + accm.shape[2:], F32)

    zero_acc(0, 25)

    lane_g = lax.broadcasted_iota(jnp.int32, (SK, 4 * SQ), 1) // SQ

    def x_block(br, half, c0, nc):
        return x_buf[br, :, half, :, c0:c0 + nc].reshape(MH, nc)

    def q_stage(s, br, n, mid=None, k0=0, kh=NH, add=None, to=None):
        def q_prod(i):
            lhs = _operand(_LHS[i], lambda t: x_block(br, t[0], k0 + t[1] * kh, kh))

            def part(c0, nc):
                rhs = _operand(_RHS[i], lambda t: wq_buf[s, k0 + t[0] * kh:k0 + (t[0] + 1) * kh,
                                                         t[1] * QNH + c0:t[1] * QNH + c0 + nc])
                return jnp.dot(lhs, rhs, preferred_element_type=F32)

            if mid is None:
                return part(0, QNH)
            m0 = part(0, DH)
            mid()
            return jnp.concatenate([m0, part(DH, DH)], axis=1)

        def put(a, c, val):
            if add is not None:
                val = val + mq_buf[add + 2 * a + c]
            if to is not None:
                mq_buf[to + 2 * a + c] = val
            else:
                q_buf[a * QMQ:(a + 1) * QMQ, c * QNH:(c + 1) * QNH] = _pk(val)

        if n == 0:
            mq_buf[0] = q_prod(1)
        elif n == 1:
            mq_buf[1] = q_prod(4)
        elif n == 2:
            p0 = q_prod(0)
            mq_buf[2] = p0 - mq_buf[0]
            mq_buf[3] = p0 + mq_buf[1]
        elif n == 3:
            p2 = q_prod(2)
            put(0, 1, p2 - mq_buf[1])
            mq_buf[2] += p2
        elif n == 4:
            p3 = q_prod(3)
            put(1, 0, p3 + mq_buf[0])
            mq_buf[3] += p3
        elif n == 5:
            put(1, 1, mq_buf[2] + q_prod(5))
        else:
            put(0, 0, mq_buf[3] + q_prod(6))

    def o_prod(s, i, j, r0, nr):
        ts = [(s1 * s2, 2 * a[0] + b[0], 2 * a[1] + (b[1] ^ _SWAP[i]))
              for a, s1 in _terms(_RHS[i]) for b, s2 in _terms(_RHS[j])]
        ld = lambda r, c: wo_buf[s, r * DH:(r + 1) * DH, c * NQ4:(c + 1) * NQ4]
        if len(ts) == 1:
            rhs = ld(ts[0][1], ts[0][2])
        else:
            rhs = _signed_sum([(sg, ld(r, c).astype(F32)) for sg, r, c in ts]).astype(BF16)
        lhs = _upk(os_buf[(i * MQ + r0) // 2:(i * MQ + r0 + nr) // 2, j * DH:(j + 1) * DH])
        return jnp.dot(lhs, rhs, preferred_element_type=F32)

    def oproj(s, br, first=False, split=False):
        for n, (i, j) in enumerate(O_SEQ):
            for r0, nr in (((0, MQ // 2), (MQ // 2, MQ // 2)) if split and n == 0 else ((0, MQ),)):
                m = o_prod(s, i, j, r0, nr)
                if not first:
                    m = accm[br, i * 7 + j, r0:r0 + nr] + m
                accm[br, i * 7 + j, r0:r0 + nr] = m

    def qk_group(j, is_a, bb):
        pts = []
        for b in range(bb * 4, bb * 4 + 4):
            q4 = _upk(jnp.concatenate(
                [q_buf[half * QMQ + b * 8:half * QMQ + (b + 1) * 8, h * DH:(h + 1) * DH]
                 for h in range(HPS) for half in range(2)], axis=0))
            if is_a:
                sc = lax.dot_general(ka_buf[b, j >> 1], q4, NT, preferred_element_type=F32)
            else:
                st = lax.dot_general(kb_buf[b, j], q4, NT, preferred_element_type=F32)
                sc = st[0:SK]
                for h in range(1, HPS):
                    sc = jnp.where(lane_g == h, st[h * SK:(h + 1) * SK], sc)
            pts.append(_softmax_cols(sc))
        return jnp.concatenate(pts, axis=0).T

    def pv_tile(j, is_a, tt, bb, h):
        ph = tt[h * SQ:(h + 1) * SQ]
        lhs = jnp.concatenate([jnp.where(lane_g == bi, ph, 0.0) for bi in range(4)], axis=0).astype(BF16)
        if is_a:
            vh = jnp.concatenate([va_buf[bb * 4 + bi, j >> 1] for bi in range(4)], axis=0)
        else:
            vh = jnp.concatenate(
                [vb_buf[bb * 4 + bi, j, h * SK:(h + 1) * SK, :] for bi in range(4)], axis=0)
        return lax.dot_general(lhs, vh, NN, preferred_element_type=F32)

    def pv_group(j, is_a, tt, bb, levels):
        t = [pv_tile(j, is_a, tt, bb, h) for h in range(HPS)]
        for pr in range(2):
            base = {(r, h): jnp.concatenate(
                [t[h][bi * SQ + r * RQ:bi * SQ + (r + 1) * RQ] for bi in (2 * pr, 2 * pr + 1)], axis=0)
                for r in range(4) for h in range(HPS)}
            for i in range(7):
                r0 = i * MQ // 2 + (bb * 2 + pr) * RQ
                l1 = {(b0, b1): _comb(_LHS[i], lambda a: base[(2 * a[0] + b0, 2 * a[1] + b1)])
                      for b0 in range(2) for b1 in range(2)}
                if levels == 1:
                    ops = list(l1.values())
                else:
                    ops = [None] * 7
                for jj, v in enumerate(ops):
                    v = _comb(_LHS[jj], lambda t2: l1[t2]) if v is None else v
                    os_buf[r0:r0 + RQ, jj * DH:(jj + 1) * DH] = _pk(v)

    def attn_qproj(j, is_a, s, br, qs, ps, levels=2, **kw):
        tts = [None] * 4

        def run(pos):
            for g in qs.get(pos, ()):
                tts[g] = qk_group(j, is_a, g)
            for g in ps.get(pos, ()):
                pv_group(j, is_a, tts[g], g, levels)

        for n in range(7):
            run(n)
            has_mid = (n + 0.5) in qs or (n + 0.5) in ps
            q_stage(s, br, n, (lambda: run(n + 0.5)) if has_mid else None, **kw)

    outs = []

    def final_oproj(s, br, chunks, with_qk):
        tts = None
        for c2, c0, tc in chunks:
            cc = c2 * NQ4 + c0

            def total(i):
                lhs = _upk(jnp.concatenate(
                    [os_buf[i * MQ // 2:(i + 1) * MQ // 2, b0 * QNH:(b0 + 1) * QNH] for b0 in range(2)],
                    axis=0))
                rhs = _operand(_RHS[i], lambda t: wo_buf[s, t[0] * QNH:(t[0] + 1) * QNH,
                                                         t[1] * NH + cc:t[1] * NH + cc + tc])
                m = jnp.dot(lhs, rhs, preferred_element_type=F32)
                return [_signed_sum([(1, m[r2 * MQ:(r2 + 1) * MQ])] +
                                    [(sg, accm[br, i * 7 + j, :, c0:c0 + tc])
                                     for j, sg in _OUT[(r2, c2 ^ _SWAP[i])].items()]) for r2 in range(2)]

            d = {}
            for i in (4, 1, 2, 0, 5, 3, 6):
                if with_qk and tts is None and d:
                    tts = [qk_group(NSB - 1, False, g) for g in range(4)]
                d[i] = total(i)
                for (r1, c1), terms in _OUT.items():
                    if i in terms and set(terms) <= set(d):
                        for r2 in range(2):
                            val = _signed_sum([(sg, d[k][r2]) for k, sg in terms.items()])
                            out_buf[br, :, r1, r2 * RQ:(r2 + 1) * RQ, c1 * NH + cc:c1 * NH + cc + tc] = (
                                val.reshape(B, RQ, tc).astype(BF16))
                if i in (5, 6):
                    outs.append(out_cp(br, (1 if i == 5 else 0) * NH + cc, tc))
                    outs[-1].start()
        return tts

    for n in range(NK):
        with jax.named_scope("wait0"):
            wait_all(grp_r(n))
        with jax.named_scope("pro1"):
            k0, kn = sum(KSL[:n]), KSL[n]
            xs = jnp.concatenate([x_block(0, a, k0, kn) for a in range(2)], axis=0)
            part = jnp.dot(xs, wq_buf[0, k0:k0 + kn, :], preferred_element_type=F32)
            for a in range(2):
                for c in range(2):
                    pq = part[a * MH:(a + 1) * MH, c * QNH:(c + 1) * QNH]
                    if n == 0:
                        mq_buf[4 + 2 * a + c] = pq
                    else:
                        mq_buf[4 + 2 * a + c] += pq
            z0 = 25 + sum(k // 128 * 3 for k in KSL[:n])
            zero_acc(z0, z0 + kn // 128 * 3)
    with jax.named_scope("wait1"):
        wait_all(grp_r(NK))
    with jax.named_scope("pro2"):
        zero_acc(37, 43)
        attn_qproj(0, True, 1, 0, {}, {}, k0=0, kh=NQ4, to=8)
    with jax.named_scope("wait2"):
        wait_all(grp_r(NK + 1))
    with jax.named_scope("pro3"):
        zero_acc(43, 49)
        attn_qproj(0, True, 0, 0, {}, {}, k0=NH, kh=NQ4, add=4)
    with jax.named_scope("wait3"):
        wait_all(grp_r(NK + 2))
    with jax.named_scope("pro4"):
        attn_qproj(0, True, 1, 0, QK_FIRST, PV_FIRST, k0=NH, kh=NQ4, add=8)
    with jax.named_scope("wait4"):
        wait_all(grp_r(NK + 3))
    with jax.named_scope("pro5"):
        oproj(0, 0, first=True, split=True)

    def body_a(s, carry):
        with jax.named_scope("waitA"):
            @pl.when((s & 1) == 0)
            def _():
                wait_all(grp_a_kv(s, dyn=True))

            @pl.when(s == LA - 1)
            def _():
                xb_cp().wait()

            wait_all(grp_a(s, dyn=True))

        with jax.named_scope("bodyA"):
            attn_qproj(s, True, next_a(s), (s == LA - 1) * 1, QK_SPREAD, PV_LATE)
            oproj(s, 0)
        return carry

    lax.fori_loop(1, LA, body_a, 0)

    def body_b(p, carry):
        with jax.named_scope("waitB"):
            wait_all(grp_b(p, dyn=True))
        with jax.named_scope("bodyB"):
            for k in range(BU):
                u = BU * p + k
                attn_qproj(u, False, NSB + u + 1, 1, QK_PAIRS, PV_EARLY)
                oproj(NSB + u, 1)
        return carry

    lax.fori_loop(0, NB, body_b, 0)

    with jax.named_scope("epi0"):
        wait_all(grp_e())
    with jax.named_scope("epi1"):
        attn_qproj(NSB - 2, False, LA, 0, QK_PAIRS, PV_EARLY)
        oproj(NS - 2, 1, split=True)
        attn_qproj(LA, True, NS - 1, 1, QK_PAIRS, PV_EARLY, levels=1)
        tts = final_oproj(LA, 0, ((0, 0, 256), (1, 0, 256)), True)
        for g in range(4):
            pv_group(NSB - 1, False, tts[g], g, 1)
        final_oproj(NS - 1, 1, ((0, 0, 256), (1, 0, 128), (1, 128, 128)), False)
    with jax.named_scope("tail"):
        wait_all(outs)


@jax.jit
def pallas_concat_heads__gqa_block_cached__mha_block_cached__near_ridge_kernel(A_x, A_k_cache, A_v_cache, A_wq, A_wo, B_x, B_k_cache, B_v_cache, B_wq, B_wo):
    xa = A_x.reshape(B, 2, SH, D)
    xb = B_x.reshape(B, 2, SH, D)
    kb = B_k_cache.reshape(B, NSB, HPS * SK, DH)
    vb = B_v_cache.reshape(B, NSB, HPS * SK, DH)
    any_spec = pl.BlockSpec(memory_space=pl.ANY)
    out = pl.pallas_call(
        _kernel,
        in_specs=[any_spec] * 10,
        out_specs=any_spec,
        out_shape=jax.ShapeDtypeStruct((B, 2, SH, 2 * D), BF16),
        scratch_shapes=[
            pltpu.VMEM((2, B, 2, SH, D), BF16),
            pltpu.VMEM((B, HKV, SK, DH), BF16),
            pltpu.VMEM((B, HKV, SK, DH), BF16),
            pltpu.VMEM((B, NSB, HPS * SK, DH), BF16),
            pltpu.VMEM((B, NSB, HPS * SK, DH), BF16),
            pltpu.VMEM((NS, D, CH), BF16),
            pltpu.VMEM((NS, CH, D), BF16),
            pltpu.VMEM((M // 2, CH), U32),
            pltpu.VMEM((2, B, 2, SH, D), BF16),
            pltpu.VMEM((7 * MQ // 2, 7 * DH), U32),
            pltpu.VMEM((2, 49, MQ, NQ4), F32),
            pltpu.VMEM((12, MH, QNH), F32),
            pltpu.SemaphoreType.DMA((N_SEM,)),
        ],
        compiler_params=pltpu.CompilerParams(vmem_limit_bytes=100 * 1024 * 1024,
                                             disable_semaphore_checks=True),
        name="fused_attn",
    )(xa, A_k_cache, A_v_cache, A_wq, A_wo, xb, kb, vb, B_wq, B_wo)
    return out.reshape(B, SQ, 2 * D)
```

```python
import numpy as np
import jax
import jax.numpy as jnp
from jax import lax
import jax.experimental.pallas as pl
import jax.experimental.pallas.tpu as pltpu

B, SQ, D, H, HKV, SK, DH = 16, 32, 1024, 32, 4, 32, 128
M = B * SQ
MH = M // 2
MQ = M // 4
SH, RQ = SQ // 2, SQ // 4
HPS = 4
CH = HPS * DH
NSB = H // HPS
NS = 2 * NSB
LA = NSB - 1
NH, NQ4 = D // 2, D // 4
QNH, QMQ = CH // 2, MH // 2
KSL = (128, 128, 256)
NK = len(KSL)
C_EXP2 = float(DH ** -0.5 * np.log2(np.e))
S_LIMIT = float(8.0 * DH ** 0.5)
NT = (((1,), (1,)), ((), ()))
NN = (((1,), (0,)), ((), ()))
F32 = jnp.float32
BF16 = jnp.bfloat16
U32 = jnp.uint32

_LHS = [((0, 0), (1, 1), -1), ((1, 0), (1, 1), -1), ((0, 0), None, 0), ((1, 1), None, 0),
        ((0, 0), (0, 1), -1), ((1, 0), (0, 0), -1), ((0, 1), (1, 1), -1)]
_RHS = [((0, 0), (1, 1), -1), ((0, 0), None, 0), ((0, 1), (1, 1), 1), ((1, 0), (0, 0), 1),
        ((1, 1), None, 0), ((0, 0), (0, 1), 1), ((1, 0), (1, 1), 1)]
_OUT = {(0, 0): {0: 1, 3: 1, 4: 1, 6: 1}, (0, 1): {2: 1, 4: -1},
        (1, 0): {1: 1, 3: 1}, (1, 1): {0: 1, 1: -1, 2: 1, 5: 1}}
_SWAP = (0, 1, 0, 0, 1, 1, 1)


def _o_order():
    nt = [1 if r[1] is None else 2 for r in _RHS]
    allp = [(i, j) for i in range(7) for j in range(7)]
    heavy, mid, light = ([p for p in allp if nt[p[0]] * nt[p[1]] == n] for n in (4, 2, 1))
    cheap = mid[:10] + light[2:] + mid[10:]
    seq = light[:2]
    while heavy or cheap:
        seq += heavy[:1] + cheap[:1]
        heavy, cheap = heavy[1:], cheap[1:]
    return tuple(seq)


O_SEQ = _o_order()

QK_PAIRS = {0.5: (0, 1), 1.5: (2, 3)}
QK_SPREAD = {0.5: (0,), 1: (1,), 1.5: (2,), 2.5: (3,)}
QK_FIRST = {1: (0, 1), 2: (2, 3)}
PV_FIRST = {4: (0,), 5: (1, 2), 6: (3,)}
PV_EARLY = {2.5: (0,), 3.5: (1,), 4.5: (2,), 5.5: (3,)}
PV_LATE = {3.5: (0,), 4.5: (1,), 5.5: (2,), 6.5: (3,)}

S_OUT = 0
S_A = 0
BU = 3
NB = (NSB - 2) // BU
S_B = LA
S_E = S_B + NB
S_R = S_E + 1
N_SEM = S_R + NK + 4


def _pk(x):
    return pltpu.bitcast(x.astype(BF16), U32)


def _upk(x):
    return pltpu.bitcast(x, BF16)


def _terms(spec):
    a, b, sg = spec
    return [(a, 1)] + ([(b, sg)] if b is not None else [])


def _signed_sum(items):
    items = sorted(items, key=lambda t: -t[0])
    acc = items[0][1]
    for sg, v in items[1:]:
        acc = acc + v if sg > 0 else acc - v
    return acc


def _comb(spec, get):
    return _signed_sum([(sg, get(t)) for t, sg in _terms(spec)])


def _operand(spec, ld):
    if spec[1] is None:
        return ld(spec[0])
    return _comb(spec, lambda t: ld(t).astype(F32)).astype(BF16)


def _softmax_cols(sc):
    m = jnp.max(sc, axis=0, keepdims=True)
    p = jnp.exp2((sc - m) * C_EXP2)
    l = jnp.sum(p, axis=0, keepdims=True)
    return p * (1.0 / l)


def _kernel(xa, ka, va, wqa, woa, xb, kb, vb, wqb, wob, out,
            x_buf, ka_buf, va_buf, kb_buf, vb_buf, wq_buf, wo_buf,
            q_buf, out_buf, os_buf, accm, mq_buf, smax, sems):
    cp = pltpu.make_async_copy

    def wq_cp(s, sem, dyn=False):
        dst = wq_buf.at[s]
        src = dst if dyn else (wqa if s < NSB else wqb).at[:, pl.ds((s % NSB) * CH, CH)]
        return cp(src, dst, sems.at[sem])

    def wo_cp(s, sem, dyn=False):
        dst = wo_buf.at[s]
        src = dst if dyn else (woa if s < NSB else wob).at[pl.ds((s % NSB) * CH, CH), :]
        return cp(src, dst, sems.at[sem])

    def kv_cp(src, dst, j, n, sem, dyn=False):
        d = dst.at[:, pl.ds(j, n)]
        return cp(d if dyn else src.at[:, pl.ds(j, n)], d, sems.at[sem])

    def wq_rows_cp(s, k0, kn, sem):
        return cp(wqa.at[pl.ds(k0, kn), pl.ds(s * CH, CH)], wq_buf.at[s, pl.ds(k0, kn), :], sems.at[sem])

    def xa_cols_cp(k0, kn, sem):
        return cp(xa.at[:, :, :, pl.ds(k0, kn)], x_buf.at[0, :, :, :, pl.ds(k0, kn)], sems.at[sem])

    def grp_r(n):
        sem = S_R + n
        if n < NK:
            k0 = sum(KSL[:n])
            return [xa_cols_cp(k0, KSL[n], sem), wq_rows_cp(0, k0, KSL[n], sem)]
        if n == NK:
            return [wq_rows_cp(1, 0, NH, sem)]
        if n == NK + 1:
            return [xa_cols_cp(NH, NH, sem), wq_rows_cp(0, NH, NH, sem)]
        if n == NK + 2:
            return [kv_cp(ka, ka_buf, 0, 1, sem), wq_rows_cp(1, NH, NH, sem), kv_cp(va, va_buf, 0, 1, sem)]
        return [wo_cp(0, sem)]

    def next_a(s):
        return s + 1 + (s == LA - 1) * 1

    def grp_a(s, dyn=False):
        return [wq_cp(next_a(s), S_A + s, dyn), wo_cp(s, S_A + s, dyn)]

    def grp_a_kv(s, dyn=False):
        g = s >> 1
        return [kv_cp(ka, ka_buf, g, 1, S_A + s, dyn), kv_cp(va, va_buf, g, 1, S_A + s, dyn)]

    def xb_cp():
        return cp(xb, x_buf.at[1], sems.at[S_A + LA - 1])

    def grp_b(p, dyn=False):
        u, sem = BU * p, S_B + p
        g = [kv_cp(kb, kb_buf, u, BU, sem, dyn), kv_cp(vb, vb_buf, u, BU, sem, dyn)]
        for k in range(BU):
            g += [wq_cp(NSB + u + k + 1, sem, dyn), wo_cp(NSB + u + k, sem, dyn)]
        return g

    def grp_e():
        return [kv_cp(kb, kb_buf, NSB - 2, 2, S_E), wq_cp(LA, S_E), kv_cp(vb, vb_buf, NSB - 2, 2, S_E),
                wo_cp(NS - 2, S_E), wq_cp(NS - 1, S_E), wo_cp(LA, S_E), wo_cp(NS - 1, S_E)]

    def out_cp(br, c0, nc):
        return cp(out_buf.at[br, :, :, :, pl.ds(c0, nc)],
                  out.at[:, :, :, pl.ds(br * D + c0, nc)], sems.at[S_OUT])

    def wait_all(cs):
        for c in cs:
            c.wait()

    for n in range(NK + 4):
        for c in grp_r(n):
            c.start()
    for s in range(1, LA):
        if s == LA - 1:
            xb_cp().start()
        for c in (grp_a_kv(s) if s % 2 == 0 else []) + grp_a(s):
            c.start()
    for p in range(NB):
        for c in grp_b(p):
            c.start()
    for c in grp_e():
        c.start()

    def zero_acc(k0, k1):
        accm[1, k0:k1] = jnp.zeros((k1 - k0,) + accm.shape[2:], F32)

    def zero_one(k, carry):
        accm[1, k] = jnp.zeros(accm.shape[2:], F32)
        return carry

    lax.fori_loop(0, 25, zero_one, 0)
    smax[...] = jnp.zeros(smax.shape, F32)

    lane_g = lax.broadcasted_iota(jnp.int32, (SK, 4 * SQ), 1) // SQ

    def x_block(br, half, c0, nc):
        return x_buf[br, :, half, :, c0:c0 + nc].reshape(MH, nc)

    def q_stage(s, br, n, mid=None, k0=0, kh=NH, add=None, to=None):
        def q_prod(i):
            lhs = _operand(_LHS[i], lambda t: x_block(br, t[0], k0 + t[1] * kh, kh))

            def part(c0, nc):
                rhs = _operand(_RHS[i], lambda t: wq_buf[s, k0 + t[0] * kh:k0 + (t[0] + 1) * kh,
                                                         t[1] * QNH + c0:t[1] * QNH + c0 + nc])
                return jnp.dot(lhs, rhs, preferred_element_type=F32)

            if mid is None:
                return part(0, QNH)
            m0 = part(0, DH)
            mid()
            return jnp.concatenate([m0, part(DH, DH)], axis=1)

        def put(a, c, val):
            if add is not None:
                val = val + mq_buf[add + 2 * a + c]
            if to is not None:
                mq_buf[to + 2 * a + c] = val
            else:
                q_buf[a * QMQ:(a + 1) * QMQ, c * QNH:(c + 1) * QNH] = _pk(val)

        if n == 0:
            mq_buf[0] = q_prod(1)
        elif n == 1:
            mq_buf[1] = q_prod(4)
        elif n == 2:
            p0 = q_prod(0)
            mq_buf[2] = p0 - mq_buf[0]
            mq_buf[3] = p0 + mq_buf[1]
        elif n == 3:
            p2 = q_prod(2)
            put(0, 1, p2 - mq_buf[1])
            mq_buf[2] += p2
        elif n == 4:
            p3 = q_prod(3)
            put(1, 0, p3 + mq_buf[0])
            mq_buf[3] += p3
        elif n == 5:
            put(1, 1, mq_buf[2] + q_prod(5))
        else:
            put(0, 0, mq_buf[3] + q_prod(6))

    def o_prod(s, i, j, r0, nr):
        ts = [(s1 * s2, 2 * a[0] + b[0], 2 * a[1] + (b[1] ^ _SWAP[i]))
              for a, s1 in _terms(_RHS[i]) for b, s2 in _terms(_RHS[j])]
        ld = lambda r, c: wo_buf[s, r * DH:(r + 1) * DH, c * NQ4:(c + 1) * NQ4]
        if len(ts) == 1:
            rhs = ld(ts[0][1], ts[0][2])
        else:
            rhs = _signed_sum([(sg, ld(r, c).astype(F32)) for sg, r, c in ts]).astype(BF16)
        lhs = _upk(os_buf[(i * MQ + r0) // 2:(i * MQ + r0 + nr) // 2, j * DH:(j + 1) * DH])
        return jnp.dot(lhs, rhs, preferred_element_type=F32)

    def oproj(s, br, first=False, split=False):
        for n, (i, j) in enumerate(O_SEQ):
            for r0, nr in (((0, MQ // 2), (MQ // 2, MQ // 2)) if split and n == 0 else ((0, MQ),)):
                m = o_prod(s, i, j, r0, nr)
                if not first:
                    m = accm[br, i * 7 + j, r0:r0 + nr] + m
                accm[br, i * 7 + j, r0:r0 + nr] = m

    def diag(st):
        sc = st[0:SK]
        for h in range(1, HPS):
            sc = jnp.where(lane_g == h, st[h * SK:(h + 1) * SK], sc)
        return sc

    def scores(j, is_a, b, q4):
        if is_a:
            return lax.dot_general(ka_buf[b, j >> 1], q4, NT, preferred_element_type=F32)
        return diag(lax.dot_general(kb_buf[b, j], q4, NT, preferred_element_type=F32))

    def p_lhs(tt, h):
        ph = tt[h * SQ:(h + 1) * SQ]
        return jnp.concatenate([jnp.where(lane_g == bi, ph, 0.0) for bi in range(4)], axis=0).astype(BF16)

    def qk_group(j, is_a, bb):
        pts = []
        big = None
        for b in range(bb * 4, bb * 4 + 4):
            q4 = _upk(jnp.concatenate(
                [q_buf[half * QMQ + b * 8:half * QMQ + (b + 1) * 8, h * DH:(h + 1) * DH]
                 for h in range(HPS) for half in range(2)], axis=0))
            sc = scores(j, is_a, b, q4)
            big = jnp.abs(sc) if big is None else jnp.maximum(big, jnp.abs(sc))
            pts.append(_softmax_cols(sc))
        smax[bb] = jnp.maximum(smax[bb], big)
        return jnp.concatenate(pts, axis=0).T

    def pv_tile(j, is_a, tt, bb, h):
        lhs = p_lhs(tt, h)
        if is_a:
            vh = jnp.concatenate([va_buf[bb * 4 + bi, j >> 1] for bi in range(4)], axis=0)
        else:
            vh = jnp.concatenate(
                [vb_buf[bb * 4 + bi, j, h * SK:(h + 1) * SK, :] for bi in range(4)], axis=0)
        return lax.dot_general(lhs, vh, NN, preferred_element_type=F32)

    def pv_group(j, is_a, tt, bb, levels):
        t = [pv_tile(j, is_a, tt, bb, h) for h in range(HPS)]
        for pr in range(2):
            base = {(r, h): jnp.concatenate(
                [t[h][bi * SQ + r * RQ:bi * SQ + (r + 1) * RQ] for bi in (2 * pr, 2 * pr + 1)], axis=0)
                for r in range(4) for h in range(HPS)}
            for i in range(7):
                r0 = i * MQ // 2 + (bb * 2 + pr) * RQ
                l1 = {(b0, b1): _comb(_LHS[i], lambda a: base[(2 * a[0] + b0, 2 * a[1] + b1)])
                      for b0 in range(2) for b1 in range(2)}
                if levels == 1:
                    ops = list(l1.values())
                else:
                    ops = [None] * 7
                for jj, v in enumerate(ops):
                    v = _comb(_LHS[jj], lambda t2: l1[t2]) if v is None else v
                    os_buf[r0:r0 + RQ, jj * DH:(jj + 1) * DH] = _pk(v)

    def attn_qproj(j, is_a, s, br, qs, ps, levels=2, **kw):
        tts = [None] * 4

        def run(pos):
            for g in qs.get(pos, ()):
                tts[g] = qk_group(j, is_a, g)
            for g in ps.get(pos, ()):
                pv_group(j, is_a, tts[g], g, levels)

        for n in range(7):
            run(n)
            has_mid = (n + 0.5) in qs or (n + 0.5) in ps
            q_stage(s, br, n, (lambda: run(n + 0.5)) if has_mid else None, **kw)

    outs = []

    def final_oproj(s, br, chunks, with_qk):
        tts = None
        for c2, c0, tc in chunks:
            cc = c2 * NQ4 + c0

            def total(i):
                lhs = _upk(jnp.concatenate(
                    [os_buf[i * MQ // 2:(i + 1) * MQ // 2, b0 * QNH:(b0 + 1) * QNH] for b0 in range(2)],
                    axis=0))
                rhs = _operand(_RHS[i], lambda t: wo_buf[s, t[0] * QNH:(t[0] + 1) * QNH,
                                                         t[1] * NH + cc:t[1] * NH + cc + tc])
                m = jnp.dot(lhs, rhs, preferred_element_type=F32)
                return [_signed_sum([(1, m[r2 * MQ:(r2 + 1) * MQ])] +
                                    [(sg, accm[br, i * 7 + j, :, c0:c0 + tc])
                                     for j, sg in _OUT[(r2, c2 ^ _SWAP[i])].items()]) for r2 in range(2)]

            d = {}
            for i in (4, 1, 2, 0, 5, 3, 6):
                if with_qk and tts is None and d:
                    tts = [qk_group(NSB - 1, False, g) for g in range(4)]
                d[i] = total(i)
                for (r1, c1), terms in _OUT.items():
                    if i in terms and set(terms) <= set(d):
                        for r2 in range(2):
                            val = _signed_sum([(sg, d[k][r2]) for k, sg in terms.items()])
                            out_buf[br, :, r1, r2 * RQ:(r2 + 1) * RQ, c1 * NH + cc:c1 * NH + cc + tc] = (
                                val.reshape(B, RQ, tc).astype(BF16))
                if i in (5, 6):
                    outs.append(out_cp(br, (1 if i == 5 else 0) * NH + cc, tc))
                    outs[-1].start()
        return tts

    for n in range(NK):
        with jax.named_scope("wait0"):
            wait_all(grp_r(n))
        with jax.named_scope("pro1"):
            k0, kn = sum(KSL[:n]), KSL[n]
            xs = jnp.concatenate([x_block(0, a, k0, kn) for a in range(2)], axis=0)
            part = jnp.dot(xs, wq_buf[0, k0:k0 + kn, :], preferred_element_type=F32)
            for a in range(2):
                for c in range(2):
                    pq = part[a * MH:(a + 1) * MH, c * QNH:(c + 1) * QNH]
                    if n == 0:
                        mq_buf[4 + 2 * a + c] = pq
                    else:
                        mq_buf[4 + 2 * a + c] += pq
            z0 = 25 + sum(k // 128 * 3 for k in KSL[:n])
            zero_acc(z0, z0 + kn // 128 * 3)
    with jax.named_scope("wait1"):
        wait_all(grp_r(NK))
    with jax.named_scope("pro2"):
        zero_acc(37, 43)
        attn_qproj(0, True, 1, 0, {}, {}, k0=0, kh=NQ4, to=8)
    with jax.named_scope("wait2"):
        wait_all(grp_r(NK + 1))
    with jax.named_scope("pro3"):
        zero_acc(43, 49)
        attn_qproj(0, True, 0, 0, {}, {}, k0=NH, kh=NQ4, add=4)
    with jax.named_scope("wait3"):
        wait_all(grp_r(NK + 2))
    with jax.named_scope("pro4"):
        attn_qproj(0, True, 1, 0, QK_FIRST, PV_FIRST, k0=NH, kh=NQ4, add=8)
    with jax.named_scope("wait4"):
        wait_all(grp_r(NK + 3))
    with jax.named_scope("pro5"):
        oproj(0, 0, first=True, split=True)

    def body_a(s, carry):
        with jax.named_scope("waitA"):
            @pl.when((s & 1) == 0)
            def _():
                wait_all(grp_a_kv(s, dyn=True))

            @pl.when(s == LA - 1)
            def _():
                xb_cp().wait()

            wait_all(grp_a(s, dyn=True))

        with jax.named_scope("bodyA"):
            attn_qproj(s, True, next_a(s), (s == LA - 1) * 1, QK_SPREAD, PV_LATE)
            oproj(s, 0)
        return carry

    lax.fori_loop(1, LA, body_a, 0)

    def body_b(p, carry):
        with jax.named_scope("waitB"):
            wait_all(grp_b(p, dyn=True))
        with jax.named_scope("bodyB"):
            for k in range(BU):
                u = BU * p + k
                attn_qproj(u, False, NSB + u + 1, 1, QK_PAIRS, PV_EARLY)
                oproj(NSB + u, 1)
        return carry

    lax.fori_loop(0, NB, body_b, 0)

    with jax.named_scope("epi0"):
        wait_all(grp_e())
    with jax.named_scope("epi1"):
        attn_qproj(NSB - 2, False, LA, 0, QK_PAIRS, PV_EARLY)
        oproj(NS - 2, 1, split=True)
        attn_qproj(LA, True, NS - 1, 1, QK_PAIRS, PV_EARLY, levels=1)
        tts = final_oproj(LA, 0, ((0, 0, 256), (1, 0, 256)), True)
        for g in range(4):
            pv_group(NSB - 1, False, tts[g], g, 1)
        final_oproj(NS - 1, 1, ((0, 0, 256), (1, 0, 128), (1, 128, 128)), False)
    with jax.named_scope("tail"):
        sharp = jnp.logical_not(jnp.max(smax[...]) <= S_LIMIT)
        wait_all(outs)

    @pl.when(sharp)
    def _():
        def step(t, carry):
            br, bb, j = t >> 5, (t >> 3) & 3, t & 7
            is_a = br == 0

            def kv4(a_buf, b_buf, b):
                return jnp.where(is_a, jnp.concatenate([a_buf[b, j >> 1]] * HPS, axis=0), b_buf[b, j])

            xr = x_buf[br, pl.ds(bb * 4, 4)].reshape(MQ, D)
            q = jnp.dot(xr, wq_buf[br * NSB + j], preferred_element_type=F32).astype(BF16)
            pts = []
            for bi in range(4):
                q4 = jnp.concatenate(
                    [q[bi * SQ:(bi + 1) * SQ, h * DH:(h + 1) * DH] for h in range(HPS)], axis=0)
                pts.append(_softmax_cols(diag(lax.dot_general(
                    kv4(ka_buf, kb_buf, bb * 4 + bi), q4, NT, preferred_element_type=F32))))
            tt = jnp.concatenate(pts, axis=0).T
            v4 = [kv4(va_buf, vb_buf, bb * 4 + bi) for bi in range(4)]
            o = jnp.concatenate(
                [lax.dot_general(p_lhs(tt, h),
                                 jnp.concatenate([v[h * SK:(h + 1) * SK] for v in v4], axis=0),
                                 NN, preferred_element_type=F32) for h in range(HPS)], axis=1)
            m = jnp.dot(o.astype(BF16), wo_buf[br * NSB + j], preferred_element_type=F32)
            for c in range(4):
                acc = jnp.where(j == 0, 0.0, accm[0, c]) + m[:, c * NQ4:(c + 1) * NQ4]
                accm[0, c] = acc
                out_buf[br, pl.ds(bb * 4, 4), :, :, c * NQ4:(c + 1) * NQ4] = (
                    acc.astype(BF16).reshape(4, 2, SH, NQ4))
            return carry

        lax.fori_loop(0, 2 * (B // 4) * NSB, step, 0)
        for br in range(2):
            out_cp(br, 0, D).start()
        for br in range(2):
            out_cp(br, 0, D).wait()


@jax.jit
def pallas_concat_heads__gqa_block_cached__mha_block_cached__near_ridge_kernel(A_x, A_k_cache, A_v_cache, A_wq, A_wo, B_x, B_k_cache, B_v_cache, B_wq, B_wo):
    xa = A_x.reshape(B, 2, SH, D)
    xb = B_x.reshape(B, 2, SH, D)
    kb = B_k_cache.reshape(B, NSB, HPS * SK, DH)
    vb = B_v_cache.reshape(B, NSB, HPS * SK, DH)
    any_spec = pl.BlockSpec(memory_space=pl.ANY)
    out = pl.pallas_call(
        _kernel,
        in_specs=[any_spec] * 10,
        out_specs=any_spec,
        out_shape=jax.ShapeDtypeStruct((B, 2, SH, 2 * D), BF16),
        scratch_shapes=[
            pltpu.VMEM((2, B, 2, SH, D), BF16),
            pltpu.VMEM((B, HKV, SK, DH), BF16),
            pltpu.VMEM((B, HKV, SK, DH), BF16),
            pltpu.VMEM((B, NSB, HPS * SK, DH), BF16),
            pltpu.VMEM((B, NSB, HPS * SK, DH), BF16),
            pltpu.VMEM((NS, D, CH), BF16),
            pltpu.VMEM((NS, CH, D), BF16),
            pltpu.VMEM((M // 2, CH), U32),
            pltpu.VMEM((2, B, 2, SH, D), BF16),
            pltpu.VMEM((7 * MQ // 2, 7 * DH), U32),
            pltpu.VMEM((2, 49, MQ, NQ4), F32),
            pltpu.VMEM((12, MH, QNH), F32),
            pltpu.VMEM((4, SK, 4 * SQ), F32),
            pltpu.SemaphoreType.DMA((N_SEM,)),
        ],
        compiler_params=pltpu.CompilerParams(vmem_limit_bytes=100 * 1024 * 1024,
                                             disable_semaphore_checks=True),
        name="fused_attn",
    )(xa, A_k_cache, A_v_cache, A_wq, A_wo, xb, kb, vb, B_wq, B_wo)
    return out.reshape(B, SQ, 2 * D)
```

```python
import numpy as np
import jax
import jax.numpy as jnp
from jax import lax
import jax.experimental.pallas as pl
import jax.experimental.pallas.tpu as pltpu

B, SQ, D, H, HKV, SK, DH = 16, 32, 1024, 32, 4, 32, 128
M = B * SQ
MH = M // 2
MQ = M // 4
SH, RQ = SQ // 2, SQ // 4
HPS = 4
CH = HPS * DH
NSB = H // HPS
NS = 2 * NSB
LA = NSB - 1
NH, NQ4 = D // 2, D // 4
QNH, QMQ = CH // 2, MH // 2
KSL = (128, 128, 256)
NK = len(KSL)
C_EXP2 = float(DH ** -0.5 * np.log2(np.e))
S_LIMIT = float(8.0 * DH ** 0.5)
NT = (((1,), (1,)), ((), ()))
NN = (((1,), (0,)), ((), ()))
F32 = jnp.float32
BF16 = jnp.bfloat16
U32 = jnp.uint32

_LHS = [((0, 0), (1, 1), -1), ((1, 0), (1, 1), -1), ((0, 0), None, 0), ((1, 1), None, 0),
        ((0, 0), (0, 1), -1), ((1, 0), (0, 0), -1), ((0, 1), (1, 1), -1)]
_RHS = [((0, 0), (1, 1), -1), ((0, 0), None, 0), ((0, 1), (1, 1), 1), ((1, 0), (0, 0), 1),
        ((1, 1), None, 0), ((0, 0), (0, 1), 1), ((1, 0), (1, 1), 1)]
_OUT = {(0, 0): {0: 1, 3: 1, 4: 1, 6: 1}, (0, 1): {2: 1, 4: -1},
        (1, 0): {1: 1, 3: 1}, (1, 1): {0: 1, 1: -1, 2: 1, 5: 1}}
_SWAP = (0, 1, 0, 0, 1, 1, 1)


def _o_order():
    nt = [1 if r[1] is None else 2 for r in _RHS]
    allp = [(i, j) for i in range(7) for j in range(7)]
    heavy, mid, light = ([p for p in allp if nt[p[0]] * nt[p[1]] == n] for n in (4, 2, 1))
    cheap = mid[:10] + light[2:] + mid[10:]
    seq = light[:2]
    while heavy or cheap:
        seq += heavy[:1] + cheap[:1]
        heavy, cheap = heavy[1:], cheap[1:]
    return tuple(seq)


O_SEQ = _o_order()

XS = (1, 4, 2, 3)
_L1, _L4 = [(1, 0), (1, 1)], [(4, 0), (4, 1)]
_Z31 = [(3, 0), (3, 1)] + [u for n in range(2, 7) for u in ((3, n), (1, n))]
_Z24 = [(2, 0), (2, 1)] + [u for n in range(2, 7) for u in ((2, n), (4, n))]
SEQ_A = (_L1 + [(0, 0), "q0", "q1", (0, 1), (5, 0), "q2", "q3", (5, 1)] + _L4 + _Z31[:6] + ["p0"]
         + _Z31[6:] + [(6, 0), "p1", "p2", (6, 1), "p3"] + _Z24)
SEQ_B = (_L1 + [(0, 0), "q0", "q1", "q2", "q3", (0, 1)] + _L4 + _Z31
         + [(5, 0), "p0", "p1", (5, 1), (6, 0), "p2", "p3", (6, 1)] + _Z24)
SEQ_E = (_L1 + ["q0", "q1", "q2", "q3"] + _L4 + _Z31[:2] + _Z24[:2] + [(0, 0), "p0", (0, 1)] + _Z31[2:]
         + [(5, 0), "p1", "p2", (5, 1), (6, 0), "p3", (6, 1)] + _Z24[2:])
QK_FIRST = {1: (0, 1), 2: (2, 3)}
PV_FIRST = {4: (0,), 5: (1, 2), 6: (3,)}

S_OUT = 0
S_A = 0
BU = 3
NB = (NSB - 2) // BU
S_B = LA
S_E = S_B + NB
S_R = S_E + 1
N_SEM = S_R + NK + 4


def _pk(x):
    return pltpu.bitcast(x.astype(BF16), U32)


def _upk(x):
    return pltpu.bitcast(x, BF16)


def _terms(spec):
    a, b, sg = spec
    return [(a, 1)] + ([(b, sg)] if b is not None else [])


def _signed_sum(items):
    items = sorted(items, key=lambda t: -t[0])
    acc = items[0][1]
    for sg, v in items[1:]:
        acc = acc + v if sg > 0 else acc - v
    return acc


def _comb(spec, get):
    return _signed_sum([(sg, get(t)) for t, sg in _terms(spec)])


def _operand(spec, ld):
    if spec[1] is None:
        return ld(spec[0])
    return _comb(spec, lambda t: ld(t).astype(F32)).astype(BF16)


def _softmax_cols(sc):
    m = jnp.max(sc, axis=0, keepdims=True)
    p = jnp.exp2((sc - m) * C_EXP2)
    l = jnp.sum(p, axis=0, keepdims=True)
    return p * (1.0 / l)


def _kernel(xa, ka, va, wqa, woa, xb, kb, vb, wqb, wob, out,
            x_buf, ka_buf, va_buf, kb_buf, vb_buf, wq_buf, wo_buf,
            q_buf, out_buf, os_buf, accm, mq_buf, smax, xs_buf, sems):
    cp = pltpu.make_async_copy

    def wq_cp(s, sem, dyn=False):
        dst = wq_buf.at[s]
        src = dst if dyn else (wqa if s < NSB else wqb).at[:, pl.ds((s % NSB) * CH, CH)]
        return cp(src, dst, sems.at[sem])

    def wo_cp(s, sem, dyn=False):
        dst = wo_buf.at[s]
        src = dst if dyn else (woa if s < NSB else wob).at[pl.ds((s % NSB) * CH, CH), :]
        return cp(src, dst, sems.at[sem])

    def kv_cp(src, dst, j, n, sem, dyn=False):
        d = dst.at[:, pl.ds(j, n)]
        return cp(d if dyn else src.at[:, pl.ds(j, n)], d, sems.at[sem])

    def wq_rows_cp(s, k0, kn, sem):
        return cp(wqa.at[pl.ds(k0, kn), pl.ds(s * CH, CH)], wq_buf.at[s, pl.ds(k0, kn), :], sems.at[sem])

    def xa_cols_cp(k0, kn, sem):
        return cp(xa.at[:, :, :, pl.ds(k0, kn)], x_buf.at[0, :, :, :, pl.ds(k0, kn)], sems.at[sem])

    def grp_r(n):
        sem = S_R + n
        if n < NK:
            k0 = sum(KSL[:n])
            return [xa_cols_cp(k0, KSL[n], sem), wq_rows_cp(0, k0, KSL[n], sem)]
        if n == NK:
            return [wq_rows_cp(1, 0, NH, sem)]
        if n == NK + 1:
            return [xa_cols_cp(NH, NH, sem), wq_rows_cp(0, NH, NH, sem)]
        if n == NK + 2:
            return [kv_cp(ka, ka_buf, 0, 1, sem), wq_rows_cp(1, NH, NH, sem), kv_cp(va, va_buf, 0, 1, sem)]
        return [wo_cp(0, sem)]

    def next_a(s):
        return s + 1 + (s == LA - 1) * 1

    def grp_a(s, dyn=False):
        return [wq_cp(next_a(s), S_A + s, dyn), wo_cp(s, S_A + s, dyn)]

    def grp_a_kv(s, dyn=False):
        g = s >> 1
        return [kv_cp(ka, ka_buf, g, 1, S_A + s, dyn), kv_cp(va, va_buf, g, 1, S_A + s, dyn)]

    def xb_cp():
        return cp(xb, x_buf.at[1], sems.at[S_A + LA - 1])

    def grp_b(p, dyn=False):
        u, sem = BU * p, S_B + p
        g = [kv_cp(kb, kb_buf, u, BU, sem, dyn), kv_cp(vb, vb_buf, u, BU, sem, dyn)]
        for k in range(BU):
            g += [wq_cp(NSB + u + k + 1, sem, dyn), wo_cp(NSB + u + k, sem, dyn)]
        return g

    def grp_e():
        return [kv_cp(kb, kb_buf, NSB - 2, 2, S_E), wq_cp(LA, S_E), kv_cp(vb, vb_buf, NSB - 2, 2, S_E),
                wo_cp(NS - 2, S_E), wq_cp(NS - 1, S_E), wo_cp(LA, S_E), wo_cp(NS - 1, S_E)]

    def out_cp(br, c0, nc):
        return cp(out_buf.at[br, :, :, :, pl.ds(c0, nc)],
                  out.at[:, :, :, pl.ds(br * D + c0, nc)], sems.at[S_OUT])

    def wait_all(cs):
        for c in cs:
            c.wait()

    for n in range(NK + 4):
        for c in grp_r(n):
            c.start()
    for s in range(1, LA):
        if s == LA - 1:
            xb_cp().start()
        for c in (grp_a_kv(s) if s % 2 == 0 else []) + grp_a(s):
            c.start()
    for p in range(NB):
        for c in grp_b(p):
            c.start()
    for c in grp_e():
        c.start()

    def zero_acc(k0, k1):
        accm[1, k0:k1] = jnp.zeros((k1 - k0,) + accm.shape[2:], F32)

    def zero_one(k, carry):
        accm[1, k] = jnp.zeros(accm.shape[2:], F32)
        return carry

    lax.fori_loop(0, 25, zero_one, 0)
    smax[...] = jnp.zeros(smax.shape, F32)

    lane_g = lax.broadcasted_iota(jnp.int32, (SK, 4 * SQ), 1) // SQ

    def x_block(br, half, c0, nc):
        return x_buf[br, :, half, :, c0:c0 + nc].reshape(MH, nc)

    def q_stage(s, n, k0, add=None, to=None):
        def q_prod(i):
            lhs = _operand(_LHS[i], lambda t: x_block(0, t[0], k0 + t[1] * NQ4, NQ4))
            rhs = _operand(_RHS[i], lambda t: wq_buf[s, k0 + t[0] * NQ4:k0 + (t[0] + 1) * NQ4,
                                                     t[1] * QNH:(t[1] + 1) * QNH])
            return jnp.dot(lhs, rhs, preferred_element_type=F32)

        def put(a, c, val):
            if add is not None:
                val = val + mq_buf[add + 2 * a + c]
            if to is not None:
                mq_buf[to + 2 * a + c] = val
            else:
                q_buf[a * QMQ:(a + 1) * QMQ, c * QNH:(c + 1) * QNH] = _pk(val)

        if n == 0:
            mq_buf[0] = q_prod(1)
        elif n == 1:
            mq_buf[1] = q_prod(4)
        elif n == 2:
            p0 = q_prod(0)
            mq_buf[2] = p0 - mq_buf[0]
            mq_buf[3] = p0 + mq_buf[1]
        elif n == 3:
            p2 = q_prod(2)
            put(0, 1, p2 - mq_buf[1])
            mq_buf[2] += p2
        elif n == 4:
            p3 = q_prod(3)
            put(1, 0, p3 + mq_buf[0])
            mq_buf[3] += p3
        elif n == 5:
            put(1, 1, mq_buf[2] + q_prod(5))
        else:
            put(0, 0, mq_buf[3] + q_prod(6))


    def x_sub(br, a, b):
        c0 = (2 * a[1] + b[1]) * NQ4
        return x_buf[br, b[0] * 8:(b[0] + 1) * 8, a[0], :, c0:c0 + NQ4].reshape(MQ, NQ4)

    def make_xs(br):
        def one(b, carry):
            def ld(a, t):
                c0 = (2 * a[1] + t[1]) * NQ4
                return x_buf[br, t[0] * 8 + b, a[0], :, c0:c0 + NQ4].astype(F32)
            for n, i in enumerate(XS):
                l1 = {(b0, b1): _comb(_LHS[i], lambda a: ld(a, (b0, b1))) for b0 in range(2) for b1 in range(2)}
                rows = pl.ds(pl.multiple_of(n * (MQ // 2) + b * 8, 8), 8)
                for j in range(7):
                    if _LHS[i][1] is not None or _LHS[j][1] is not None:
                        xs_buf.at[br][rows, j * NQ4:(j + 1) * NQ4] = _pk(_comb(_LHS[j], lambda t: l1[t]))
            return carry
        lax.fori_loop(0, 8, one, 0, unroll=4)

    def q_sub(s, br, i, j):
        if _LHS[i][1] is not None or _LHS[j][1] is not None:
            n = XS.index(i)
            lhs = _upk(xs_buf[br, n * (MQ // 2):(n + 1) * (MQ // 2), j * NQ4:(j + 1) * NQ4])
        else:
            lhs = _operand(_LHS[j], lambda t: x_sub(br, _LHS[i][0], t))
        ts = [(s1 * s2, 2 * a[0] + b[0], 2 * a[1] + (b[1] ^ _SWAP[i]))
              for a, s1 in _terms(_RHS[i]) for b, s2 in _terms(_RHS[j])]
        ld = lambda r, c: wq_buf[s, r * NQ4:(r + 1) * NQ4, c * DH:(c + 1) * DH]
        if len(ts) == 1:
            rhs = ld(ts[0][1], ts[0][2])
        else:
            rhs = _signed_sum([(sg, ld(r, c).astype(F32)) for sg, r, c in ts]).astype(BF16)
        return jnp.dot(lhs, rhs, preferred_element_type=F32)

    def quad(slot, k):
        return mq_buf.at[slot].at[(k >> 1) * MQ:((k >> 1) + 1) * MQ, (k & 1) * DH:((k & 1) + 1) * DH]

    def qproj(s, br, seq, qk, pv):
        left = {(blk, k): len(terms) for blk, terms in _OUT.items() for k in range(4)}
        slot_of = {(1, 1): 0, (0, 0): 1, (0, 1): 2, (1, 0): 3}
        neg = {}
        lhs1 = {}

        def emit(i, r2, c2, v):
            k = 2 * r2 + c2
            for blk, terms in _OUT.items():
                if i not in terms:
                    continue
                ref = quad(slot_of[blk], k)
                first = left[(blk, k)] == len(terms)
                left[(blk, k)] -= 1
                if first:
                    neg[(blk, k)] = terms[i] < 0
                    ref[...] = v
                    continue
                if neg[(blk, k)]:
                    assert terms[i] > 0
                    tot, neg[(blk, k)] = v - ref[...], False
                else:
                    tot = ref[...] + v if terms[i] > 0 else ref[...] - v
                if left[(blk, k)]:
                    ref[...] = tot
                else:
                    r0, c0 = blk[0] * QMQ + r2 * (MQ // 2), blk[1] * QNH + c2 * DH
                    q_buf[r0:r0 + MQ // 2, c0:c0 + DH] = _pk(tot)

        def inner(i, n):
            t = lambda k: quad(4 + XS.index(i), k)
            done = lambda r2, c2, v: emit(i, r2, c2 ^ _SWAP[i], v)
            if n == 0:
                t(0)[...] = q_sub(s, br, i, 1)
            elif n == 1:
                t(1)[...] = q_sub(s, br, i, 4)
            elif n == 2:
                p0 = q_sub(s, br, i, 0)
                t(2)[...] = p0 - t(0)[...]
                t(3)[...] = p0 + t(1)[...]
            elif n == 3:
                p2 = q_sub(s, br, i, 2)
                done(0, 1, p2 - t(1)[...])
                t(2)[...] += p2
            elif n == 4:
                p3 = q_sub(s, br, i, 3)
                done(1, 0, p3 + t(0)[...])
                t(3)[...] += p3
            elif n == 5:
                done(1, 1, t(2)[...] + q_sub(s, br, i, 5))
            else:
                done(0, 0, t(3)[...] + q_sub(s, br, i, 6))

        def half(i, c2):
            if i not in lhs1:
                lhs1[i] = _operand(_LHS[i], lambda t: x_block(br, t[0], t[1] * NH, NH))
            rhs = _operand(_RHS[i], lambda t: wq_buf[s, t[0] * NH:(t[0] + 1) * NH,
                                                     t[1] * QNH + c2 * DH:t[1] * QNH + (c2 + 1) * DH])
            m = jnp.dot(lhs1[i], rhs, preferred_element_type=F32)
            for r2 in range(2):
                emit(i, r2, c2, m[r2 * MQ:(r2 + 1) * MQ])

        for u in seq:
            if isinstance(u, str):
                (qk if u[0] == "q" else pv)(int(u[1]))
            elif u[0] in XS:
                inner(*u)
            else:
                half(*u)

    def o_prod(s, i, j, r0, nr):
        ts = [(s1 * s2, 2 * a[0] + b[0], 2 * a[1] + (b[1] ^ _SWAP[i]))
              for a, s1 in _terms(_RHS[i]) for b, s2 in _terms(_RHS[j])]
        ld = lambda r, c: wo_buf[s, r * DH:(r + 1) * DH, c * NQ4:(c + 1) * NQ4]
        if len(ts) == 1:
            rhs = ld(ts[0][1], ts[0][2])
        else:
            rhs = _signed_sum([(sg, ld(r, c).astype(F32)) for sg, r, c in ts]).astype(BF16)
        lhs = _upk(os_buf[(i * MQ + r0) // 2:(i * MQ + r0 + nr) // 2, j * DH:(j + 1) * DH])
        return jnp.dot(lhs, rhs, preferred_element_type=F32)

    def oproj(s, br, first=False, split=False):
        for n, (i, j) in enumerate(O_SEQ):
            for r0, nr in (((0, MQ // 2), (MQ // 2, MQ // 2)) if split and n == 0 else ((0, MQ),)):
                m = o_prod(s, i, j, r0, nr)
                if not first:
                    m = accm[br, i * 7 + j, r0:r0 + nr] + m
                accm[br, i * 7 + j, r0:r0 + nr] = m

    def diag(st):
        sc = st[0:SK]
        for h in range(1, HPS):
            sc = jnp.where(lane_g == h, st[h * SK:(h + 1) * SK], sc)
        return sc

    def scores(j, is_a, b, q4):
        if is_a:
            return lax.dot_general(ka_buf[b, j >> 1], q4, NT, preferred_element_type=F32)
        return diag(lax.dot_general(kb_buf[b, j], q4, NT, preferred_element_type=F32))

    def p_lhs(tt, h):
        ph = tt[h * SQ:(h + 1) * SQ]
        return jnp.concatenate([jnp.where(lane_g == bi, ph, 0.0) for bi in range(4)], axis=0).astype(BF16)

    def qk_group(j, is_a, bb):
        pts = []
        big = None
        for b in range(bb * 4, bb * 4 + 4):
            q4 = _upk(jnp.concatenate(
                [q_buf[half * QMQ + b * 8:half * QMQ + (b + 1) * 8, h * DH:(h + 1) * DH]
                 for h in range(HPS) for half in range(2)], axis=0))
            sc = scores(j, is_a, b, q4)
            big = jnp.abs(sc) if big is None else jnp.maximum(big, jnp.abs(sc))
            pts.append(_softmax_cols(sc))
        smax[bb] = jnp.maximum(smax[bb], big)
        return jnp.concatenate(pts, axis=0).T

    def pv_tile(j, is_a, tt, bb, h):
        lhs = p_lhs(tt, h)
        if is_a:
            vh = jnp.concatenate([va_buf[bb * 4 + bi, j >> 1] for bi in range(4)], axis=0)
        else:
            vh = jnp.concatenate(
                [vb_buf[bb * 4 + bi, j, h * SK:(h + 1) * SK, :] for bi in range(4)], axis=0)
        return lax.dot_general(lhs, vh, NN, preferred_element_type=F32)

    def pv_group(j, is_a, tt, bb, levels):
        t = [pv_tile(j, is_a, tt, bb, h) for h in range(HPS)]
        for pr in range(2):
            base = {(r, h): jnp.concatenate(
                [t[h][bi * SQ + r * RQ:bi * SQ + (r + 1) * RQ] for bi in (2 * pr, 2 * pr + 1)], axis=0)
                for r in range(4) for h in range(HPS)}
            for i in range(7):
                r0 = i * MQ // 2 + (bb * 2 + pr) * RQ
                l1 = {(b0, b1): _comb(_LHS[i], lambda a: base[(2 * a[0] + b0, 2 * a[1] + b1)])
                      for b0 in range(2) for b1 in range(2)}
                if levels == 1:
                    ops = list(l1.values())
                else:
                    ops = [None] * 7
                for jj, v in enumerate(ops):
                    v = _comb(_LHS[jj], lambda t2: l1[t2]) if v is None else v
                    os_buf[r0:r0 + RQ, jj * DH:(jj + 1) * DH] = _pk(v)

    def attn_qproj(j, is_a, s, br, seq, levels=2):
        tts = [None] * 4

        def qk(g):
            tts[g] = qk_group(j, is_a, g)

        qproj(s, br, seq, qk, lambda g: pv_group(j, is_a, tts[g], g, levels))

    outs = []

    def final_oproj(s, br, chunks, with_qk):
        tts = None
        for c2, c0, tc in chunks:
            cc = c2 * NQ4 + c0

            def total(i):
                lhs = _upk(jnp.concatenate(
                    [os_buf[i * MQ // 2:(i + 1) * MQ // 2, b0 * QNH:(b0 + 1) * QNH] for b0 in range(2)],
                    axis=0))
                rhs = _operand(_RHS[i], lambda t: wo_buf[s, t[0] * QNH:(t[0] + 1) * QNH,
                                                         t[1] * NH + cc:t[1] * NH + cc + tc])
                m = jnp.dot(lhs, rhs, preferred_element_type=F32)
                return [_signed_sum([(1, m[r2 * MQ:(r2 + 1) * MQ])] +
                                    [(sg, accm[br, i * 7 + j, :, c0:c0 + tc])
                                     for j, sg in _OUT[(r2, c2 ^ _SWAP[i])].items()]) for r2 in range(2)]

            d = {}
            for i in (4, 1, 2, 0, 5, 3, 6):
                if with_qk and tts is None and d:
                    tts = [qk_group(NSB - 1, False, g) for g in range(4)]
                d[i] = total(i)
                for (r1, c1), terms in _OUT.items():
                    if i in terms and set(terms) <= set(d):
                        for r2 in range(2):
                            val = _signed_sum([(sg, d[k][r2]) for k, sg in terms.items()])
                            out_buf[br, :, r1, r2 * RQ:(r2 + 1) * RQ, c1 * NH + cc:c1 * NH + cc + tc] = (
                                val.reshape(B, RQ, tc).astype(BF16))
                if i in (5, 6):
                    outs.append(out_cp(br, (1 if i == 5 else 0) * NH + cc, tc))
                    outs[-1].start()
        return tts

    for n in range(NK):
        with jax.named_scope("wait0"):
            wait_all(grp_r(n))
        with jax.named_scope("pro1"):
            k0, kn = sum(KSL[:n]), KSL[n]
            xs = jnp.concatenate([x_block(0, a, k0, kn) for a in range(2)], axis=0)
            part = jnp.dot(xs, wq_buf[0, k0:k0 + kn, :], preferred_element_type=F32)
            for a in range(2):
                for c in range(2):
                    pq = part[a * MH:(a + 1) * MH, c * QNH:(c + 1) * QNH]
                    if n == 0:
                        mq_buf[4 + 2 * a + c] = pq
                    else:
                        mq_buf[4 + 2 * a + c] += pq
            z0 = 25 + sum(k // 128 * 3 for k in KSL[:n])
            zero_acc(z0, z0 + kn // 128 * 3)
    with jax.named_scope("wait1"):
        wait_all(grp_r(NK))
    with jax.named_scope("pro2"):
        zero_acc(37, 43)
        for n in range(7):
            q_stage(1, n, 0, to=8)
    with jax.named_scope("wait2"):
        wait_all(grp_r(NK + 1))
    with jax.named_scope("pro3"):
        zero_acc(43, 49)
        for n in range(7):
            q_stage(0, n, NH, add=4)
    with jax.named_scope("wait3"):
        wait_all(grp_r(NK + 2))
    with jax.named_scope("pro4"):
        tts = [None] * 4
        for n in range(7):
            for g in QK_FIRST.get(n, ()):
                tts[g] = qk_group(0, True, g)
            for g in PV_FIRST.get(n, ()):
                pv_group(0, True, tts[g], g, 2)
            q_stage(1, n, NH, add=8)
    with jax.named_scope("wait4"):
        wait_all(grp_r(NK + 3))
    with jax.named_scope("pro5"):
        oproj(0, 0, first=True, split=True)
    with jax.named_scope("xsA"):
        make_xs(0)

    def body_a(s, carry):
        with jax.named_scope("waitA"):
            @pl.when((s & 1) == 0)
            def _():
                wait_all(grp_a_kv(s, dyn=True))

            wait_all(grp_a(s, dyn=True))

            @pl.when(s == LA - 1)
            def _():
                xb_cp().wait()
                make_xs(1)

        with jax.named_scope("bodyA"):
            attn_qproj(s, True, next_a(s), (s == LA - 1) * 1, SEQ_A)
            oproj(s, 0)
        return carry

    lax.fori_loop(1, LA, body_a, 0)

    def body_b(p, carry):
        with jax.named_scope("waitB"):
            wait_all(grp_b(p, dyn=True))
        with jax.named_scope("bodyB"):
            for k in range(BU):
                u = BU * p + k
                attn_qproj(u, False, NSB + u + 1, 1, SEQ_B)
                oproj(NSB + u, 1)
        return carry

    lax.fori_loop(0, NB, body_b, 0)

    with jax.named_scope("epi0"):
        wait_all(grp_e())
    with jax.named_scope("epi1"):
        attn_qproj(NSB - 2, False, LA, 0, SEQ_E)
        oproj(NS - 2, 1)
        attn_qproj(LA, True, NS - 1, 1, SEQ_A, levels=1)
        tts = final_oproj(LA, 0, ((0, 0, 256), (1, 0, 256)), True)
        for g in range(4):
            pv_group(NSB - 1, False, tts[g], g, 1)
        final_oproj(NS - 1, 1, ((0, 0, 256), (1, 0, 128), (1, 128, 128)), False)
    with jax.named_scope("tail"):
        sharp = jnp.logical_not(jnp.max(smax[...]) <= S_LIMIT)
        wait_all(outs)

    @pl.when(sharp)
    def _():
        def step(t, carry):
            br, bb, j = t >> 5, (t >> 3) & 3, t & 7
            is_a = br == 0

            def kv4(a_buf, b_buf, b):
                return jnp.where(is_a, jnp.concatenate([a_buf[b, j >> 1]] * HPS, axis=0), b_buf[b, j])

            xr = x_buf[br, pl.ds(bb * 4, 4)].reshape(MQ, D)
            q = jnp.dot(xr, wq_buf[br * NSB + j], preferred_element_type=F32).astype(BF16)
            pts = []
            for bi in range(4):
                q4 = jnp.concatenate(
                    [q[bi * SQ:(bi + 1) * SQ, h * DH:(h + 1) * DH] for h in range(HPS)], axis=0)
                pts.append(_softmax_cols(diag(lax.dot_general(
                    kv4(ka_buf, kb_buf, bb * 4 + bi), q4, NT, preferred_element_type=F32))))
            tt = jnp.concatenate(pts, axis=0).T
            v4 = [kv4(va_buf, vb_buf, bb * 4 + bi) for bi in range(4)]
            o = jnp.concatenate(
                [lax.dot_general(p_lhs(tt, h),
                                 jnp.concatenate([v[h * SK:(h + 1) * SK] for v in v4], axis=0),
                                 NN, preferred_element_type=F32) for h in range(HPS)], axis=1)
            m = jnp.dot(o.astype(BF16), wo_buf[br * NSB + j], preferred_element_type=F32)
            for c in range(4):
                acc = jnp.where(j == 0, 0.0, accm[0, c]) + m[:, c * NQ4:(c + 1) * NQ4]
                accm[0, c] = acc
                out_buf[br, pl.ds(bb * 4, 4), :, :, c * NQ4:(c + 1) * NQ4] = (
                    acc.astype(BF16).reshape(4, 2, SH, NQ4))
            return carry

        lax.fori_loop(0, 2 * (B // 4) * NSB, step, 0)
        for br in range(2):
            out_cp(br, 0, D).start()
        for br in range(2):
            out_cp(br, 0, D).wait()


@jax.jit
def pallas_concat_heads__gqa_block_cached__mha_block_cached__near_ridge_kernel(A_x, A_k_cache, A_v_cache, A_wq, A_wo, B_x, B_k_cache, B_v_cache, B_wq, B_wo):
    xa = A_x.reshape(B, 2, SH, D)
    xb = B_x.reshape(B, 2, SH, D)
    kb = B_k_cache.reshape(B, NSB, HPS * SK, DH)
    vb = B_v_cache.reshape(B, NSB, HPS * SK, DH)
    any_spec = pl.BlockSpec(memory_space=pl.ANY)
    out = pl.pallas_call(
        _kernel,
        in_specs=[any_spec] * 10,
        out_specs=any_spec,
        out_shape=jax.ShapeDtypeStruct((B, 2, SH, 2 * D), BF16),
        scratch_shapes=[
            pltpu.VMEM((2, B, 2, SH, D), BF16),
            pltpu.VMEM((B, HKV, SK, DH), BF16),
            pltpu.VMEM((B, HKV, SK, DH), BF16),
            pltpu.VMEM((B, NSB, HPS * SK, DH), BF16),
            pltpu.VMEM((B, NSB, HPS * SK, DH), BF16),
            pltpu.VMEM((NS, D, CH), BF16),
            pltpu.VMEM((NS, CH, D), BF16),
            pltpu.VMEM((M // 2, CH), U32),
            pltpu.VMEM((2, B, 2, SH, D), BF16),
            pltpu.VMEM((7 * MQ // 2, 7 * DH), U32),
            pltpu.VMEM((2, 49, MQ, NQ4), F32),
            pltpu.VMEM((12, MH, QNH), F32),
            pltpu.VMEM((4, SK, 4 * SQ), F32),
            pltpu.VMEM((2, len(XS) * MQ // 2, 7 * NQ4), U32),
            pltpu.SemaphoreType.DMA((N_SEM,)),
        ],
        compiler_params=pltpu.CompilerParams(vmem_limit_bytes=100 * 1024 * 1024,
                                             disable_semaphore_checks=True),
        name="fused_attn",
    )(xa, A_k_cache, A_v_cache, A_wq, A_wo, xb, kb, vb, B_wq, B_wo)
    return out.reshape(B, SQ, 2 * D)
```

```python
import numpy as np
import jax
import jax.numpy as jnp
from jax import lax
import jax.experimental.pallas as pl
import jax.experimental.pallas.tpu as pltpu

B, SQ, D, H, HKV, SK, DH = 16, 32, 1024, 32, 4, 32, 128
M = B * SQ
MH = M // 2
MQ = M // 4
SH, RQ = SQ // 2, SQ // 4
HPS = 4
CH = HPS * DH
NSB = H // HPS
NS = 2 * NSB
LA = NSB - 1
NH, NQ4 = D // 2, D // 4
QNH, QMQ = CH // 2, MH // 2
KSL = (128, 128, 256)
NK = len(KSL)
C_EXP2 = float(DH ** -0.5 * np.log2(np.e))
S_LIMIT = float(6.0 * DH ** 0.5)
NT = (((1,), (1,)), ((), ()))
NN = (((1,), (0,)), ((), ()))
F32 = jnp.float32
BF16 = jnp.bfloat16
U32 = jnp.uint32

_LHS = [((0, 0), (1, 1), -1), ((1, 0), (1, 1), -1), ((0, 0), None, 0), ((1, 1), None, 0),
        ((0, 0), (0, 1), -1), ((1, 0), (0, 0), -1), ((0, 1), (1, 1), -1)]
_RHS = [((0, 0), (1, 1), -1), ((0, 0), None, 0), ((0, 1), (1, 1), 1), ((1, 0), (0, 0), 1),
        ((1, 1), None, 0), ((0, 0), (0, 1), 1), ((1, 0), (1, 1), 1)]
_OUT = {(0, 0): {0: 1, 3: 1, 4: 1, 6: 1}, (0, 1): {2: 1, 4: -1},
        (1, 0): {1: 1, 3: 1}, (1, 1): {0: 1, 1: -1, 2: 1, 5: 1}}
_SWAP = (0, 1, 0, 0, 1, 1, 1)


def _o_order():
    nt = [1 if r[1] is None else 2 for r in _RHS]
    allp = [(i, j) for i in range(7) for j in range(7)]
    heavy, mid, light = ([p for p in allp if nt[p[0]] * nt[p[1]] == n] for n in (4, 2, 1))
    cheap = mid[:10] + light[2:] + mid[10:]
    seq = light[:2]
    while heavy or cheap:
        seq += heavy[:1] + cheap[:1]
        heavy, cheap = heavy[1:], cheap[1:]
    return tuple(seq)


O_SEQ = _o_order()


def _q_order(slots):
    g = lambda i: [(i, n) for n in range(7)]
    seq = []
    for n, u in enumerate(g(1)[:2] + g(0) + g(5) + g(6) + g(1)[2:] + g(3) + g(4) + g(2)):
        seq += slots.get(n, "").split() + [u]
    return tuple(seq)


SEQ_A = _q_order({2: "q0 q1", 6: "q2 q3", 34: "p0 p1 p2 p3"})
SEQ_B = _q_order({3: "q0 q1 q2 q3", 21: "p0", 33: "p1", 35: "p2", 37: "p3"})
SEQ_EB = _q_order({6: "q0 q1 q2 q3", 20: "p0", 32: "p1", 34: "p2", 36: "p3"})
SEQ_EA = _q_order({2: "q0 q1", 6: "q2 q3", 20: "p0", 32: "p1", 34: "p2", 36: "p3"})
XS = (1, 4, 2, 3, 0, 5, 6)
QK_FIRST = {1: (0, 1), 2: (2, 3)}
PV_FIRST = {4: (0,), 5: (1, 2), 6: (3,)}

S_OUT = 0
S_A = 0
BU = 3
NB = (NSB - 2) // BU
S_B = LA
S_E = S_B + NB
S_R = S_E + 1
N_SEM = S_R + NK + 4


def _pk(x):
    return pltpu.bitcast(x.astype(BF16), U32)


def _upk(x):
    return pltpu.bitcast(x, BF16)


def _terms(spec):
    a, b, sg = spec
    return [(a, 1)] + ([(b, sg)] if b is not None else [])


def _signed_sum(items):
    items = sorted(items, key=lambda t: -t[0])
    acc = items[0][1]
    for sg, v in items[1:]:
        acc = acc + v if sg > 0 else acc - v
    return acc


def _comb(spec, get):
    return _signed_sum([(sg, get(t)) for t, sg in _terms(spec)])


def _operand(spec, ld):
    if spec[1] is None:
        return ld(spec[0])
    return _comb(spec, lambda t: ld(t).astype(F32)).astype(BF16)


def _softmax_cols(sc):
    m = jnp.max(sc, axis=0, keepdims=True)
    p = jnp.exp2((sc - m) * C_EXP2)
    l = jnp.sum(p, axis=0, keepdims=True)
    return p * (1.0 / l)


def _kernel(xa, ka, va, wqa, woa, xb, kb, vb, wqb, wob, out,
            x_buf, ka_buf, va_buf, kb_buf, vb_buf, wq_buf, wo_buf,
            q_buf, out_buf, os_buf, accm, mq_buf, smax, xs_buf, sems):
    cp = pltpu.make_async_copy

    def wq_cp(s, sem, dyn=False):
        dst = wq_buf.at[s]
        src = dst if dyn else (wqa if s < NSB else wqb).at[:, pl.ds((s % NSB) * CH, CH)]
        return cp(src, dst, sems.at[sem])

    def wo_cp(s, sem, dyn=False):
        dst = wo_buf.at[s]
        src = dst if dyn else (woa if s < NSB else wob).at[pl.ds((s % NSB) * CH, CH), :]
        return cp(src, dst, sems.at[sem])

    def kv_cp(src, dst, j, n, sem, dyn=False):
        d = dst.at[:, pl.ds(j, n)]
        return cp(d if dyn else src.at[:, pl.ds(j, n)], d, sems.at[sem])

    def wq_rows_cp(s, k0, kn, sem):
        return cp(wqa.at[pl.ds(k0, kn), pl.ds(s * CH, CH)], wq_buf.at[s, pl.ds(k0, kn), :], sems.at[sem])

    def xa_cols_cp(k0, kn, sem):
        return cp(xa.at[:, :, :, pl.ds(k0, kn)], x_buf.at[0, :, :, :, pl.ds(k0, kn)], sems.at[sem])

    def grp_r(n):
        sem = S_R + n
        if n < NK:
            k0 = sum(KSL[:n])
            return [xa_cols_cp(k0, KSL[n], sem), wq_rows_cp(0, k0, KSL[n], sem)]
        if n == NK:
            return [wq_rows_cp(1, 0, NH, sem)]
        if n == NK + 1:
            return [xa_cols_cp(NH, NH, sem), wq_rows_cp(0, NH, NH, sem)]
        if n == NK + 2:
            return [kv_cp(ka, ka_buf, 0, 1, sem), wq_rows_cp(1, NH, NH, sem), kv_cp(va, va_buf, 0, 1, sem)]
        return [wo_cp(0, sem)]

    def next_a(s):
        return s + 1 + (s == LA - 1) * 1

    def grp_a(s, dyn=False):
        return [wq_cp(next_a(s), S_A + s, dyn), wo_cp(s, S_A + s, dyn)]

    def grp_a_kv(s, dyn=False):
        g = s >> 1
        return [kv_cp(ka, ka_buf, g, 1, S_A + s, dyn), kv_cp(va, va_buf, g, 1, S_A + s, dyn)]

    def xb_cp():
        return cp(xb, x_buf.at[1], sems.at[S_A + LA - 1])

    def grp_b(p, dyn=False):
        u, sem = BU * p, S_B + p
        g = [kv_cp(kb, kb_buf, u, BU, sem, dyn), kv_cp(vb, vb_buf, u, BU, sem, dyn)]
        for k in range(BU):
            g += [wq_cp(NSB + u + k + 1, sem, dyn), wo_cp(NSB + u + k, sem, dyn)]
        return g

    def grp_e():
        return [kv_cp(kb, kb_buf, NSB - 2, 2, S_E), wq_cp(LA, S_E), kv_cp(vb, vb_buf, NSB - 2, 2, S_E),
                wo_cp(NS - 2, S_E), wq_cp(NS - 1, S_E), wo_cp(LA, S_E), wo_cp(NS - 1, S_E)]

    def out_cp(br, c0, nc):
        return cp(out_buf.at[br, :, :, :, pl.ds(c0, nc)],
                  out.at[:, :, :, pl.ds(br * D + c0, nc)], sems.at[S_OUT])

    def wait_all(cs):
        for c in cs:
            c.wait()

    for n in range(NK + 4):
        for c in grp_r(n):
            c.start()
    for s in range(1, LA):
        if s == LA - 1:
            xb_cp().start()
        for c in (grp_a_kv(s) if s % 2 == 0 else []) + grp_a(s):
            c.start()
    for p in range(NB):
        for c in grp_b(p):
            c.start()
    for c in grp_e():
        c.start()

    def zero_acc(k0, k1):
        accm[1, k0:k1] = jnp.zeros((k1 - k0,) + accm.shape[2:], F32)

    def zero_one(k, carry):
        accm[1, k] = jnp.zeros(accm.shape[2:], F32)
        return carry

    lax.fori_loop(0, 25, zero_one, 0)
    smax[...] = jnp.zeros(smax.shape, F32)

    lane_g = lax.broadcasted_iota(jnp.int32, (SK, 4 * SQ), 1) // SQ

    def x_block(br, half, c0, nc):
        return x_buf[br, :, half, :, c0:c0 + nc].reshape(MH, nc)

    def q_stage(s, n, k0, add=None, to=None):
        def q_prod(i):
            lhs = _operand(_LHS[i], lambda t: x_block(0, t[0], k0 + t[1] * NQ4, NQ4))
            rhs = _operand(_RHS[i], lambda t: wq_buf[s, k0 + t[0] * NQ4:k0 + (t[0] + 1) * NQ4,
                                                     t[1] * QNH:(t[1] + 1) * QNH])
            return jnp.dot(lhs, rhs, preferred_element_type=F32)

        def put(a, c, val):
            if add is not None:
                val = val + mq_buf[add + 2 * a + c]
            if to is not None:
                mq_buf[to + 2 * a + c] = val
            else:
                q_buf[a * QMQ:(a + 1) * QMQ, c * QNH:(c + 1) * QNH] = _pk(val)

        if n == 0:
            mq_buf[0] = q_prod(1)
        elif n == 1:
            mq_buf[1] = q_prod(4)
        elif n == 2:
            p0 = q_prod(0)
            mq_buf[2] = p0 - mq_buf[0]
            mq_buf[3] = p0 + mq_buf[1]
        elif n == 3:
            p2 = q_prod(2)
            put(0, 1, p2 - mq_buf[1])
            mq_buf[2] += p2
        elif n == 4:
            p3 = q_prod(3)
            put(1, 0, p3 + mq_buf[0])
            mq_buf[3] += p3
        elif n == 5:
            put(1, 1, mq_buf[2] + q_prod(5))
        else:
            put(0, 0, mq_buf[3] + q_prod(6))

    def make_xs(br):
        def one(b, carry):
            r8 = pl.multiple_of(b * 8, 8)
            for c in range(0, NQ4, DH):
                blk = {(a0, b0, kq): x_buf[br, b0 * 8 + b, a0, :, kq * NQ4 + c:kq * NQ4 + c + DH].astype(F32)
                       for a0 in range(2) for b0 in range(2) for kq in range(4)}
                for n, i in enumerate(XS):
                    l1 = {(b0, b1): _comb(_LHS[i], lambda a: blk[(a[0], b0, 2 * a[1] + b1)])
                          for b0 in range(2) for b1 in range(2)}
                    rows = pl.ds(n * (MQ // 2) + r8, 8)
                    for j in range(7):
                        if _LHS[i][1] is not None or _LHS[j][1] is not None:
                            xs_buf.at[br][rows, j * NQ4 + c:j * NQ4 + c + DH] = _pk(
                                _comb(_LHS[j], lambda t: l1[t]))
            return carry
        lax.fori_loop(0, B // 2, one, 0, unroll=2)

    def q_sub(s, br, i, j, cache):
        if _LHS[i][1] is not None or _LHS[j][1] is not None:
            n = XS.index(i)
            lhs = _upk(xs_buf[br, n * (MQ // 2):(n + 1) * (MQ // 2), j * NQ4:(j + 1) * NQ4])
        else:
            a, b = _LHS[i][0], _LHS[j][0]
            c0 = (2 * a[1] + b[1]) * NQ4
            lhs = x_buf[br, b[0] * 8:(b[0] + 1) * 8, a[0], :, c0:c0 + NQ4].reshape(MQ, NQ4)

        def ld(a, b):
            r, c = 2 * a[0] + b[0], 2 * a[1] + (b[1] ^ _SWAP[i])
            return wq_buf[s, r * NQ4:(r + 1) * NQ4, c * DH:(c + 1) * DH]

        if _RHS[i][1] is None:
            rhs = _operand(_RHS[j], lambda b: ld(_RHS[i][0], b))
        else:
            def sub(b):
                if (i, b) not in cache:
                    cache[(i, b)] = _comb(_RHS[i], lambda a: ld(a, b).astype(F32))
                return cache[(i, b)]
            rhs = _comb(_RHS[j], sub).astype(BF16)
        return jnp.dot(lhs, rhs, preferred_element_type=F32)

    def quad(slot, k):
        return mq_buf.at[slot].at[(k >> 1) * MQ:((k >> 1) + 1) * MQ, (k & 1) * DH:((k & 1) + 1) * DH]

    def qproj(s, br, seq, qk, pv):
        left = {(blk, k): len(terms) for blk, terms in _OUT.items() for k in range(4)}
        slot_of = {(1, 1): 0, (0, 0): 1, (0, 1): 2, (1, 0): 3}
        neg = {}
        cache = {}

        def emit(i, r2, c2, v):
            k = 2 * r2 + c2
            for blk, terms in _OUT.items():
                if i not in terms:
                    continue
                ref = quad(slot_of[blk], k)
                first = left[(blk, k)] == len(terms)
                left[(blk, k)] -= 1
                if first:
                    neg[(blk, k)] = terms[i] < 0
                    ref[...] = v
                    continue
                if neg[(blk, k)]:
                    assert terms[i] > 0
                    tot, neg[(blk, k)] = v - ref[...], False
                else:
                    tot = ref[...] + v if terms[i] > 0 else ref[...] - v
                if left[(blk, k)]:
                    ref[...] = tot
                else:
                    r0, c0 = blk[0] * QMQ + r2 * (MQ // 2), blk[1] * QNH + c2 * DH
                    q_buf[r0:r0 + MQ // 2, c0:c0 + DH] = _pk(tot)

        def inner(i, n):
            t = lambda k: quad(4 + XS.index(i), k)
            done = lambda r2, c2, v: emit(i, r2, c2 ^ _SWAP[i], v)
            if n == 0:
                t(0)[...] = q_sub(s, br, i, 1, cache)
            elif n == 1:
                t(1)[...] = q_sub(s, br, i, 4, cache)
            elif n == 2:
                p0 = q_sub(s, br, i, 0, cache)
                t(2)[...] = p0 - t(0)[...]
                t(3)[...] = p0 + t(1)[...]
            elif n == 3:
                p2 = q_sub(s, br, i, 2, cache)
                done(0, 1, p2 - t(1)[...])
                t(2)[...] += p2
            elif n == 4:
                p3 = q_sub(s, br, i, 3, cache)
                done(1, 0, p3 + t(0)[...])
                t(3)[...] += p3
            elif n == 5:
                done(1, 1, t(2)[...] + q_sub(s, br, i, 5, cache))
            else:
                done(0, 0, t(3)[...] + q_sub(s, br, i, 6, cache))

        for u in seq:
            if isinstance(u, str):
                (qk if u[0] == "q" else pv)(int(u[1]))
            else:
                inner(*u)

    def o_prod(s, i, j, r0, nr):
        ts = [(s1 * s2, 2 * a[0] + b[0], 2 * a[1] + (b[1] ^ _SWAP[i]))
              for a, s1 in _terms(_RHS[i]) for b, s2 in _terms(_RHS[j])]
        ld = lambda r, c: wo_buf[s, r * DH:(r + 1) * DH, c * NQ4:(c + 1) * NQ4]
        if len(ts) == 1:
            rhs = ld(ts[0][1], ts[0][2])
        else:
            rhs = _signed_sum([(sg, ld(r, c).astype(F32)) for sg, r, c in ts]).astype(BF16)
        lhs = _upk(os_buf[(i * MQ + r0) // 2:(i * MQ + r0 + nr) // 2, j * DH:(j + 1) * DH])
        return jnp.dot(lhs, rhs, preferred_element_type=F32)

    def oproj(s, br, first=False, split=False):
        for n, (i, j) in enumerate(O_SEQ):
            for r0, nr in (((0, MQ // 2), (MQ // 2, MQ // 2)) if split and n == 0 else ((0, MQ),)):
                m = o_prod(s, i, j, r0, nr)
                if not first:
                    m = accm[br, i * 7 + j, r0:r0 + nr] + m
                accm[br, i * 7 + j, r0:r0 + nr] = m

    def diag(st):
        sc = st[0:SK]
        for h in range(1, HPS):
            sc = jnp.where(lane_g == h, st[h * SK:(h + 1) * SK], sc)
        return sc

    def scores(j, is_a, b, q4):
        if is_a:
            return lax.dot_general(ka_buf[b, j >> 1], q4, NT, preferred_element_type=F32)
        return diag(lax.dot_general(kb_buf[b, j], q4, NT, preferred_element_type=F32))

    def p_lhs(tt, h):
        ph = tt[h * SQ:(h + 1) * SQ]
        return jnp.concatenate([jnp.where(lane_g == bi, ph, 0.0) for bi in range(4)], axis=0).astype(BF16)

    def qk_group(j, is_a, bb):
        pts = []
        big = None
        for b in range(bb * 4, bb * 4 + 4):
            q4 = _upk(jnp.concatenate(
                [q_buf[half * QMQ + b * 8:half * QMQ + (b + 1) * 8, h * DH:(h + 1) * DH]
                 for h in range(HPS) for half in range(2)], axis=0))
            sc = scores(j, is_a, b, q4)
            big = jnp.abs(sc) if big is None else jnp.maximum(big, jnp.abs(sc))
            pts.append(_softmax_cols(sc))
        smax[bb] = jnp.maximum(smax[bb], big)
        return jnp.concatenate(pts, axis=0).T

    def pv_tile(j, is_a, tt, bb, h):
        lhs = p_lhs(tt, h)
        if is_a:
            vh = jnp.concatenate([va_buf[bb * 4 + bi, j >> 1] for bi in range(4)], axis=0)
        else:
            vh = jnp.concatenate(
                [vb_buf[bb * 4 + bi, j, h * SK:(h + 1) * SK, :] for bi in range(4)], axis=0)
        return lax.dot_general(lhs, vh, NN, preferred_element_type=F32)

    def pv_group(j, is_a, tt, bb, levels):
        t = [pv_tile(j, is_a, tt, bb, h) for h in range(HPS)]
        for pr in range(2):
            base = {(r, h): jnp.concatenate(
                [t[h][bi * SQ + r * RQ:bi * SQ + (r + 1) * RQ] for bi in (2 * pr, 2 * pr + 1)], axis=0)
                for r in range(4) for h in range(HPS)}
            for i in range(7):
                r0 = i * MQ // 2 + (bb * 2 + pr) * RQ
                l1 = {(b0, b1): _comb(_LHS[i], lambda a: base[(2 * a[0] + b0, 2 * a[1] + b1)])
                      for b0 in range(2) for b1 in range(2)}
                if levels == 1:
                    ops = list(l1.values())
                else:
                    ops = [None] * 7
                for jj, v in enumerate(ops):
                    v = _comb(_LHS[jj], lambda t2: l1[t2]) if v is None else v
                    os_buf[r0:r0 + RQ, jj * DH:(jj + 1) * DH] = _pk(v)

    def attn_qproj(j, is_a, s, br, seq, levels=2):
        tts = [None] * 4

        def qk(g):
            tts[g] = qk_group(j, is_a, g)

        qproj(s, br, seq, qk, lambda g: pv_group(j, is_a, tts[g], g, levels))

    outs = []

    def final_oproj(s, br, chunks, with_qk):
        tts = None
        for c2, c0, tc in chunks:
            cc = c2 * NQ4 + c0

            def total(i):
                lhs = _upk(jnp.concatenate(
                    [os_buf[i * MQ // 2:(i + 1) * MQ // 2, b0 * QNH:(b0 + 1) * QNH] for b0 in range(2)],
                    axis=0))
                rhs = _operand(_RHS[i], lambda t: wo_buf[s, t[0] * QNH:(t[0] + 1) * QNH,
                                                         t[1] * NH + cc:t[1] * NH + cc + tc])
                m = jnp.dot(lhs, rhs, preferred_element_type=F32)
                return [_signed_sum([(1, m[r2 * MQ:(r2 + 1) * MQ])] +
                                    [(sg, accm[br, i * 7 + j, :, c0:c0 + tc])
                                     for j, sg in _OUT[(r2, c2 ^ _SWAP[i])].items()]) for r2 in range(2)]

            d = {}
            for i in (4, 1, 2, 0, 5, 3, 6):
                if with_qk and tts is None and d:
                    tts = [qk_group(NSB - 1, False, g) for g in range(4)]
                d[i] = total(i)
                for (r1, c1), terms in _OUT.items():
                    if i in terms and set(terms) <= set(d):
                        for r2 in range(2):
                            val = _signed_sum([(sg, d[k][r2]) for k, sg in terms.items()])
                            out_buf[br, :, r1, r2 * RQ:(r2 + 1) * RQ, c1 * NH + cc:c1 * NH + cc + tc] = (
                                val.reshape(B, RQ, tc).astype(BF16))
                if i in (5, 6):
                    outs.append(out_cp(br, (1 if i == 5 else 0) * NH + cc, tc))
                    outs[-1].start()
        return tts

    for n in range(NK):
        with jax.named_scope("wait0"):
            wait_all(grp_r(n))
        with jax.named_scope("pro1"):
            k0, kn = sum(KSL[:n]), KSL[n]
            xs = jnp.concatenate([x_block(0, a, k0, kn) for a in range(2)], axis=0)
            part = jnp.dot(xs, wq_buf[0, k0:k0 + kn, :], preferred_element_type=F32)
            for a in range(2):
                for c in range(2):
                    pq = part[a * MH:(a + 1) * MH, c * QNH:(c + 1) * QNH]
                    if n == 0:
                        mq_buf[4 + 2 * a + c] = pq
                    else:
                        mq_buf[4 + 2 * a + c] += pq
            z0 = 25 + sum(k // 128 * 3 for k in KSL[:n])
            zero_acc(z0, z0 + kn // 128 * 3)
    with jax.named_scope("wait1"):
        wait_all(grp_r(NK))
    with jax.named_scope("pro2"):
        zero_acc(37, 43)
        for n in range(7):
            q_stage(1, n, 0, to=8)
    with jax.named_scope("wait2"):
        wait_all(grp_r(NK + 1))
    with jax.named_scope("pro3"):
        zero_acc(43, 49)
        for n in range(7):
            q_stage(0, n, NH, add=4)
    with jax.named_scope("wait3"):
        wait_all(grp_r(NK + 2))
    with jax.named_scope("pro4"):
        tts = [None] * 4
        for n in range(7):
            for g in QK_FIRST.get(n, ()):
                tts[g] = qk_group(0, True, g)
            for g in PV_FIRST.get(n, ()):
                pv_group(0, True, tts[g], g, 2)
            q_stage(1, n, NH, add=8)
    with jax.named_scope("wait4"):
        wait_all(grp_r(NK + 3))
    with jax.named_scope("pro5"):
        oproj(0, 0, first=True, split=True)
    with jax.named_scope("xsA"):
        make_xs(0)

    def body_a(s, carry):
        with jax.named_scope("waitA"):
            @pl.when((s & 1) == 0)
            def _():
                wait_all(grp_a_kv(s, dyn=True))

            wait_all(grp_a(s, dyn=True))

            @pl.when(s == LA - 1)
            def _():
                xb_cp().wait()
                make_xs(1)

        with jax.named_scope("bodyA"):
            attn_qproj(s, True, next_a(s), (s == LA - 1) * 1, SEQ_A)
            oproj(s, 0)
        return carry

    lax.fori_loop(1, LA, body_a, 0)

    def body_b(p, carry):
        with jax.named_scope("waitB"):
            wait_all(grp_b(p, dyn=True))
        with jax.named_scope("bodyB"):
            for k in range(BU):
                u = BU * p + k
                attn_qproj(u, False, NSB + u + 1, 1, SEQ_B)
                oproj(NSB + u, 1)
        return carry

    lax.fori_loop(0, NB, body_b, 0)

    with jax.named_scope("epi0"):
        wait_all(grp_e())
    with jax.named_scope("epi1"):
        attn_qproj(NSB - 2, False, LA, 0, SEQ_EB)
        oproj(NS - 2, 1)
        attn_qproj(LA, True, NS - 1, 1, SEQ_EA, levels=1)
        tts = final_oproj(LA, 0, ((0, 0, 256), (1, 0, 256)), True)
        for g in range(4):
            pv_group(NSB - 1, False, tts[g], g, 1)
        final_oproj(NS - 1, 1, ((0, 0, 256), (1, 0, 128), (1, 128, 128)), False)
    with jax.named_scope("tail"):
        sharp = jnp.logical_not(jnp.max(smax[...]) <= S_LIMIT)
        wait_all(outs)

    @pl.when(sharp)
    def _():
        def step(t, carry):
            br, bb, j = t >> 5, (t >> 3) & 3, t & 7
            is_a = br == 0

            def kv4(a_buf, b_buf, b):
                return jnp.where(is_a, jnp.concatenate([a_buf[b, j >> 1]] * HPS, axis=0), b_buf[b, j])

            xr = x_buf[br, pl.ds(bb * 4, 4)].reshape(MQ, D)
            q = jnp.dot(xr, wq_buf[br * NSB + j], preferred_element_type=F32).astype(BF16)
            pts = []
            for bi in range(4):
                q4 = jnp.concatenate(
                    [q[bi * SQ:(bi + 1) * SQ, h * DH:(h + 1) * DH] for h in range(HPS)], axis=0)
                pts.append(_softmax_cols(diag(lax.dot_general(
                    kv4(ka_buf, kb_buf, bb * 4 + bi), q4, NT, preferred_element_type=F32))))
            tt = jnp.concatenate(pts, axis=0).T
            v4 = [kv4(va_buf, vb_buf, bb * 4 + bi) for bi in range(4)]
            o = jnp.concatenate(
                [lax.dot_general(p_lhs(tt, h),
                                 jnp.concatenate([v[h * SK:(h + 1) * SK] for v in v4], axis=0),
                                 NN, preferred_element_type=F32) for h in range(HPS)], axis=1)
            m = jnp.dot(o.astype(BF16), wo_buf[br * NSB + j], preferred_element_type=F32)
            for c in range(4):
                acc = jnp.where(j == 0, 0.0, accm[0, c]) + m[:, c * NQ4:(c + 1) * NQ4]
                accm[0, c] = acc
                out_buf[br, pl.ds(bb * 4, 4), :, :, c * NQ4:(c + 1) * NQ4] = (
                    acc.astype(BF16).reshape(4, 2, SH, NQ4))
            return carry

        lax.fori_loop(0, 2 * (B // 4) * NSB, step, 0)
        for br in range(2):
            out_cp(br, 0, D).start()
        for br in range(2):
            out_cp(br, 0, D).wait()


@jax.jit
def pallas_concat_heads__gqa_block_cached__mha_block_cached__near_ridge_kernel(A_x, A_k_cache, A_v_cache, A_wq, A_wo, B_x, B_k_cache, B_v_cache, B_wq, B_wo):
    xa = A_x.reshape(B, 2, SH, D)
    xb = B_x.reshape(B, 2, SH, D)
    kb = B_k_cache.reshape(B, NSB, HPS * SK, DH)
    vb = B_v_cache.reshape(B, NSB, HPS * SK, DH)
    any_spec = pl.BlockSpec(memory_space=pl.ANY)
    out = pl.pallas_call(
        _kernel,
        in_specs=[any_spec] * 10,
        out_specs=any_spec,
        out_shape=jax.ShapeDtypeStruct((B, 2, SH, 2 * D), BF16),
        scratch_shapes=[
            pltpu.VMEM((2, B, 2, SH, D), BF16),
            pltpu.VMEM((B, HKV, SK, DH), BF16),
            pltpu.VMEM((B, HKV, SK, DH), BF16),
            pltpu.VMEM((B, NSB, HPS * SK, DH), BF16),
            pltpu.VMEM((B, NSB, HPS * SK, DH), BF16),
            pltpu.VMEM((NS, D, CH), BF16),
            pltpu.VMEM((NS, CH, D), BF16),
            pltpu.VMEM((M // 2, CH), U32),
            pltpu.VMEM((2, B, 2, SH, D), BF16),
            pltpu.VMEM((7 * MQ // 2, 7 * DH), U32),
            pltpu.VMEM((2, 49, MQ, NQ4), F32),
            pltpu.VMEM((12, MH, QNH), F32),
            pltpu.VMEM((4, SK, 4 * SQ), F32),
            pltpu.VMEM((2, 7 * MQ // 2, 7 * NQ4), U32),
            pltpu.SemaphoreType.DMA((N_SEM,)),
        ],
        compiler_params=pltpu.CompilerParams(vmem_limit_bytes=100 * 1024 * 1024,
                                             disable_semaphore_checks=True),
        name="fused_attn",
    )(xa, A_k_cache, A_v_cache, A_wq, A_wo, xb, kb, vb, B_wq, B_wo)
    return out.reshape(B, SQ, 2 * D)
```

```python
import numpy as np
import jax
import jax.numpy as jnp
from jax import lax
import jax.experimental.pallas as pl
import jax.experimental.pallas.tpu as pltpu

B, SQ, D, H, HKV, SK, DH = 16, 32, 1024, 32, 4, 32, 128
M = B * SQ
MH = M // 2
MQ = M // 4
SH, RQ = SQ // 2, SQ // 4
HPS = 4
CH = HPS * DH
NSB = H // HPS
NS = 2 * NSB
LA = NSB - 1
NH, NQ4 = D // 2, D // 4
QNH, QMQ = CH // 2, MH // 2
C_EXP2 = float(DH ** -0.5 * np.log2(np.e))
S_LIMIT = float(6.0 * DH ** 0.5)
NT = (((1,), (1,)), ((), ()))
NN = (((1,), (0,)), ((), ()))
F32 = jnp.float32
BF16 = jnp.bfloat16
U32 = jnp.uint32

_LHS = [((0, 0), (1, 1), -1), ((1, 0), (1, 1), -1), ((0, 0), None, 0), ((1, 1), None, 0),
        ((0, 0), (0, 1), -1), ((1, 0), (0, 0), -1), ((0, 1), (1, 1), -1)]
_RHS = [((0, 0), (1, 1), -1), ((0, 0), None, 0), ((0, 1), (1, 1), 1), ((1, 0), (0, 0), 1),
        ((1, 1), None, 0), ((0, 0), (0, 1), 1), ((1, 0), (1, 1), 1)]
_OUT = {(0, 0): {0: 1, 3: 1, 4: 1, 6: 1}, (0, 1): {2: 1, 4: -1},
        (1, 0): {1: 1, 3: 1}, (1, 1): {0: 1, 1: -1, 2: 1, 5: 1}}
_SWAP = (0, 1, 0, 0, 1, 1, 1)


def _o_order():
    nt = [1 if r[1] is None else 2 for r in _RHS]
    allp = [(i, j) for i in range(7) for j in range(7)]
    heavy, mid, light = ([p for p in allp if nt[p[0]] * nt[p[1]] == n] for n in (4, 2, 1))
    cheap = mid[:10] + light[2:] + mid[10:]
    seq = light[:2]
    while heavy or cheap:
        seq += heavy[:1] + cheap[:1]
        heavy, cheap = heavy[1:], cheap[1:]
    return tuple(seq)


O_SEQ = _o_order()


def _g(*idx):
    return [(i, n) for i in idx for n in range(7)]


def _q_order(slots, base=None):
    base = base or _g(1)[:2] + _g(0, 5, 6) + _g(1)[2:] + _g(3, 4, 2)
    seq = []
    for n, u in enumerate(base):
        seq += slots.get(n, "").split() + [u]
    return tuple(seq)


SEQ_A = _q_order({2: "q0 q1", 6: "q2 q3", 34: "p0 p1 p2 p3"})
SEQ_B = _q_order({3: "q0 q1 q2 q3", 21: "p0", 33: "p1", 35: "p2", 37: "p3"})
SEQ_EB = _q_order({6: "q0 q1 q2 q3", 20: "p0", 32: "p1", 34: "p2", 36: "p3"})
SEQ_EA = _q_order({2: "q0 q1", 6: "q2 q3", 20: "p0", 32: "p1", 34: "p2", 36: "p3"})
SEQ_0 = _q_order({0: "w0", 6: "w1", 20: "w2", 48: "w3"},
                 _g(1)[:6] + _g(4)[:2] + _g(1)[6:] + _g(4)[2:] + _g(0, 2, 5, 3, 6))
SEQ_1 = _q_order({3: "q0 q1", 7: "q2 q3", 19: "w4 p0 p1 p2 p3"}, _g(1, 4, 0, 2, 5, 3, 6))
XS = (1, 4, 2, 3, 0, 5, 6)

S_OUT = 0
S_A = 0
BU = 3
NB = (NSB - 2) // BU
S_B = LA
S_E = S_B + NB
S_X = S_E + 1
S_R = S_X + 4
N_SEM = S_R + 6


def _pk(x):
    return pltpu.bitcast(x.astype(BF16), U32)


def _upk(x):
    return pltpu.bitcast(x, BF16)


def _terms(spec):
    a, b, sg = spec
    return [(a, 1)] + ([(b, sg)] if b is not None else [])


def _signed_sum(items):
    items = sorted(items, key=lambda t: -t[0])
    acc = items[0][1]
    for sg, v in items[1:]:
        acc = acc + v if sg > 0 else acc - v
    return acc


def _comb(spec, get):
    return _signed_sum([(sg, get(t)) for t, sg in _terms(spec)])


def _operand(spec, ld):
    if spec[1] is None:
        return ld(spec[0])
    return _comb(spec, lambda t: ld(t).astype(F32)).astype(BF16)


def _softmax_cols(sc):
    m = jnp.max(sc, axis=0, keepdims=True)
    p = jnp.exp2((sc - m) * C_EXP2)
    l = jnp.sum(p, axis=0, keepdims=True)
    return p * (1.0 / l)


def _kernel(xa, ka, va, wqa, woa, xb, kb, vb, wqb, wob, out,
            x_buf, ka_buf, va_buf, kb_buf, vb_buf, wq_buf, wo_buf,
            q_buf, out_buf, os_buf, accm, mq_buf, smax, xs_buf, sems):
    cp = pltpu.make_async_copy

    def wq_cp(s, sem, dyn=False):
        dst = wq_buf.at[s]
        src = dst if dyn else (wqa if s < NSB else wqb).at[:, pl.ds((s % NSB) * CH, CH)]
        return cp(src, dst, sems.at[sem])

    def wo_cp(s, sem, dyn=False):
        dst = wo_buf.at[s]
        src = dst if dyn else (woa if s < NSB else wob).at[pl.ds((s % NSB) * CH, CH), :]
        return cp(src, dst, sems.at[sem])

    def kv_cp(src, dst, j, n, sem, dyn=False):
        d = dst.at[:, pl.ds(j, n)]
        return cp(d if dyn else src.at[:, pl.ds(j, n)], d, sems.at[sem])

    def wq_quad_cp(s, a, b, sem):
        r, c = pl.ds(a * NH, NH), b * QNH
        return cp(wqa.at[r, pl.ds(s * CH + c, QNH)], wq_buf.at[s, r, pl.ds(c, QNH)], sems.at[sem])

    def grp_x(g, dyn=False):
        cs = []
        for b0 in (2 * g, 8 + 2 * g):
            d = x_buf.at[0, pl.ds(b0, 2)]
            cs.append(cp(d if dyn else xa.at[pl.ds(b0, 2)], d, sems.at[S_X + g]))
        return cs

    def grp_r(n):
        sem = S_R + n
        if n < 2:
            return [wq_quad_cp(0, n, n, sem)]
        if n == 2:
            return [wq_quad_cp(0, 0, 1, sem), wq_quad_cp(0, 1, 0, sem)]
        if n == 3:
            return [wq_quad_cp(1, 0, 0, sem), kv_cp(ka, ka_buf, 0, 1, sem), wq_quad_cp(1, 1, 1, sem)]
        if n == 4:
            return [wq_quad_cp(1, 0, 1, sem), kv_cp(va, va_buf, 0, 1, sem), wq_quad_cp(1, 1, 0, sem)]
        return [wo_cp(0, sem)]

    def next_a(s):
        return s + 1 + (s == LA - 1) * 1

    def grp_a(s, dyn=False):
        return [wq_cp(next_a(s), S_A + s, dyn), wo_cp(s, S_A + s, dyn)]

    def grp_a_kv(s, dyn=False):
        g = s >> 1
        return [kv_cp(ka, ka_buf, g, 1, S_A + s, dyn), kv_cp(va, va_buf, g, 1, S_A + s, dyn)]

    def xb_cp():
        return cp(xb, x_buf.at[1], sems.at[S_A + LA - 1])

    def grp_b(p, dyn=False):
        u, sem = BU * p, S_B + p
        g = [kv_cp(kb, kb_buf, u, BU, sem, dyn), kv_cp(vb, vb_buf, u, BU, sem, dyn)]
        for k in range(BU):
            g += [wq_cp(NSB + u + k + 1, sem, dyn), wo_cp(NSB + u + k, sem, dyn)]
        return g

    def grp_e():
        return [kv_cp(kb, kb_buf, NSB - 2, 2, S_E), wq_cp(LA, S_E), kv_cp(vb, vb_buf, NSB - 2, 2, S_E),
                wo_cp(NS - 2, S_E), wq_cp(NS - 1, S_E), wo_cp(LA, S_E), wo_cp(NS - 1, S_E)]

    def out_cp(br, c0, nc):
        return cp(out_buf.at[br, :, :, :, pl.ds(c0, nc)],
                  out.at[:, :, :, pl.ds(br * D + c0, nc)], sems.at[S_OUT])

    def wait_all(cs):
        for c in cs:
            c.wait()

    for g in range(4):
        for c in grp_x(g):
            c.start()
    for n in range(6):
        for c in grp_r(n):
            c.start()
    for s in range(1, LA):
        if s == LA - 1:
            xb_cp().start()
        for c in (grp_a_kv(s) if s % 2 == 0 else []) + grp_a(s):
            c.start()
    for p in range(NB):
        for c in grp_b(p):
            c.start()
    for c in grp_e():
        c.start()

    def zero_one(k, carry):
        accm[1, k] = jnp.zeros(accm.shape[2:], F32)
        return carry

    lax.fori_loop(0, 25, zero_one, 0)
    smax[...] = jnp.zeros(smax.shape, F32)

    lane_g = lax.broadcasted_iota(jnp.int32, (SK, 4 * SQ), 1) // SQ

    def xs_rows(br, b):
        r8 = pl.multiple_of(b * 8, 8)
        for c in range(0, NQ4, DH):
            blk = {(a0, b0, kq): x_buf[br, b0 * 8 + b, a0, :, kq * NQ4 + c:kq * NQ4 + c + DH].astype(F32)
                   for a0 in range(2) for b0 in range(2) for kq in range(4)}
            for n, i in enumerate(XS):
                l1 = {(b0, b1): _comb(_LHS[i], lambda a: blk[(a[0], b0, 2 * a[1] + b1)])
                      for b0 in range(2) for b1 in range(2)}
                rows = pl.ds(n * (MQ // 2) + r8, 8)
                for j in range(7):
                    if _LHS[i][1] is not None or _LHS[j][1] is not None:
                        xs_buf.at[br][rows, j * NQ4 + c:j * NQ4 + c + DH] = _pk(
                            _comb(_LHS[j], lambda t: l1[t]))

    def make_xs(br):
        def pair(g, carry):
            if br == 0:
                wait_all(grp_x(g, dyn=True))
            xs_rows(br, 2 * g)
            xs_rows(br, 2 * g + 1)
            if br == 0:
                lax.fori_loop(25 + 6 * g, 31 + 6 * g, zero_one, 0)
            return carry
        lax.fori_loop(0, 4, pair, 0)

    def q_sub(s, br, i, j, cache):
        if _LHS[i][1] is not None or _LHS[j][1] is not None:
            n = XS.index(i)
            lhs = _upk(xs_buf[br, n * (MQ // 2):(n + 1) * (MQ // 2), j * NQ4:(j + 1) * NQ4])
        else:
            a, b = _LHS[i][0], _LHS[j][0]
            c0 = (2 * a[1] + b[1]) * NQ4
            lhs = x_buf[br, b[0] * 8:(b[0] + 1) * 8, a[0], :, c0:c0 + NQ4].reshape(MQ, NQ4)

        def ld(a, b):
            r, c = 2 * a[0] + b[0], 2 * a[1] + (b[1] ^ _SWAP[i])
            return wq_buf[s, r * NQ4:(r + 1) * NQ4, c * DH:(c + 1) * DH]

        if _RHS[i][1] is None:
            rhs = _operand(_RHS[j], lambda b: ld(_RHS[i][0], b))
        else:
            def sub(b):
                if (i, b) not in cache:
                    cache[(i, b)] = _comb(_RHS[i], lambda a: ld(a, b).astype(F32))
                return cache[(i, b)]
            rhs = _comb(_RHS[j], sub).astype(BF16)
        return jnp.dot(lhs, rhs, preferred_element_type=F32)

    def quad(slot, k):
        return mq_buf.at[slot].at[(k >> 1) * MQ:((k >> 1) + 1) * MQ, (k & 1) * DH:((k & 1) + 1) * DH]

    def qproj(s, br, seq, qk, pv):
        left = {(blk, k): len(terms) for blk, terms in _OUT.items() for k in range(4)}
        slot_of = {(1, 1): 0, (0, 0): 1, (0, 1): 2, (1, 0): 3}
        neg = {}
        cache = {}

        def emit(i, r2, c2, v):
            k = 2 * r2 + c2
            for blk, terms in _OUT.items():
                if i not in terms:
                    continue
                ref = quad(slot_of[blk], k)
                first = left[(blk, k)] == len(terms)
                left[(blk, k)] -= 1
                if first:
                    neg[(blk, k)] = terms[i] < 0
                    ref[...] = v
                    continue
                if neg[(blk, k)]:
                    assert terms[i] > 0
                    tot, neg[(blk, k)] = v - ref[...], False
                else:
                    tot = ref[...] + v if terms[i] > 0 else ref[...] - v
                if left[(blk, k)]:
                    ref[...] = tot
                else:
                    r0, c0 = blk[0] * QMQ + r2 * (MQ // 2), blk[1] * QNH + c2 * DH
                    q_buf[r0:r0 + MQ // 2, c0:c0 + DH] = _pk(tot)

        def inner(i, n):
            t = lambda k: quad(4 + XS.index(i), k)
            done = lambda r2, c2, v: emit(i, r2, c2 ^ _SWAP[i], v)
            if n == 0:
                t(0)[...] = q_sub(s, br, i, 1, cache)
            elif n == 1:
                t(1)[...] = q_sub(s, br, i, 4, cache)
            elif n == 2:
                p0 = q_sub(s, br, i, 0, cache)
                t(2)[...] = p0 - t(0)[...]
                t(3)[...] = p0 + t(1)[...]
            elif n == 3:
                p2 = q_sub(s, br, i, 2, cache)
                done(0, 1, p2 - t(1)[...])
                t(2)[...] += p2
            elif n == 4:
                p3 = q_sub(s, br, i, 3, cache)
                done(1, 0, p3 + t(0)[...])
                t(3)[...] += p3
            elif n == 5:
                done(1, 1, t(2)[...] + q_sub(s, br, i, 5, cache))
            else:
                done(0, 0, t(3)[...] + q_sub(s, br, i, 6, cache))

        for u in seq:
            if isinstance(u, str):
                {"q": qk, "p": pv, "w": lambda n: wait_all(grp_r(n))}[u[0]](int(u[1]))
            else:
                inner(*u)

    def o_prod(s, i, j, r0, nr):
        ts = [(s1 * s2, 2 * a[0] + b[0], 2 * a[1] + (b[1] ^ _SWAP[i]))
              for a, s1 in _terms(_RHS[i]) for b, s2 in _terms(_RHS[j])]
        ld = lambda r, c: wo_buf[s, r * DH:(r + 1) * DH, c * NQ4:(c + 1) * NQ4]
        if len(ts) == 1:
            rhs = ld(ts[0][1], ts[0][2])
        else:
            rhs = _signed_sum([(sg, ld(r, c).astype(F32)) for sg, r, c in ts]).astype(BF16)
        lhs = _upk(os_buf[(i * MQ + r0) // 2:(i * MQ + r0 + nr) // 2, j * DH:(j + 1) * DH])
        return jnp.dot(lhs, rhs, preferred_element_type=F32)

    def oproj(s, br, first=False, split=False):
        for n, (i, j) in enumerate(O_SEQ):
            for r0, nr in (((0, MQ // 2), (MQ // 2, MQ // 2)) if split and n == 0 else ((0, MQ),)):
                m = o_prod(s, i, j, r0, nr)
                if not first:
                    m = accm[br, i * 7 + j, r0:r0 + nr] + m
                accm[br, i * 7 + j, r0:r0 + nr] = m

    def diag(st):
        sc = st[0:SK]
        for h in range(1, HPS):
            sc = jnp.where(lane_g == h, st[h * SK:(h + 1) * SK], sc)
        return sc

    def scores(j, is_a, b, q4):
        if is_a:
            return lax.dot_general(ka_buf[b, j >> 1], q4, NT, preferred_element_type=F32)
        return diag(lax.dot_general(kb_buf[b, j], q4, NT, preferred_element_type=F32))

    def p_lhs(tt, h):
        ph = tt[h * SQ:(h + 1) * SQ]
        return jnp.concatenate([jnp.where(lane_g == bi, ph, 0.0) for bi in range(4)], axis=0).astype(BF16)

    def qk_group(j, is_a, bb):
        pts = []
        big = None
        for b in range(bb * 4, bb * 4 + 4):
            q4 = _upk(jnp.concatenate(
                [q_buf[half * QMQ + b * 8:half * QMQ + (b + 1) * 8, h * DH:(h + 1) * DH]
                 for h in range(HPS) for half in range(2)], axis=0))
            sc = scores(j, is_a, b, q4)
            big = jnp.abs(sc) if big is None else jnp.maximum(big, jnp.abs(sc))
            pts.append(_softmax_cols(sc))
        smax[bb] = jnp.maximum(smax[bb], big)
        return jnp.concatenate(pts, axis=0).T

    def pv_tile(j, is_a, tt, bb, h):
        lhs = p_lhs(tt, h)
        if is_a:
            vh = jnp.concatenate([va_buf[bb * 4 + bi, j >> 1] for bi in range(4)], axis=0)
        else:
            vh = jnp.concatenate(
                [vb_buf[bb * 4 + bi, j, h * SK:(h + 1) * SK, :] for bi in range(4)], axis=0)
        return lax.dot_general(lhs, vh, NN, preferred_element_type=F32)

    def pv_group(j, is_a, tt, bb, levels):
        t = [pv_tile(j, is_a, tt, bb, h) for h in range(HPS)]
        for pr in range(2):
            base = {(r, h): jnp.concatenate(
                [t[h][bi * SQ + r * RQ:bi * SQ + (r + 1) * RQ] for bi in (2 * pr, 2 * pr + 1)], axis=0)
                for r in range(4) for h in range(HPS)}
            for i in range(7):
                r0 = i * MQ // 2 + (bb * 2 + pr) * RQ
                l1 = {(b0, b1): _comb(_LHS[i], lambda a: base[(2 * a[0] + b0, 2 * a[1] + b1)])
                      for b0 in range(2) for b1 in range(2)}
                if levels == 1:
                    ops = list(l1.values())
                else:
                    ops = [None] * 7
                for jj, v in enumerate(ops):
                    v = _comb(_LHS[jj], lambda t2: l1[t2]) if v is None else v
                    os_buf[r0:r0 + RQ, jj * DH:(jj + 1) * DH] = _pk(v)

    def attn_qproj(j, is_a, s, br, seq, levels=2):
        tts = [None] * 4

        def qk(g):
            tts[g] = qk_group(j, is_a, g)

        qproj(s, br, seq, qk, lambda g: pv_group(j, is_a, tts[g], g, levels))

    outs = []

    def final_oproj(s, br, chunks, with_qk):
        tts = None
        for c2, c0, tc in chunks:
            cc = c2 * NQ4 + c0

            def total(i):
                lhs = _upk(jnp.concatenate(
                    [os_buf[i * MQ // 2:(i + 1) * MQ // 2, b0 * QNH:(b0 + 1) * QNH] for b0 in range(2)],
                    axis=0))
                rhs = _operand(_RHS[i], lambda t: wo_buf[s, t[0] * QNH:(t[0] + 1) * QNH,
                                                         t[1] * NH + cc:t[1] * NH + cc + tc])
                m = jnp.dot(lhs, rhs, preferred_element_type=F32)
                return [_signed_sum([(1, m[r2 * MQ:(r2 + 1) * MQ])] +
                                    [(sg, accm[br, i * 7 + j, :, c0:c0 + tc])
                                     for j, sg in _OUT[(r2, c2 ^ _SWAP[i])].items()]) for r2 in range(2)]

            d = {}
            for i in (4, 1, 2, 0, 5, 3, 6):
                if with_qk and tts is None and d:
                    tts = [qk_group(NSB - 1, False, g) for g in range(4)]
                d[i] = total(i)
                for (r1, c1), terms in _OUT.items():
                    if i in terms and set(terms) <= set(d):
                        for r2 in range(2):
                            val = _signed_sum([(sg, d[k][r2]) for k, sg in terms.items()])
                            out_buf[br, :, r1, r2 * RQ:(r2 + 1) * RQ, c1 * NH + cc:c1 * NH + cc + tc] = (
                                val.reshape(B, RQ, tc).astype(BF16))
                if i in (5, 6):
                    outs.append(out_cp(br, (1 if i == 5 else 0) * NH + cc, tc))
                    outs[-1].start()
        return tts

    with jax.named_scope("xsA"):
        make_xs(0)
    with jax.named_scope("pro1"):
        qproj(0, 0, SEQ_0, None, None)
        attn_qproj(0, True, 1, 0, SEQ_1)
    with jax.named_scope("wait4"):
        wait_all(grp_r(5))
    with jax.named_scope("pro5"):
        oproj(0, 0, first=True, split=True)

    def body_a(s, carry):
        with jax.named_scope("waitA"):
            @pl.when((s & 1) == 0)
            def _():
                wait_all(grp_a_kv(s, dyn=True))

            wait_all(grp_a(s, dyn=True))

            @pl.when(s == LA - 1)
            def _():
                xb_cp().wait()
                make_xs(1)

        with jax.named_scope("bodyA"):
            attn_qproj(s, True, next_a(s), (s == LA - 1) * 1, SEQ_A)
            oproj(s, 0)
        return carry

    lax.fori_loop(1, LA, body_a, 0)

    def body_b(p, carry):
        with jax.named_scope("waitB"):
            wait_all(grp_b(p, dyn=True))
        with jax.named_scope("bodyB"):
            for k in range(BU):
                u = BU * p + k
                attn_qproj(u, False, NSB + u + 1, 1, SEQ_B)
                oproj(NSB + u, 1)
        return carry

    lax.fori_loop(0, NB, body_b, 0)

    with jax.named_scope("epi0"):
        wait_all(grp_e())
    with jax.named_scope("epi1"):
        attn_qproj(NSB - 2, False, LA, 0, SEQ_EB)
        oproj(NS - 2, 1)
        attn_qproj(LA, True, NS - 1, 1, SEQ_EA, levels=1)
        tts = final_oproj(LA, 0, ((0, 0, 256), (1, 0, 256)), True)
        for g in range(4):
            pv_group(NSB - 1, False, tts[g], g, 1)
        final_oproj(NS - 1, 1, ((0, 0, 256), (1, 0, 128), (1, 128, 128)), False)
    with jax.named_scope("tail"):
        sharp = jnp.logical_not(jnp.max(smax[...]) <= S_LIMIT)
        wait_all(outs)

    @pl.when(sharp)
    def _():
        def step(t, carry):
            br, bb, j = t >> 5, (t >> 3) & 3, t & 7
            is_a = br == 0

            def kv4(a_buf, b_buf, b):
                return jnp.where(is_a, jnp.concatenate([a_buf[b, j >> 1]] * HPS, axis=0), b_buf[b, j])

            xr = x_buf[br, pl.ds(bb * 4, 4)].reshape(MQ, D)
            q = jnp.dot(xr, wq_buf[br * NSB + j], preferred_element_type=F32).astype(BF16)
            pts = []
            for bi in range(4):
                q4 = jnp.concatenate(
                    [q[bi * SQ:(bi + 1) * SQ, h * DH:(h + 1) * DH] for h in range(HPS)], axis=0)
                pts.append(_softmax_cols(diag(lax.dot_general(
                    kv4(ka_buf, kb_buf, bb * 4 + bi), q4, NT, preferred_element_type=F32))))
            tt = jnp.concatenate(pts, axis=0).T
            v4 = [kv4(va_buf, vb_buf, bb * 4 + bi) for bi in range(4)]
            o = jnp.concatenate(
                [lax.dot_general(p_lhs(tt, h),
                                 jnp.concatenate([v[h * SK:(h + 1) * SK] for v in v4], axis=0),
                                 NN, preferred_element_type=F32) for h in range(HPS)], axis=1)
            m = jnp.dot(o.astype(BF16), wo_buf[br * NSB + j], preferred_element_type=F32)
            for c in range(4):
                acc = jnp.where(j == 0, 0.0, accm[0, c]) + m[:, c * NQ4:(c + 1) * NQ4]
                accm[0, c] = acc
                out_buf[br, pl.ds(bb * 4, 4), :, :, c * NQ4:(c + 1) * NQ4] = (
                    acc.astype(BF16).reshape(4, 2, SH, NQ4))
            return carry

        lax.fori_loop(0, 2 * (B // 4) * NSB, step, 0)
        for br in range(2):
            out_cp(br, 0, D).start()
        for br in range(2):
            out_cp(br, 0, D).wait()


@jax.jit
def pallas_concat_heads__gqa_block_cached__mha_block_cached__near_ridge_kernel(A_x, A_k_cache, A_v_cache, A_wq, A_wo, B_x, B_k_cache, B_v_cache, B_wq, B_wo):
    xa = A_x.reshape(B, 2, SH, D)
    xb = B_x.reshape(B, 2, SH, D)
    kb = B_k_cache.reshape(B, NSB, HPS * SK, DH)
    vb = B_v_cache.reshape(B, NSB, HPS * SK, DH)
    any_spec = pl.BlockSpec(memory_space=pl.ANY)
    out = pl.pallas_call(
        _kernel,
        in_specs=[any_spec] * 10,
        out_specs=any_spec,
        out_shape=jax.ShapeDtypeStruct((B, 2, SH, 2 * D), BF16),
        scratch_shapes=[
            pltpu.VMEM((2, B, 2, SH, D), BF16),
            pltpu.VMEM((B, HKV, SK, DH), BF16),
            pltpu.VMEM((B, HKV, SK, DH), BF16),
            pltpu.VMEM((B, NSB, HPS * SK, DH), BF16),
            pltpu.VMEM((B, NSB, HPS * SK, DH), BF16),
            pltpu.VMEM((NS, D, CH), BF16),
            pltpu.VMEM((NS, CH, D), BF16),
            pltpu.VMEM((M // 2, CH), U32),
            pltpu.VMEM((2, B, 2, SH, D), BF16),
            pltpu.VMEM((7 * MQ // 2, 7 * DH), U32),
            pltpu.VMEM((2, 49, MQ, NQ4), F32),
            pltpu.VMEM((11, MH, QNH), F32),
            pltpu.VMEM((4, SK, 4 * SQ), F32),
            pltpu.VMEM((2, 7 * MQ // 2, 7 * NQ4), U32),
            pltpu.SemaphoreType.DMA((N_SEM,)),
        ],
        compiler_params=pltpu.CompilerParams(vmem_limit_bytes=100 * 1024 * 1024,
                                             disable_semaphore_checks=True),
        name="fused_attn",
    )(xa, A_k_cache, A_v_cache, A_wq, A_wo, xb, kb, vb, B_wq, B_wo)
    return out.reshape(B, SQ, 2 * D)
```

```python
import numpy as np
import jax
import jax.numpy as jnp
from jax import lax
import jax.experimental.pallas as pl
import jax.experimental.pallas.tpu as pltpu

B, SQ, D, H, HKV, SK, DH = 16, 32, 1024, 32, 4, 32, 128
M = B * SQ
MH = M // 2
MQ = M // 4
SH, RQ = SQ // 2, SQ // 4
HPS = 4
CH = HPS * DH
NSB = H // HPS
NS = 2 * NSB
LA = NSB - 1
NH, NQ4 = D // 2, D // 4
QNH, QMQ = CH // 2, MH // 2
C_EXP2 = float(DH ** -0.5 * np.log2(np.e))
SCALE_BF16 = 0.08837890625
S_LIMIT = float(6.0 * DH ** 0.5)
NT = (((1,), (1,)), ((), ()))
NN = (((1,), (0,)), ((), ()))
F32 = jnp.float32
BF16 = jnp.bfloat16
U32 = jnp.uint32

_LHS = [((0, 0), (1, 1), -1), ((1, 0), (1, 1), -1), ((0, 0), None, 0), ((1, 1), None, 0),
        ((0, 0), (0, 1), -1), ((1, 0), (0, 0), -1), ((0, 1), (1, 1), -1)]
_RHS = [((0, 0), (1, 1), -1), ((0, 0), None, 0), ((0, 1), (1, 1), 1), ((1, 0), (0, 0), 1),
        ((1, 1), None, 0), ((0, 0), (0, 1), 1), ((1, 0), (1, 1), 1)]
_OUT = {(0, 0): {0: 1, 3: 1, 4: 1, 6: 1}, (0, 1): {2: 1, 4: -1},
        (1, 0): {1: 1, 3: 1}, (1, 1): {0: 1, 1: -1, 2: 1, 5: 1}}
_SWAP = (0, 1, 0, 0, 1, 1, 1)


def _o_order():
    nt = [1 if r[1] is None else 2 for r in _RHS]
    allp = [(i, j) for i in range(7) for j in range(7)]
    heavy, mid, light = ([p for p in allp if nt[p[0]] * nt[p[1]] == n] for n in (4, 2, 1))
    cheap = mid[:10] + light[2:] + mid[10:]
    seq = light[:2]
    while heavy or cheap:
        seq += heavy[:1] + cheap[:1]
        heavy, cheap = heavy[1:], cheap[1:]
    return tuple(seq)


O_SEQ = _o_order()


def _g(*idx):
    return [(i, n) for i in idx for n in range(7)]


def _q_order(slots, base=None):
    base = base or _g(1)[:2] + _g(0, 5, 6) + _g(1)[2:] + _g(3, 4, 2)
    seq = []
    for n, u in enumerate(base):
        seq += slots.get(n, "").split() + [u]
    return tuple(seq)


SEQ_A = _q_order({2: "q0 q1", 6: "q2 q3", 34: "p0 p1 p2 p3"})
SEQ_B = _q_order({3: "q0 q1 q2 q3", 21: "p0", 33: "p1", 35: "p2", 37: "p3"})
SEQ_EB = _q_order({6: "q0 q1 q2 q3", 20: "p0", 32: "p1", 34: "p2", 36: "p3"})
SEQ_EA = _q_order({2: "q0 q1", 6: "q2 q3", 20: "p0", 32: "p1", 34: "p2", 36: "p3"})
SEQ_0 = _q_order({0: "w0", 6: "w1", 20: "w2", 48: "w3"},
                 _g(1)[:6] + _g(4)[:2] + _g(1)[6:] + _g(4)[2:] + _g(0, 2, 5, 3, 6))
SEQ_1 = _q_order({3: "q0 q1", 7: "q2 q3", 19: "w4 p0 p1 p2 p3"}, _g(1, 4, 0, 2, 5, 3, 6))
XS = (1, 4, 2, 3, 0, 5, 6)

S_OUT = 0
S_A = 0
BU = 3
NB = (NSB - 2) // BU
S_B = LA
S_E = S_B + NB
S_X = S_E + 1
S_R = S_X + 4
N_SEM = S_R + 6


def _pk(x):
    return pltpu.bitcast(x.astype(BF16), U32)


def _upk(x):
    return pltpu.bitcast(x, BF16)


def _terms(spec):
    a, b, sg = spec
    return [(a, 1)] + ([(b, sg)] if b is not None else [])


def _signed_sum(items):
    items = sorted(items, key=lambda t: -t[0])
    acc = items[0][1]
    for sg, v in items[1:]:
        acc = acc + v if sg > 0 else acc - v
    return acc


def _comb(spec, get):
    return _signed_sum([(sg, get(t)) for t, sg in _terms(spec)])


def _operand(spec, ld):
    if spec[1] is None:
        return ld(spec[0])
    return _comb(spec, lambda t: ld(t).astype(F32)).astype(BF16)


def _softmax_cols(sc):
    m = jnp.max(sc, axis=0, keepdims=True)
    p = jnp.exp2((sc - m) * C_EXP2)
    l = jnp.sum(p, axis=0, keepdims=True)
    return p * (1.0 / l)


def _softmax_cols_bf16(sc):
    sc = sc.astype(BF16).astype(F32) * SCALE_BF16
    sc = sc.astype(BF16).astype(F32)
    p = jnp.exp(sc - jnp.max(sc, axis=0, keepdims=True))
    return p * (1.0 / jnp.sum(p, axis=0, keepdims=True))


def _kernel(xa, ka, va, wqa, woa, xb, kb, vb, wqb, wob, out,
            x_buf, ka_buf, va_buf, kb_buf, vb_buf, wq_buf, wo_buf,
            q_buf, out_buf, os_buf, accm, mq_buf, smax, xs_buf, sems):
    cp = pltpu.make_async_copy

    def wq_cp(s, sem, dyn=False):
        dst = wq_buf.at[s]
        src = dst if dyn else (wqa if s < NSB else wqb).at[:, pl.ds((s % NSB) * CH, CH)]
        return cp(src, dst, sems.at[sem])

    def wo_cp(s, sem, dyn=False):
        dst = wo_buf.at[s]
        src = dst if dyn else (woa if s < NSB else wob).at[pl.ds((s % NSB) * CH, CH), :]
        return cp(src, dst, sems.at[sem])

    def kv_cp(src, dst, j, n, sem, dyn=False):
        d = dst.at[:, pl.ds(j, n)]
        return cp(d if dyn else src.at[:, pl.ds(j, n)], d, sems.at[sem])

    def wq_quad_cp(s, a, b, sem):
        r, c = pl.ds(a * NH, NH), b * QNH
        return cp(wqa.at[r, pl.ds(s * CH + c, QNH)], wq_buf.at[s, r, pl.ds(c, QNH)], sems.at[sem])

    def grp_x(g, dyn=False):
        cs = []
        for b0 in (2 * g, 8 + 2 * g):
            d = x_buf.at[0, pl.ds(b0, 2)]
            cs.append(cp(d if dyn else xa.at[pl.ds(b0, 2)], d, sems.at[S_X + g]))
        return cs

    def grp_r(n):
        sem = S_R + n
        if n < 2:
            return [wq_quad_cp(0, n, n, sem)]
        if n == 2:
            return [wq_quad_cp(0, 0, 1, sem), wq_quad_cp(0, 1, 0, sem)]
        if n == 3:
            return [wq_quad_cp(1, 0, 0, sem), kv_cp(ka, ka_buf, 0, 1, sem), wq_quad_cp(1, 1, 1, sem)]
        if n == 4:
            return [wq_quad_cp(1, 0, 1, sem), kv_cp(va, va_buf, 0, 1, sem), wq_quad_cp(1, 1, 0, sem)]
        return [wo_cp(0, sem)]

    def next_a(s):
        return s + 1 + (s == LA - 1) * 1

    def grp_a(s, dyn=False):
        return [wq_cp(next_a(s), S_A + s, dyn), wo_cp(s, S_A + s, dyn)]

    def grp_a_kv(s, dyn=False):
        g = s >> 1
        return [kv_cp(ka, ka_buf, g, 1, S_A + s, dyn), kv_cp(va, va_buf, g, 1, S_A + s, dyn)]

    def xb_cp():
        return cp(xb, x_buf.at[1], sems.at[S_A + LA - 1])

    def grp_b(p, dyn=False):
        u, sem = BU * p, S_B + p
        g = [kv_cp(kb, kb_buf, u, BU, sem, dyn), kv_cp(vb, vb_buf, u, BU, sem, dyn)]
        for k in range(BU):
            g += [wq_cp(NSB + u + k + 1, sem, dyn), wo_cp(NSB + u + k, sem, dyn)]
        return g

    def grp_e():
        return [kv_cp(kb, kb_buf, NSB - 2, 2, S_E), wq_cp(LA, S_E), kv_cp(vb, vb_buf, NSB - 2, 2, S_E),
                wo_cp(NS - 2, S_E), wq_cp(NS - 1, S_E), wo_cp(LA, S_E), wo_cp(NS - 1, S_E)]

    def out_cp(br, c0, nc):
        return cp(out_buf.at[br, :, :, :, pl.ds(c0, nc)],
                  out.at[:, :, :, pl.ds(br * D + c0, nc)], sems.at[S_OUT])

    def wait_all(cs):
        for c in cs:
            c.wait()

    for g in range(4):
        for c in grp_x(g):
            c.start()
    for n in range(6):
        for c in grp_r(n):
            c.start()
    for s in range(1, LA):
        if s == LA - 1:
            xb_cp().start()
        for c in (grp_a_kv(s) if s % 2 == 0 else []) + grp_a(s):
            c.start()
    for p in range(NB):
        for c in grp_b(p):
            c.start()
    for c in grp_e():
        c.start()

    def zero_one(k, carry):
        accm[1, k] = jnp.zeros(accm.shape[2:], F32)
        return carry

    lax.fori_loop(0, 25, zero_one, 0)
    smax[...] = jnp.zeros(smax.shape, F32)

    lane_g = lax.broadcasted_iota(jnp.int32, (SK, 4 * SQ), 1) // SQ

    def xs_rows(br, b):
        r8 = pl.multiple_of(b * 8, 8)
        for c in range(0, NQ4, DH):
            blk = {(a0, b0, kq): x_buf[br, b0 * 8 + b, a0, :, kq * NQ4 + c:kq * NQ4 + c + DH].astype(F32)
                   for a0 in range(2) for b0 in range(2) for kq in range(4)}
            for n, i in enumerate(XS):
                l1 = {(b0, b1): _comb(_LHS[i], lambda a: blk[(a[0], b0, 2 * a[1] + b1)])
                      for b0 in range(2) for b1 in range(2)}
                rows = pl.ds(n * (MQ // 2) + r8, 8)
                for j in range(7):
                    if _LHS[i][1] is not None or _LHS[j][1] is not None:
                        xs_buf.at[br][rows, j * NQ4 + c:j * NQ4 + c + DH] = _pk(
                            _comb(_LHS[j], lambda t: l1[t]))

    def make_xs(br):
        def pair(g, carry):
            if br == 0:
                wait_all(grp_x(g, dyn=True))
            xs_rows(br, 2 * g)
            xs_rows(br, 2 * g + 1)
            if br == 0:
                lax.fori_loop(25 + 6 * g, 31 + 6 * g, zero_one, 0)
            return carry
        lax.fori_loop(0, 4, pair, 0)

    def q_sub(s, br, i, j, cache):
        if _LHS[i][1] is not None or _LHS[j][1] is not None:
            n = XS.index(i)
            lhs = _upk(xs_buf[br, n * (MQ // 2):(n + 1) * (MQ // 2), j * NQ4:(j + 1) * NQ4])
        else:
            a, b = _LHS[i][0], _LHS[j][0]
            c0 = (2 * a[1] + b[1]) * NQ4
            lhs = x_buf[br, b[0] * 8:(b[0] + 1) * 8, a[0], :, c0:c0 + NQ4].reshape(MQ, NQ4)

        def ld(a, b):
            r, c = 2 * a[0] + b[0], 2 * a[1] + (b[1] ^ _SWAP[i])
            return wq_buf[s, r * NQ4:(r + 1) * NQ4, c * DH:(c + 1) * DH]

        if _RHS[i][1] is None:
            rhs = _operand(_RHS[j], lambda b: ld(_RHS[i][0], b))
        else:
            def sub(b):
                if (i, b) not in cache:
                    cache[(i, b)] = _comb(_RHS[i], lambda a: ld(a, b).astype(F32))
                return cache[(i, b)]
            rhs = _comb(_RHS[j], sub).astype(BF16)
        return jnp.dot(lhs, rhs, preferred_element_type=F32)

    def quad(slot, k):
        return mq_buf.at[slot].at[(k >> 1) * MQ:((k >> 1) + 1) * MQ, (k & 1) * DH:((k & 1) + 1) * DH]

    def qproj(s, br, seq, qk, pv):
        left = {(blk, k): len(terms) for blk, terms in _OUT.items() for k in range(4)}
        slot_of = {(1, 1): 0, (0, 0): 1, (0, 1): 2, (1, 0): 3}
        neg = {}
        cache = {}

        def emit(i, r2, c2, v):
            k = 2 * r2 + c2
            for blk, terms in _OUT.items():
                if i not in terms:
                    continue
                ref = quad(slot_of[blk], k)
                first = left[(blk, k)] == len(terms)
                left[(blk, k)] -= 1
                if first:
                    neg[(blk, k)] = terms[i] < 0
                    ref[...] = v
                    continue
                if neg[(blk, k)]:
                    assert terms[i] > 0
                    tot, neg[(blk, k)] = v - ref[...], False
                else:
                    tot = ref[...] + v if terms[i] > 0 else ref[...] - v
                if left[(blk, k)]:
                    ref[...] = tot
                else:
                    r0, c0 = blk[0] * QMQ + r2 * (MQ // 2), blk[1] * QNH + c2 * DH
                    q_buf[r0:r0 + MQ // 2, c0:c0 + DH] = _pk(tot)

        def inner(i, n):
            t = lambda k: quad(4 + XS.index(i), k)
            done = lambda r2, c2, v: emit(i, r2, c2 ^ _SWAP[i], v)
            if n == 0:
                t(0)[...] = q_sub(s, br, i, 1, cache)
            elif n == 1:
                t(1)[...] = q_sub(s, br, i, 4, cache)
            elif n == 2:
                p0 = q_sub(s, br, i, 0, cache)
                t(2)[...] = p0 - t(0)[...]
                t(3)[...] = p0 + t(1)[...]
            elif n == 3:
                p2 = q_sub(s, br, i, 2, cache)
                done(0, 1, p2 - t(1)[...])
                t(2)[...] += p2
            elif n == 4:
                p3 = q_sub(s, br, i, 3, cache)
                done(1, 0, p3 + t(0)[...])
                t(3)[...] += p3
            elif n == 5:
                done(1, 1, t(2)[...] + q_sub(s, br, i, 5, cache))
            else:
                done(0, 0, t(3)[...] + q_sub(s, br, i, 6, cache))

        for u in seq:
            if isinstance(u, str):
                {"q": qk, "p": pv, "w": lambda n: wait_all(grp_r(n))}[u[0]](int(u[1]))
            else:
                inner(*u)

    def o_prod(s, i, j, r0, nr):
        ts = [(s1 * s2, 2 * a[0] + b[0], 2 * a[1] + (b[1] ^ _SWAP[i]))
              for a, s1 in _terms(_RHS[i]) for b, s2 in _terms(_RHS[j])]
        ld = lambda r, c: wo_buf[s, r * DH:(r + 1) * DH, c * NQ4:(c + 1) * NQ4]
        if len(ts) == 1:
            rhs = ld(ts[0][1], ts[0][2])
        else:
            rhs = _signed_sum([(sg, ld(r, c).astype(F32)) for sg, r, c in ts]).astype(BF16)
        lhs = _upk(os_buf[(i * MQ + r0) // 2:(i * MQ + r0 + nr) // 2, j * DH:(j + 1) * DH])
        return jnp.dot(lhs, rhs, preferred_element_type=F32)

    def oproj(s, br, first=False, split=False):
        for n, (i, j) in enumerate(O_SEQ):
            for r0, nr in (((0, MQ // 2), (MQ // 2, MQ // 2)) if split and n == 0 else ((0, MQ),)):
                m = o_prod(s, i, j, r0, nr)
                if not first:
                    m = accm[br, i * 7 + j, r0:r0 + nr] + m
                accm[br, i * 7 + j, r0:r0 + nr] = m

    def diag(st):
        sc = st[0:SK]
        for h in range(1, HPS):
            sc = jnp.where(lane_g == h, st[h * SK:(h + 1) * SK], sc)
        return sc

    def scores(j, is_a, b, q4):
        if is_a:
            return lax.dot_general(ka_buf[b, j >> 1], q4, NT, preferred_element_type=F32)
        return diag(lax.dot_general(kb_buf[b, j], q4, NT, preferred_element_type=F32))

    def p_lhs(tt, h):
        ph = tt[h * SQ:(h + 1) * SQ]
        return jnp.concatenate([jnp.where(lane_g == bi, ph, 0.0) for bi in range(4)], axis=0).astype(BF16)

    def qk_group(j, is_a, bb):
        pts = []
        big = None
        for b in range(bb * 4, bb * 4 + 4):
            q4 = _upk(jnp.concatenate(
                [q_buf[half * QMQ + b * 8:half * QMQ + (b + 1) * 8, h * DH:(h + 1) * DH]
                 for h in range(HPS) for half in range(2)], axis=0))
            sc = scores(j, is_a, b, q4)
            big = jnp.abs(sc) if big is None else jnp.maximum(big, jnp.abs(sc))
            pts.append(_softmax_cols(sc))
        smax[bb] = jnp.maximum(smax[bb], big)
        return jnp.concatenate(pts, axis=0).T

    def pv_tile(j, is_a, tt, bb, h):
        lhs = p_lhs(tt, h)
        if is_a:
            vh = jnp.concatenate([va_buf[bb * 4 + bi, j >> 1] for bi in range(4)], axis=0)
        else:
            vh = jnp.concatenate(
                [vb_buf[bb * 4 + bi, j, h * SK:(h + 1) * SK, :] for bi in range(4)], axis=0)
        return lax.dot_general(lhs, vh, NN, preferred_element_type=F32)

    def pv_group(j, is_a, tt, bb, levels):
        t = [pv_tile(j, is_a, tt, bb, h) for h in range(HPS)]
        for pr in range(2):
            base = {(r, h): jnp.concatenate(
                [t[h][bi * SQ + r * RQ:bi * SQ + (r + 1) * RQ] for bi in (2 * pr, 2 * pr + 1)], axis=0)
                for r in range(4) for h in range(HPS)}
            for i in range(7):
                r0 = i * MQ // 2 + (bb * 2 + pr) * RQ
                l1 = {(b0, b1): _comb(_LHS[i], lambda a: base[(2 * a[0] + b0, 2 * a[1] + b1)])
                      for b0 in range(2) for b1 in range(2)}
                if levels == 1:
                    ops = list(l1.values())
                else:
                    ops = [None] * 7
                for jj, v in enumerate(ops):
                    v = _comb(_LHS[jj], lambda t2: l1[t2]) if v is None else v
                    os_buf[r0:r0 + RQ, jj * DH:(jj + 1) * DH] = _pk(v)

    def attn_qproj(j, is_a, s, br, seq, levels=2):
        tts = [None] * 4

        def qk(g):
            tts[g] = qk_group(j, is_a, g)

        qproj(s, br, seq, qk, lambda g: pv_group(j, is_a, tts[g], g, levels))

    outs = []

    def final_oproj(s, br, chunks, with_qk):
        tts = None
        for c2, c0, tc in chunks:
            cc = c2 * NQ4 + c0

            def total(i):
                lhs = _upk(jnp.concatenate(
                    [os_buf[i * MQ // 2:(i + 1) * MQ // 2, b0 * QNH:(b0 + 1) * QNH] for b0 in range(2)],
                    axis=0))
                rhs = _operand(_RHS[i], lambda t: wo_buf[s, t[0] * QNH:(t[0] + 1) * QNH,
                                                         t[1] * NH + cc:t[1] * NH + cc + tc])
                m = jnp.dot(lhs, rhs, preferred_element_type=F32)
                return [_signed_sum([(1, m[r2 * MQ:(r2 + 1) * MQ])] +
                                    [(sg, accm[br, i * 7 + j, :, c0:c0 + tc])
                                     for j, sg in _OUT[(r2, c2 ^ _SWAP[i])].items()]) for r2 in range(2)]

            d = {}
            for i in (4, 1, 2, 0, 5, 3, 6):
                if with_qk and tts is None and d:
                    tts = [qk_group(NSB - 1, False, g) for g in range(4)]
                d[i] = total(i)
                for (r1, c1), terms in _OUT.items():
                    if i in terms and set(terms) <= set(d):
                        for r2 in range(2):
                            val = _signed_sum([(sg, d[k][r2]) for k, sg in terms.items()])
                            out_buf[br, :, r1, r2 * RQ:(r2 + 1) * RQ, c1 * NH + cc:c1 * NH + cc + tc] = (
                                val.reshape(B, RQ, tc).astype(BF16))
                if i in (5, 6):
                    outs.append(out_cp(br, (1 if i == 5 else 0) * NH + cc, tc))
                    outs[-1].start()
        return tts

    with jax.named_scope("xsA"):
        make_xs(0)
    with jax.named_scope("pro1"):
        qproj(0, 0, SEQ_0, None, None)
        attn_qproj(0, True, 1, 0, SEQ_1)
    with jax.named_scope("wait4"):
        wait_all(grp_r(5))
    with jax.named_scope("pro5"):
        oproj(0, 0, first=True, split=True)

    def body_a(s, carry):
        with jax.named_scope("waitA"):
            @pl.when((s & 1) == 0)
            def _():
                wait_all(grp_a_kv(s, dyn=True))

            wait_all(grp_a(s, dyn=True))

            @pl.when(s == LA - 1)
            def _():
                xb_cp().wait()
                make_xs(1)

        with jax.named_scope("bodyA"):
            attn_qproj(s, True, next_a(s), (s == LA - 1) * 1, SEQ_A)
            oproj(s, 0)
        return carry

    lax.fori_loop(1, LA, body_a, 0)

    def body_b(p, carry):
        with jax.named_scope("waitB"):
            wait_all(grp_b(p, dyn=True))
        with jax.named_scope("bodyB"):
            for k in range(BU):
                u = BU * p + k
                attn_qproj(u, False, NSB + u + 1, 1, SEQ_B)
                oproj(NSB + u, 1)
        return carry

    lax.fori_loop(0, NB, body_b, 0)

    with jax.named_scope("epi0"):
        wait_all(grp_e())
    with jax.named_scope("epi1"):
        attn_qproj(NSB - 2, False, LA, 0, SEQ_EB)
        oproj(NS - 2, 1)
        attn_qproj(LA, True, NS - 1, 1, SEQ_EA, levels=1)
        tts = final_oproj(LA, 0, ((0, 0, 256), (1, 0, 256)), True)
        for g in range(4):
            pv_group(NSB - 1, False, tts[g], g, 1)
        final_oproj(NS - 1, 1, ((0, 0, 256), (1, 0, 128), (1, 128, 128)), False)
    with jax.named_scope("tail"):
        sharp = jnp.logical_not(jnp.max(smax[...]) <= S_LIMIT)
        wait_all(outs)

    @pl.when(sharp)
    def _():
        def step(t, carry):
            br, bb, j = t >> 5, (t >> 3) & 3, t & 7
            is_a = br == 0

            def kv4(a_buf, b_buf, b):
                return jnp.where(is_a, jnp.concatenate([a_buf[b, j >> 1]] * HPS, axis=0), b_buf[b, j])

            xr = x_buf[br, pl.ds(bb * 4, 4)].reshape(MQ, D)
            q = jnp.dot(xr, wq_buf[br * NSB + j], preferred_element_type=F32).astype(BF16)
            pts = []
            for bi in range(4):
                q4 = jnp.concatenate(
                    [q[bi * SQ:(bi + 1) * SQ, h * DH:(h + 1) * DH] for h in range(HPS)], axis=0)
                pts.append(_softmax_cols_bf16(diag(lax.dot_general(
                    kv4(ka_buf, kb_buf, bb * 4 + bi), q4, NT, preferred_element_type=F32))))
            tt = jnp.concatenate(pts, axis=0).T
            v4 = [kv4(va_buf, vb_buf, bb * 4 + bi) for bi in range(4)]
            o = jnp.concatenate(
                [lax.dot_general(p_lhs(tt, h),
                                 jnp.concatenate([v[h * SK:(h + 1) * SK] for v in v4], axis=0),
                                 NN, preferred_element_type=F32) for h in range(HPS)], axis=1)
            m = jnp.dot(o.astype(BF16), wo_buf[br * NSB + j], preferred_element_type=F32)
            for c in range(4):
                acc = jnp.where(j == 0, 0.0, accm[0, c]) + m[:, c * NQ4:(c + 1) * NQ4]
                accm[0, c] = acc
                out_buf[br, pl.ds(bb * 4, 4), :, :, c * NQ4:(c + 1) * NQ4] = (
                    acc.astype(BF16).reshape(4, 2, SH, NQ4))
            return carry

        lax.fori_loop(0, 2 * (B // 4) * NSB, step, 0)
        for br in range(2):
            out_cp(br, 0, D).start()
        for br in range(2):
            out_cp(br, 0, D).wait()


@jax.jit
def pallas_concat_heads__gqa_block_cached__mha_block_cached__near_ridge_kernel(A_x, A_k_cache, A_v_cache, A_wq, A_wo, B_x, B_k_cache, B_v_cache, B_wq, B_wo):
    xa = A_x.reshape(B, 2, SH, D)
    xb = B_x.reshape(B, 2, SH, D)
    kb = B_k_cache.reshape(B, NSB, HPS * SK, DH)
    vb = B_v_cache.reshape(B, NSB, HPS * SK, DH)
    any_spec = pl.BlockSpec(memory_space=pl.ANY)
    out = pl.pallas_call(
        _kernel,
        in_specs=[any_spec] * 10,
        out_specs=any_spec,
        out_shape=jax.ShapeDtypeStruct((B, 2, SH, 2 * D), BF16),
        scratch_shapes=[
            pltpu.VMEM((2, B, 2, SH, D), BF16),
            pltpu.VMEM((B, HKV, SK, DH), BF16),
            pltpu.VMEM((B, HKV, SK, DH), BF16),
            pltpu.VMEM((B, NSB, HPS * SK, DH), BF16),
            pltpu.VMEM((B, NSB, HPS * SK, DH), BF16),
            pltpu.VMEM((NS, D, CH), BF16),
            pltpu.VMEM((NS, CH, D), BF16),
            pltpu.VMEM((M // 2, CH), U32),
            pltpu.VMEM((2, B, 2, SH, D), BF16),
            pltpu.VMEM((7 * MQ // 2, 7 * DH), U32),
            pltpu.VMEM((2, 49, MQ, NQ4), F32),
            pltpu.VMEM((11, MH, QNH), F32),
            pltpu.VMEM((4, SK, 4 * SQ), F32),
            pltpu.VMEM((2, 7 * MQ // 2, 7 * NQ4), U32),
            pltpu.SemaphoreType.DMA((N_SEM,)),
        ],
        compiler_params=pltpu.CompilerParams(vmem_limit_bytes=100 * 1024 * 1024,
                                             disable_semaphore_checks=True),
        name="fused_attn",
    )(xa, A_k_cache, A_v_cache, A_wq, A_wo, xb, kb, vb, B_wq, B_wo)
    return out.reshape(B, SQ, 2 * D)
```
